```python
import jax
import jax.numpy as jnp

def _softmax(x, axis=-1):
    return jax.nn.softmax(x, axis=axis)

def _gelu(x):
    return jax.nn.gelu(x, approximate=True)

def _silu(x):
    return jax.nn.silu(x)

def _sigmoid(x):
    return jax.nn.sigmoid(x)

def _layernorm(x, axis=-1, eps=1e-05):
    m = jnp.mean(x, axis=axis, keepdims=True)
    v = jnp.var(x, axis=axis, keepdims=True)
    return (x - m) / jnp.sqrt(v + eps)

def _scatter_add(tgt, idx, src, axis=0):
    return tgt.at[idx].add(src)

def _segment_sum(src, seg, n):
    return jax.ops.segment_sum(src, seg, n)

class _Rng:

    def __init__(self, key):
        self._k = key

    def _next(self):
        self._k, sub = jax.random.split(self._k)
        return sub

    def normal(self, shape):
        return jax.random.normal(self._next(), shape, dtype=jnp.bfloat16)

    def randint(self, lo, hi, shape):
        return jax.random.randint(self._next(), shape, lo, hi, dtype=jnp.int32)

    def uniform(self, shape, lo=0.0, hi=1.0):
        return jax.random.uniform(self._next(), shape, jnp.bfloat16, lo, hi)

    def permutation(self, n):
        return jax.random.permutation(self._next(), n)
kernel_name = 'standalone__conformer_family_conformer__speech'

def setup_inputs():
    _rng = _Rng(jax.random.key(int.from_bytes(__import__("os").urandom(4), "little")))
    _w = lambda a: (lambda t: t.astype(jnp.bfloat16) if jnp.issubdtype(t.dtype, jnp.floating) else t)(jnp.asarray(a))
    B, T, D, K = (2, 4000, 512, 15)
    F = 4 * D
    s = D ** (-0.5)
    sf = F ** (-0.5)
    return {'x': _w((lambda *s: _rng.normal(s) * 0.05)(B, T, D)), 'w_ff1_a': _w((lambda *s: _rng.normal(s) * 0.05)(D, F) * s), 'w_ff1_b': _w((lambda *s: _rng.normal(s) * 0.05)(F, D) * sf), 'w_q': _w((lambda *s: _rng.normal(s) * 0.05)(D, D) * s), 'w_k': _w((lambda *s: _rng.normal(s) * 0.05)(D, D) * s), 'w_v': _w((lambda *s: _rng.normal(s) * 0.05)(D, D) * s), 'w_o': _w((lambda *s: _rng.normal(s) * 0.05)(D, D) * s), 'w_pw1': _w((lambda *s: _rng.normal(s) * 0.05)(D, 2 * D) * s), 'dw': _w((lambda *s: _rng.normal(s) * 0.05)(K, D) * K ** (-0.5)), 'w_pw2': _w((lambda *s: _rng.normal(s) * 0.05)(D, D) * s), 'w_ff2_a': _w((lambda *s: _rng.normal(s) * 0.05)(D, F) * s), 'w_ff2_b': _w((lambda *s: _rng.normal(s) * 0.05)(F, D) * sf)}

def reference(x, w_ff1_a, w_ff1_b, w_q, w_k, w_v, w_o, w_pw1, dw, w_pw2, w_ff2_a, w_ff2_b):
    B, T, D = x.shape
    K = dw.shape[0]
    scale = D ** (-0.5)
    h = _layernorm(x, axis=-1)
    h = _silu(h @ w_ff1_a) @ w_ff1_b
    x1 = x + 0.5 * h
    h = _layernorm(x1, axis=-1)
    q = h @ w_q
    k = h @ w_k
    v = h @ w_v
    scores = jnp.einsum('btd,bsd->bts', q, k) * scale
    p = _softmax(scores, axis=-1)
    attn = jnp.einsum('bts,bsd->btd', p, v) @ w_o
    x2 = x1 + attn
    h = _layernorm(x2, axis=-1)
    h = h @ w_pw1
    a = h[..., :D].copy()
    b = h[..., D:].copy()
    h = a * _sigmoid(b)
    pad = K // 2
    hp = jnp.pad(h, ((0, 0), (pad, K - 1 - pad), (0, 0)))
    dc = jnp.zeros_like(h)
    for i in range(K):
        dc = dc + hp[:, i:i + T, :] * dw[i][None, None, :]
    flat = dc.reshape(-1, D)
    mu = flat.mean(0)
    var = ((flat - mu) ** 2).mean(0)
    dc = (dc - mu[None, None, :]) / jnp.sqrt(var[None, None, :] + 1e-05)
    h = _silu(dc) @ w_pw2
    x3 = x2 + h
    h = _layernorm(x3, axis=-1)
    h = _silu(h @ w_ff2_a) @ w_ff2_b
    x4 = x3 + 0.5 * h
    return _layernorm(x4, axis=-1)
```

```python
import functools
import math
import jax
import jax.numpy as jnp
from jax import lax
import jax.experimental.pallas as pl
import jax.experimental.pallas.tpu as pltpu

TM1 = 400
TM2 = 400
TM4 = 400
EPS = 1e-5
LOG2E = 1.4426950408889634

bf16 = jnp.bfloat16
f32 = jnp.float32


def _ln(x):
    m = jnp.mean(x, axis=-1, keepdims=True)
    c = x - m
    v = jnp.mean(c * c, axis=-1, keepdims=True)
    return c * lax.rsqrt(v + EPS)


def _sigmoid(x):
    return 0.5 * jnp.tanh(0.5 * x) + 0.5


def _silu(x):
    return x * _sigmoid(x)


def _dot(a, b):
    return jnp.dot(a, b, preferred_element_type=f32)


def _dot_nt(a, b):
    return lax.dot_general(a, b, (((1,), (1,)), ((), ())), preferred_element_type=f32)


def _kernel(x_ref, w1a, w1b, wq, wk, wv, wo, wpw1, dw_ref, wpw2, w2a, w2b, out_ref,
            xr, hb, qb, vb, gb, dcb, wqv, *, B, T, D, K, TP):
    N = B * T
    PAD = K // 2
    GOFF = 8
    GS = T + 2 * GOFF

    wqv[:, :D] = (_dot_nt(wq[...], wk[...]) * (D ** -0.5 * LOG2E)).astype(bf16)
    wqv[:, D:] = _dot(wv[...], wo[...]).astype(bf16)
    for b in range(B):
        hb[b, T:, :] = jnp.zeros((TP - T, D), bf16)
        vb[b, T:, :] = jnp.zeros((TP - T, D), bf16)
        gb[b * GS: b * GS + GOFF, :] = jnp.zeros((GOFF, D), f32)
        gb[b * GS + GOFF + T: (b + 1) * GS, :] = jnp.zeros((GOFF, D), f32)

    n1 = T // TM1

    def p1(i, c):
        b = i // n1
        t = pl.multiple_of((i % n1) * TM1, 16)
        r = pl.multiple_of(i * TM1, 16)
        xt = x_ref[pl.ds(r, TM1), :].astype(f32)
        hn = _ln(xt).astype(bf16)
        u = _silu(_dot(hn, w1a[...])).astype(bf16)
        x1 = xt + 0.5 * _dot(u, w1b[...])
        xr[pl.ds(r, TM1), :] = x1
        h = _ln(x1).astype(bf16)
        hb[b, pl.ds(t, TM1), :] = h
        qv = _dot(h, wqv[...])
        qb[pl.ds(r, TM1), :] = qv[:, :D].astype(bf16)
        vb[b, pl.ds(t, TM1), :] = qv[:, D:].astype(bf16)
        return c

    lax.fori_loop(0, B * n1, p1, 0)

    n2 = T // TM2

    def p2(i, c):
        b = i // n2
        t = (i % n2) * TM2
        r = pl.multiple_of(i * TM2, 16)
        q = qb[pl.ds(r, TM2), :]
        s = _dot_nt(q, hb[b])
        col = lax.broadcasted_iota(jnp.int32, (TM2, TP), 1)
        s = jnp.where(col < T, s, -1e30)
        m = jnp.max(s, axis=-1, keepdims=True)
        p = jnp.exp2(s - m)
        l = jnp.sum(p, axis=-1, keepdims=True)
        o = _dot(p.astype(bf16), vb[b])
        x2 = xr[pl.ds(r, TM2), :] + o * (1.0 / l)
        xr[pl.ds(r, TM2), :] = x2
        hn = _ln(x2).astype(bf16)
        y = _dot(hn, wpw1[...])
        g = y[:, :D] * _sigmoid(y[:, D:])
        go = pl.multiple_of(b * GS + GOFF + t, 8)
        gb[pl.ds(go, TM2), :] = g
        return c

    lax.fori_loop(0, B * n2, p2, 0)

    TC = 400
    nc = T // TC
    dwv = dw_ref[...].astype(f32)

    def p3(i, c):
        b = i // nc
        t = (i % nc) * TC
        go = pl.multiple_of(b * GS + t, 8)
        win = gb[pl.ds(go, TC + 2 * GOFF), :]
        acc = jnp.zeros((TC, D), f32)
        for k in range(K):
            o = GOFF - PAD + k
            acc = acc + win[o:o + TC, :] * dwv[k:k + 1, :]
        r = pl.multiple_of(i * TC, 8)
        dcb[pl.ds(r, TC), :] = acc
        return c + jnp.sum(acc, axis=0, keepdims=True)

    tot = lax.fori_loop(0, B * nc, p3, jnp.zeros((1, D), f32))
    mu = tot * (1.0 / N)

    def p3b(i, c):
        r = pl.multiple_of(i * TC, 8)
        d = dcb[pl.ds(r, TC), :] - mu
        return c + jnp.sum(d * d, axis=0, keepdims=True)

    var = lax.fori_loop(0, B * nc, p3b, jnp.zeros((1, D), f32)) * (1.0 / N)
    rs = lax.rsqrt(var + EPS)

    def p4(i, c):
        r = pl.multiple_of(i * TM4, 16)
        z = _silu((dcb[pl.ds(r, TM4), :] - mu) * rs).astype(bf16)
        x3 = xr[pl.ds(r, TM4), :] + _dot(z, wpw2[...])
        hn = _ln(x3).astype(bf16)
        u = _silu(_dot(hn, w2a[...])).astype(bf16)
        x4 = x3 + 0.5 * _dot(u, w2b[...])
        out_ref[pl.ds(r, TM4), :] = _ln(x4).astype(out_ref.dtype)
        return c

    lax.fori_loop(0, N // TM4, p4, 0)


@jax.jit
def pallas_standalone__conformer_family_conformer__speech_kernel(
    x, w_ff1_a, w_ff1_b, w_q, w_k, w_v, w_o, w_pw1, dw, w_pw2, w_ff2_a, w_ff2_b):
    B, T, D = x.shape
    K = dw.shape[0]
    N = B * T
    TP = (T + 127) // 128 * 128
    kern = functools.partial(_kernel, B=B, T=T, D=D, K=K, TP=TP)
    vm = pl.BlockSpec(memory_space=pltpu.VMEM)
    out = pl.pallas_call(
        kern,
        out_shape=jax.ShapeDtypeStruct((N, D), x.dtype),
        in_specs=[vm] * 12,
        out_specs=vm,
        scratch_shapes=[
            pltpu.VMEM((N, D), f32),
            pltpu.VMEM((B, TP, D), bf16),
            pltpu.VMEM((N, D), bf16),
            pltpu.VMEM((B, TP, D), bf16),
            pltpu.VMEM((B * (T + 16), D), f32),
            pltpu.VMEM((N, D), f32),
            pltpu.VMEM((D, 2 * D), bf16),
        ],
        compiler_params=pltpu.CompilerParams(vmem_limit_bytes=120 * 1024 * 1024),
    )(x.reshape(N, D), w_ff1_a, w_ff1_b, w_q, w_k, w_v, w_o, w_pw1, dw, w_pw2, w_ff2_a, w_ff2_b)
    return out.reshape(B, T, D)
```

```python
import functools
import jax
import jax.numpy as jnp
from jax import lax
import jax.experimental.pallas as pl
import jax.experimental.pallas.tpu as pltpu

H = 400
W = 512
EPS = 1e-5
LOG2E = 1.4426950408889634
NEG = -1e30
ELAG = 3
UPO = (1, 2, 0, 5, 3, 4, 6)
DNO = (1, 3, 6, 0, 2, 4, 5)
PR = (40, 40, 40, 40)
P2G = 16
PCH = 4
ECH = 1
PEEL_UNROLL = True
VMEM_LIMIT = 127 * 1024 * 1024

bf16 = jnp.bfloat16
f32 = jnp.float32


def _ln(x):
    m = jnp.mean(x, axis=-1, keepdims=True)
    c = x - m
    v = jnp.mean(c * c, axis=-1, keepdims=True)
    return c * lax.rsqrt(v + EPS)


def _hsilu(h):
    return h * jnp.tanh(h) + h


def _hglu(a, b):
    return a * jnp.tanh(b) + a


def _dot(a, b):
    return jnp.dot(a, b, preferred_element_type=f32)


def _dot_nt(a, b):
    return lax.dot_general(a, b, (((1,), (1,)), ((), ())), preferred_element_type=f32)


def _a_sums(A11, A12, A21, A22):
    return [A11 + A22, A21 + A22, A11, A22, A11 + A12, A21 - A11, A12 - A22]


def _a_ops(*q):
    return [t.astype(bf16) for t in _a_sums(*q)]


def _b_ops(B11, B12, B21, B22):
    return [t.astype(bf16) for t in
            (B11 + B22, B11, B12 - B22, B21 - B11, B22, B11 + B12, B21 + B22)]


def _smm(a, w, order=UPO, dot=_dot):
    M = [None] * 7
    for k in order:
        M[k] = dot(a(k), w(k))
    return (M[0] + M[3] - M[4] + M[6], M[2] + M[4], M[1] + M[3], M[0] - M[1] + M[2] + M[5])


def _cat(a, b):
    return jnp.concatenate([a, b], axis=1)


def _kernel(x_hbm, w1a_h, w1b_h, wq_h, wk_h, wv_h, wo_h, wp1_h, dw_h, wp2_h, w2a_h, w2b_h, out_hbm,
            xr, hops, kops, vops, wa, wb, wp1, wp2, dwb, sbuf, mbuf, zref, *, B, T, D, K, F):
    N = B * T
    TM = 2 * H
    NTB = T // TM
    NT = B * NTB
    TH = T // 2
    TP = kops.shape[2]
    NC = TP // W
    Dh = D // 2
    cat = _cat
    ident = tuple(range(7))

    zref[...] = jnp.zeros_like(zref)

    def tie(prev, v):
        if prev is None:
            return v
        never = jnp.tile(zref[...], (v.shape[0] // 8, 1)) != 0
        return jnp.where(never, prev, v)

    def tie0(prev, v):
        return v if prev is None else cat(tie(prev, v[:, :128]), v[:, 128:])

    def rows(i, off=0, n=H):
        return pl.ds(pl.multiple_of(i * TM + off, 16), n)

    def ln_chain(load, store=None, prev=None, chained=True):
        if not chained:
            ht, hb = _ln(load(0, H)), _ln(load(H, H))
            ops = _a_ops(ht[:, :Dh], ht[:, Dh:], hb[:, :Dh], hb[:, Dh:])
            if store is not None:
                for k in range(7):
                    store(k, 0, H, ops[k])
            return ops, None
        outs = [[] for _ in range(7)]
        for r in range(0, H, 16):
            ht, hb = _ln(tie0(prev, load(r, 16))), _ln(load(H + r, 16))
            s = _a_sums(ht[:, :Dh], ht[:, Dh:], hb[:, :Dh], hb[:, Dh:])
            prev = s[0][:, :128]
            for k in range(7):
                o = s[k].astype(bf16)
                outs[k].append(o)
                if store is not None:
                    store(k, r, 16, o)
        return [jnp.concatenate(o, axis=0) for o in outs], prev

    def chained(fn, x, pr):
        if pr == 0:
            return fn(x)
        prev = None
        cols = []
        for t in range(x.shape[1] // 128):
            parts = []
            for r in range(0, x.shape[0], pr):
                prev = fn(tie(prev, x[r:r + pr, t * 128:(t + 1) * 128]))
                parts.append(prev)
            cols.append(jnp.concatenate(parts, axis=0))
        return jnp.concatenate(cols, axis=1)

    def build_b_ops(raw, dst, r0, nr, c0, n, scale):
        k = raw.shape[0] // 2
        nh = n // 2
        prev = None
        for r in range(0, nr, 16):
            for c in range(0, nh, 128):
                def blk(ro, co):
                    return raw[pl.ds(ro + r0 + r, 16), c0 + co + c:c0 + co + c + 128].astype(f32) * scale
                B11, B12, B21, B22 = tie(prev, blk(0, 0)), blk(0, nh), blk(k, 0), blk(k, nh)
                prev = (B11 + B12) + (B21 + B22)
                ops = _b_ops(B11, B12, B21, B22)
                for i in range(7):
                    dst[i, pl.ds(r0 + r, 16), c:c + 128] = ops[i]

    def ff_up(hnops, slot):
        C = _smm(lambda k: hnops[slot, k], lambda k: wa[k], UPO)
        return [chained(_hsilu, C[q], PR[q]) for q in range(4)]

    def ff_down(U):
        a = _a_ops(*U)
        D11, D12, D21, D22 = _smm(lambda k: a[k], lambda k: wb[k], DNO)
        return cat(D11, D12), cat(D21, D22)

    def stage_C1(i, prev=None):
        def st(k, r, n, v):
            hops[i, k, r:r + n, :] = v
        return ln_chain(lambda r, n: xr[rows(i, r, n), :], st, prev)

    def stage_C2(wkv, i, a):
        b = i // NTB
        r = pl.ds(pl.multiple_of((i % NTB) * H, 16), H)
        c = D ** -0.5 * LOG2E
        ktl, kth, kbl, kbh = [t * c for t in _smm(lambda k: a[k], lambda k: wkv[0, k])]
        ops = _b_ops(ktl, kbl, kth, kbh)
        for k in range(7):
            kops[b, k, r, :] = ops[k]
        vtl, vth, vbl, vbh = _smm(lambda k: a[k], lambda k: wkv[1, k])
        ops = _b_ops(vtl, vth, vbl, vbh)
        for k in range(7):
            vops[b, k, r, :] = ops[k]

    def att_qk(i):
        b = i // NTB
        for c in range(NC):
            s = list(_smm(lambda k: hops[i, k], lambda k: kops[b, k, c * W:(c + 1) * W, :], ident, _dot_nt))
            nv = TH - c * W
            for j in range(4):
                t = s[j]
                if nv < W:
                    lo = nv // 128 * 128
                    col = lax.broadcasted_iota(jnp.int32, (H, W - lo), 1)
                    t = cat(t[:, :lo], jnp.where(col < nv - lo, t[:, lo:], NEG))
                sbuf[c, j] = t

    def att_stats():
        prev = [None] * PCH
        n = 0
        for r in range(0, H, P2G):
            for half in range(2):
                blocks = [sbuf[c, 2 * half + j, r:r + P2G, :] for c in range(NC) for j in (0, 1)]
                blocks[0] = tie0(prev[n % PCH], blocks[0])
                m = jnp.max(functools.reduce(jnp.maximum, blocks), axis=-1, keepdims=True)
                l = jnp.sum(functools.reduce(jnp.add, [jnp.exp2(t - m) for t in blocks]), axis=-1, keepdims=True)
                mp = jnp.broadcast_to(m + jnp.log2(l), (P2G, 128))
                mbuf[half, r:r + P2G, :] = mp
                prev[n % PCH] = mp
                n += 1

    def att_pv(i, side, unroll=False):
        b = i // NTB

        def trip(c, carry):
            mt = jnp.concatenate([mbuf[0]] * (W // 128), axis=1)
            mb = jnp.concatenate([mbuf[1]] * (W // 128), axis=1)
            ms = (mt, mt, mb, mb)
            a = _a_ops(*[jnp.exp2(sbuf[c, j] - ms[j]) for j in range(4)])
            kr = pl.ds(pl.multiple_of(c * W, W), W)
            O11, O12, O21, O22 = _smm(lambda k: a[k], lambda k: vops[b, k, kr, :])
            xr[rows(i), :] = xr[rows(i), :] + cat(O11, O12)
            xr[rows(i, H), :] = xr[rows(i, H), :] + cat(O21, O22)
            side(c)
            return carry

        if unroll:
            for c in range(NC):
                trip(c, 0)
        else:
            lax.fori_loop(0, NC, trip, 0)

    def front(hnops, wkv, xbuf, rawa, rawb, rawq, rawp1, rawp2, rawdw, xsem, wsem):
        def xcopy(t, slot):
            return pltpu.make_async_copy(x_hbm.at[pl.ds(pl.multiple_of(t * TM, 16), TM), :], xbuf.at[slot], xsem.at[slot])

        cp = [
            pltpu.make_async_copy(wq_h, rawq.at[0], wsem.at[0]),
            pltpu.make_async_copy(wk_h, rawq.at[1], wsem.at[1]),
            pltpu.make_async_copy(wv_h, rawq.at[2], wsem.at[2]),
            pltpu.make_async_copy(wo_h, rawq.at[3], wsem.at[3]),
            pltpu.make_async_copy(w1a_h, rawa, wsem.at[4]),
            pltpu.make_async_copy(w1b_h, rawb, wsem.at[5]),
            pltpu.make_async_copy(dw_h, rawdw, wsem.at[6]),
            pltpu.make_async_copy(wp1_h, rawp1, wsem.at[7]),
            pltpu.make_async_copy(wp2_h, rawp2, wsem.at[8]),
            pltpu.make_async_copy(w2a_h, rawa, wsem.at[9]),
            pltpu.make_async_copy(w2b_h, rawb, wsem.at[10]),
        ]
        CQ, CK, CV, CO, C1A, C1B, CDW, CP1, CP2, C2A, C2B = range(11)

        def stage_A(t, slot, chained=True):
            xs = t % 3

            def st(k, r, n, v):
                hnops[slot, k, r:r + n, :] = v
            return ln_chain(lambda r, n: xbuf[xs, r:r + n, :].astype(f32), st, chained=chained)[1]

        def stage_B2(i, U):
            dt, db = ff_down(U)
            xs = i % 3
            xr[rows(i), :] = xbuf[xs, 0:H, :].astype(f32) + dt
            xr[rows(i, H), :] = xbuf[xs, H:TM, :].astype(f32) + db

        cp[CQ].start()
        cp[CK].start()
        xcopy(0, 0).start()
        cp[C1A].start()
        cp[CV].start()
        cp[CO].start()
        cp[C1B].start()
        xcopy(1, 1).start()
        cp[CDW].start()
        xcopy(2, 2).start()
        cp[CP1].start()
        cp[CP2].start()

        for b in range(B):
            for k in range(7):
                kops[b, k, TH:, :] = jnp.zeros((TP - TH, Dh), bf16)
                vops[b, k, TH:, :] = jnp.zeros((TP - TH, Dh), bf16)

        cp[CQ].wait()
        cp[CK].wait()
        wf = _dot_nt(rawq[1], rawq[0])
        ops = _b_ops(wf[:Dh, :Dh], wf[:Dh, Dh:], wf[Dh:, :Dh], wf[Dh:, Dh:])
        for k in range(7):
            wkv[0, k] = ops[k]
        cp[CV].wait()
        cp[CO].wait()
        wf = _dot(rawq[2], rawq[3])
        ops = _b_ops(wf[:Dh, :Dh], wf[:Dh, Dh:], wf[Dh:, :Dh], wf[Dh:, Dh:])
        for k in range(7):
            wkv[1, k] = ops[k]
        xcopy(0, 0).wait()
        stage_A(0, 0, chained=False)
        cp[C1A].wait()
        build_b_ops(rawa, wa, 0, Dh, 0, F, 0.5)
        cp[C1B].wait()
        build_b_ops(rawb, wb, 0, F // 2, 0, D, 0.5)
        cp[C2A].start()
        cp[C2B].start()
        cp[CDW].wait()
        dwv = rawdw[...].astype(f32)
        for k in range(K):
            for cb in range(4):
                dwb[k, cb] = jnp.broadcast_to(dwv[k:k + 1, cb * 128:(cb + 1) * 128], (8, 128))

        xcopy(1, 1).wait()
        U = ff_up(hnops, 0)
        stage_A(1, 1)
        stage_B2(0, U)

        def p1(i, carry):
            @pl.when(i + 2 < NT)
            def _():
                xcopy(i + 2, (i + 2) % 3).start()

            @pl.when(i + 1 < NT)
            def _():
                xcopy(i + 1, (i + 1) % 3).wait()
            U = ff_up(hnops, i % 2)
            prev = stage_A(jnp.minimum(i + 1, NT - 1), (i + 1) % 2)
            hq, _ = stage_C1(i - 1, prev)
            stage_B2(i, U)
            stage_C2(wkv, i - 1, hq)
            return carry

        with jax.named_scope("p1loop"):
            lax.fori_loop(1, NT, p1, 0)

        cp[CP1].wait()
        cp[CP2].wait()
        cp[C2A].wait()
        cp[C2B].wait()

        def wops(c):
            q = Dh // NC
            r0 = c * q if isinstance(c, int) else pl.multiple_of(c * q, 16)
            r1 = c * (F // 2 // NC) if isinstance(c, int) else pl.multiple_of(c * (F // 2 // NC), 16)
            build_b_ops(rawp1, wp1.at[0], r0, q, 0, D, 0.5)
            build_b_ops(rawp1, wp1.at[1], r0, q, D, D, 0.5)
            build_b_ops(rawp2, wp2, r0, q, 0, D, 1.0)
            build_b_ops(rawa, wa, r0, q, 0, F, 0.5)
            build_b_ops(rawb, wb, r1, F // 2 // NC, 0, D, 0.5)

        with jax.named_scope("p2peel"):
            hq, _ = stage_C1(NT - 1)
            att_qk(0)
            stage_C2(wkv, NT - 1, hq)
            att_stats()
            att_pv(0, wops, unroll=PEEL_UNROLL)

    V = pltpu.VMEM
    with jax.named_scope("front"):
        pl.run_scoped(front, V((2, 7, H, Dh), bf16), V((2, 7, Dh, Dh), bf16), V((3, TM, D), bf16), V((D, F), bf16), V((F, D), bf16), V((4, D, D), bf16),
                      V((D, 2 * D), bf16), V((D, D), bf16), V((K, D), bf16),
                      pltpu.SemaphoreType.DMA((3,)), pltpu.SemaphoreType.DMA((11,)))

    def back(dc, stats):
        def attention(gbuf):
            def stage_D1(j, chained=True):
                return ln_chain(lambda r, n: xr[rows(j, r, n), :], chained=chained)[0]

            def stage_D2(j, a):
                ga = _smm(lambda k: a[k], lambda k: wp1[0, k])
                gb_ = _smm(lambda k: a[k], lambda k: wp1[1, k])
                g = [_hglu(u, v) for u, v in zip(ga, gb_)]
                slot = j % 4
                jb = j % NTB
                first = jb == 0
                last = jb == NTB - 1
                for cb in range(4):
                    top = g[cb // 2][:, (cb % 2) * 128:(cb % 2 + 1) * 128]
                    bot = g[2 + cb // 2][:, (cb % 2) * 128:(cb % 2 + 1) * 128]
                    gbuf[slot, cb, 8:8 + H, :] = top
                    gbuf[slot, cb, 8 + H:8 + TM, :] = bot
                    gbuf[(j + 3) % 4, cb, 8 + TM:16 + TM, :] = jnp.where(first, 0.0, top[0:8])
                    gbuf[(j + 1) % 4, cb, 0:8, :] = jnp.where(last, 0.0, bot[H - 8:H])

            def stage_E(j, cb, nch):
                slot = j % 4
                w = [dwb[k, cb] for k in range(K)]
                rc = 8 if nch else 80
                wt = [jnp.tile(t, (rc // 8, 1)) for t in w]
                prev = [None] * max(nch, 1)
                tot = None
                for n, r0 in enumerate(range(0, TM, rc)):
                    acc = None
                    for k in range(K):
                        t = gbuf[slot, cb, pl.ds(r0 + k + 8 - K // 2, rc), :] * wt[k]
                        if acc is None:
                            acc = tie(prev[n % nch], t) if nch else t
                        else:
                            acc = acc + t
                    dc[cb, pl.ds(pl.multiple_of(j * TM + r0, 8), rc), :] = acc
                    tot = acc if tot is None else tot + acc
                    if nch:
                        prev[n % nch] = acc
                mean = jnp.sum(tot, axis=0, keepdims=True) * (1.0 / TM)
                d = dc[cb, pl.ds(pl.multiple_of(j * TM, 8), TM), :] - mean
                m2 = jnp.sum(d * d, axis=0, keepdims=True)
                js = pl.ds(pl.multiple_of(j * 8, 8), 8)
                stats[0, cb, js, :] = jnp.broadcast_to(mean, (8, 128))
                stats[1, cb, js, :] = jnp.broadcast_to(m2, (8, 128))

            for cb in range(4):
                gbuf[0, cb, 0:8, :] = jnp.zeros((8, 128), f32)

            def p2(i, carry):
                je = jnp.maximum(i - ELAG, 0)
                a = stage_D1(i - 1)
                att_qk(i)
                stage_D2(i - 1, a)
                att_stats()
                att_pv(i, lambda c: stage_E(je, c, ECH))
                return carry

            with jax.named_scope("p2loop"):
                lax.fori_loop(1, NT, p2, 0)

            a = stage_D1(NT - 1, chained=False)
            for cb in range(4):
                stage_E(NT - 3, cb, 1)
            stage_D2(NT - 1, a)
            for cb in range(4):
                gbuf[(NT - 1) % 4, cb, 8 + TM:16 + TM, :] = jnp.zeros((8, 128), f32)
            for j in range(NT - 2, NT):
                for cb in range(4):
                    stage_E(j, cb, 0)

        pl.run_scoped(attention, V((4, 4, TM + 16, 128), f32))

        st0 = jnp.concatenate([stats[0, cb] for cb in range(4)], axis=1)
        st1 = jnp.concatenate([stats[1, cb] for cb in range(4)], axis=1)
        mu = jnp.sum(st0, axis=0, keepdims=True) * (1.0 / (8 * NT))
        dm = st0 - mu
        var = jnp.sum(st1 + TM * dm * dm, axis=0, keepdims=True) * (1.0 / (8 * N))
        rsd = 0.5 * lax.rsqrt(var + EPS)

        def final(hnops, obuf, osem):
            def ocopy(t, slot):
                return pltpu.make_async_copy(obuf.at[slot], out_hbm.at[pl.ds(pl.multiple_of(t * TM, 16), TM), :], osem.at[slot])

            def stage_F1(j, chained=True):
                def zq(r0, n, hi):
                    d = jnp.concatenate([dc[2 * hi + t, rows(j, r0, n), :] for t in range(2)], axis=1)
                    return (d - mu[:, hi * Dh:(hi + 1) * Dh]) * rsd[:, hi * Dh:(hi + 1) * Dh]
                if not chained:
                    return _a_ops(*[_hsilu(zq(r0, H, hi)) for r0 in (0, H) for hi in (0, 1)])
                outs = [[] for _ in range(7)]
                prev = None
                for r in range(0, H, 16):
                    z = []
                    for r0 in (0, H):
                        for hi in (0, 1):
                            t = _hsilu(tie0(prev, zq(r0 + r, 16, hi)))
                            prev = t[:, :128] + t[:, 128:]
                            z.append(t)
                    for k, s in enumerate(_a_ops(*z)):
                        outs[k].append(s)
                return [jnp.concatenate(o, axis=0) for o in outs]

            def stage_F2(j, slot, zops, prev=None, chained=True):
                E11, E12, E21, E22 = _smm(lambda k: zops[k], lambda k: wp2[k])
                x3t = xr[rows(j), :] + cat(E11, E12)
                x3b = xr[rows(j, H), :] + cat(E21, E22)
                xr[rows(j), :] = x3t
                xr[rows(j, H), :] = x3b
                x3 = (x3t, x3b)

                def st(k, r, n, v):
                    hnops[slot, k, r:r + n, :] = v
                ln_chain(lambda r, n: x3[r // H][r % H:r % H + n], st, prev, chained=chained)

            def stage_G2(i, U):
                dt, db = ff_down(U)
                xr[rows(i), :] = xr[rows(i), :] + dt
                xr[rows(i, H), :] = xr[rows(i, H), :] + db

            def stage_Hh(j, chained=True):
                slot = j % 2
                if not chained:
                    obuf[slot, 0:H, :] = _ln(xr[rows(j), :]).astype(bf16)
                    obuf[slot, H:TM, :] = _ln(xr[rows(j, H), :]).astype(bf16)
                    return None
                prev = None
                for r in range(0, TM, 32):
                    y = _ln(tie0(prev, xr[rows(j, r, 32), :]))
                    prev = y[:, :128]
                    obuf[slot, r:r + 32, :] = y.astype(bf16)
                return prev

            stage_F2(0, 0, stage_F1(0, chained=False), chained=False)

            def p4(i, carry):
                @pl.when(i >= 3)
                def _():
                    ocopy(i - 3, (i - 3) % 2).wait()
                U = ff_up(hnops, i % 2)
                zops = stage_F1(i + 1)
                prev = stage_Hh(jnp.maximum(i - 1, 0))
                stage_F2(i + 1, (i + 1) % 2, zops, None if prev is None else prev[0:16])
                stage_G2(i, U)

                @pl.when(i >= 1)
                def _():
                    ocopy(i - 1, (i - 1) % 2).start()
                return carry

            with jax.named_scope("p4loop"):
                lax.fori_loop(0, NT - 1, p4, 0)

            ocopy(NT - 4, (NT - 4) % 2).wait()
            U = ff_up(hnops, (NT - 1) % 2)
            stage_Hh(NT - 2)
            stage_G2(NT - 1, U)
            ocopy(NT - 3, (NT - 3) % 2).wait()
            ocopy(NT - 2, (NT - 2) % 2).start()
            stage_Hh(NT - 1, chained=False)
            ocopy(NT - 1, (NT - 1) % 2).start()
            ocopy(NT - 2, (NT - 2) % 2).wait()
            ocopy(NT - 1, (NT - 1) % 2).wait()

        pl.run_scoped(final, V((2, 7, H, Dh), bf16), V((2, TM, D), bf16), pltpu.SemaphoreType.DMA((2,)))

    with jax.named_scope("back"):
        pl.run_scoped(back, V((4, N, 128), f32), V((2, 4, 8 * NT, 128), f32))


@jax.jit
def pallas_standalone__conformer_family_conformer__speech_kernel(
    x, w_ff1_a, w_ff1_b, w_q, w_k, w_v, w_o, w_pw1, dw, w_pw2, w_ff2_a, w_ff2_b):
    B, T, D = x.shape
    K = dw.shape[0]
    F = w_ff1_a.shape[1]
    N = B * T
    TM = 2 * H
    NT = N // TM
    TP = (T // 2 + 127) // 128 * 128
    Dh = D // 2
    kern = functools.partial(_kernel, B=B, T=T, D=D, K=K, F=F)
    hbm = pl.BlockSpec(memory_space=pl.ANY)
    V = pltpu.VMEM
    out = pl.pallas_call(
        kern,
        out_shape=jax.ShapeDtypeStruct((N, D), x.dtype),
        in_specs=[hbm] * 12,
        out_specs=hbm,
        scratch_shapes=[
            V((N, D), f32),
            V((NT, 7, H, Dh), bf16),
            V((B, 7, TP, Dh), bf16),
            V((B, 7, TP, Dh), bf16),
            V((7, Dh, F // 2), bf16),
            V((7, F // 2, Dh), bf16),
            V((2, 7, Dh, Dh), bf16),
            V((7, Dh, Dh), bf16),
            V((K, 4, 8, 128), f32),
            V((TP // W, 4, H, W), f32),
            V((2, H, 128), f32),
            V((8, 128), jnp.int32),
        ],
        compiler_params=pltpu.CompilerParams(vmem_limit_bytes=VMEM_LIMIT),
    )(x.reshape(N, D), w_ff1_a, w_ff1_b, w_q, w_k, w_v, w_o, w_pw1, dw, w_pw2, w_ff2_a, w_ff2_b)
    return out.reshape(B, T, D)
```

```python
import functools
import jax
import jax.numpy as jnp
from jax import lax
import jax.experimental.pallas as pl
import jax.experimental.pallas.tpu as pltpu

H = 400
W = 512
EPS = 1e-5
LOG2E = 1.4426950408889634
NEG = -1e30
ELAG = 2
UPO = (1, 2, 0, 5, 3, 4, 6)
DNO = (1, 3, 6, 0, 2, 4, 5)
DQORD = (2, 0, 1, 3)
PR = (40, 40, 40, 40)
P2G = 8
EPI_CH = 1
EPI_LAST = 2
HG = 32
LINK = 1
PCHF = 8
PCH = 4
ECH = 1
PEEL_UNROLL = True
ONLY = None
VMEM_LIMIT = 127 * 1024 * 1024

bf16 = jnp.bfloat16
f32 = jnp.float32


def _ln(x):
    m = jnp.mean(x, axis=-1, keepdims=True)
    c = x - m
    v = jnp.mean(c * c, axis=-1, keepdims=True)
    return c * lax.rsqrt(v + EPS)


def _hsilu(h):
    return h * jnp.tanh(h) + h


def _hglu(a, b):
    return a * jnp.tanh(b) + a


def _dot(a, b):
    return jnp.dot(a, b, preferred_element_type=f32)


def _dot_nt(a, b):
    return lax.dot_general(a, b, (((1,), (1,)), ((), ())), preferred_element_type=f32)


def _a_sums(A11, A12, A21, A22):
    return [A11 + A22, A21 + A22, A11, A22, A11 + A12, A21 - A11, A12 - A22]


def _a_ops(*q):
    return [t.astype(bf16) for t in _a_sums(*q)]


def _b_ops(B11, B12, B21, B22):
    return [t.astype(bf16) for t in
            (B11 + B22, B11, B12 - B22, B21 - B11, B22, B11 + B12, B21 + B22)]


def _smm(a, w, order=UPO, dot=_dot):
    M = [None] * 7
    for k in order:
        M[k] = dot(a(k), w(k))
    return (M[0] + M[3] - M[4] + M[6], M[2] + M[4], M[1] + M[3], M[0] - M[1] + M[2] + M[5])


def _cat(a, b):
    return jnp.concatenate([a, b], axis=1)


def _kernel(x_hbm, w1a_h, w1b_h, wq_h, wk_h, wv_h, wo_h, wp1_h, dw_h, wp2_h, w2a_h, w2b_h, out_hbm,
            xr, hops, kops, vops, wa, wb, wp1, wp2, dwb, sbuf, mbuf, cstat, zref, *, B, T, D, K, F):
    N = B * T
    TM = 2 * H
    NTB = T // TM
    NT = B * NTB
    TH = T // 2
    TP = kops.shape[2]
    NC = TP // W
    Dh = D // 2
    cat = _cat
    ident = tuple(range(7))

    zref[...] = jnp.zeros_like(zref)

    def tie(prev, v):
        if prev is None:
            return v
        never = jnp.tile(zref[...], (v.shape[0] // 8, 1)) != 0
        return jnp.where(never, prev, v)

    def tie0(prev, v):
        return v if prev is None else cat(tie(prev, v[:, :128]), v[:, 128:])

    def rows(i, off=0, n=H):
        return pl.ds(pl.multiple_of(i * TM + off, 16), n)

    def ln_chain(load, store=None, prev=None, chained=True):
        if not chained:
            ht, hb = _ln(load(0, H)), _ln(load(H, H))
            ops = _a_ops(ht[:, :Dh], ht[:, Dh:], hb[:, :Dh], hb[:, Dh:])
            if store is not None:
                for k in range(7):
                    store(k, 0, H, ops[k])
            return ops, None
        outs = [[] for _ in range(7)]
        for r in range(0, H, 16):
            ht, hb = _ln(tie0(prev, load(r, 16))), _ln(load(H + r, 16))
            s = _a_sums(ht[:, :Dh], ht[:, Dh:], hb[:, :Dh], hb[:, Dh:])
            prev = s[0][:, :128]
            for k in range(7):
                o = s[k].astype(bf16)
                outs[k].append(o)
                if store is not None:
                    store(k, r, 16, o)
        return [jnp.concatenate(o, axis=0) for o in outs], prev

    def chained(fn, x, pr):
        if pr == 0:
            return fn(x)
        prev = None
        cols = []
        for t in range(x.shape[1] // 128):
            parts = []
            for r in range(0, x.shape[0], pr):
                prev = fn(tie(prev, x[r:r + pr, t * 128:(t + 1) * 128]))
                parts.append(prev)
            cols.append(jnp.concatenate(parts, axis=0))
        return jnp.concatenate(cols, axis=1)

    def build_b_ops(raw, dst, r0, nr, c0, n, scale, chained=True):
        k = raw.shape[0] // 2
        nh = n // 2
        prev = None
        for r in range(0, nr, 16):
            for c in range(0, nh, 128):
                def blk(ro, co):
                    return raw[pl.ds(ro + r0 + r, 16), c0 + co + c:c0 + co + c + 128].astype(f32) * scale
                B11, B12, B21, B22 = tie(prev if chained else None, blk(0, 0)), blk(0, nh), blk(k, 0), blk(k, nh)
                prev = (B11 + B12) + (B21 + B22)
                ops = _b_ops(B11, B12, B21, B22)
                for i in range(7):
                    dst[i, pl.ds(r0 + r, 16), c:c + 128] = ops[i]

    QORD = (3, 2, 1, 0)

    def qidx(i, q):
        return rows(i, (q // 2) * H), slice((q % 2) * Dh, (q % 2 + 1) * Dh)

    def ff_up(hnops, slot):
        C = _smm(lambda k: hnops[slot, k], lambda k: wa[k], UPO)
        return [chained(_hsilu, C[q], PR[q]) for q in range(4)]

    def ff_down(U):
        a = _a_ops(*U)
        return _smm(lambda k: a[k], lambda k: wb[k], DNO)

    def stage_C1(i, prev=None):
        def st(k, r, n, v):
            hops[i, k, r:r + n, :] = v
        return ln_chain(lambda r, n: xr[rows(i, r, n), :], st, prev)

    def stage_C2(wkv, i, a):
        b = i // NTB
        r = pl.ds(pl.multiple_of((i % NTB) * H, 16), H)
        c = D ** -0.5 * LOG2E
        ktl, kth, kbl, kbh = [t * c for t in _smm(lambda k: a[k], lambda k: wkv[0, k])]
        ops = _b_ops(ktl, kbl, kth, kbh)
        for k in range(7):
            kops[b, k, r, :] = ops[k]
        vtl, vth, vbl, vbh = _smm(lambda k: a[k], lambda k: wkv[1, k])
        ops = _b_ops(vtl, vth, vbl, vbh)
        for k in range(7):
            vops[b, k, r, :] = ops[k]

    def att_qk(i):
        b = i // NTB
        for c in range(NC):
            s = list(_smm(lambda k: hops[i, k], lambda k: kops[b, k, c * W:(c + 1) * W, :], ident, _dot_nt))
            nv = TH - c * W
            for j in range(4):
                t = s[j]
                if nv < W:
                    lo = nv // 128 * 128
                    col = lax.broadcasted_iota(jnp.int32, (H, W - lo), 1)
                    t = cat(t[:, :lo], jnp.where(col < nv - lo, t[:, lo:], NEG))
                sbuf[c, j] = t

    def att_stats():
        prev = [None] * PCH
        n = 0
        for c in range(NC):
            if c == NC - 1:
                prev = [prev[t % PCH] for t in range(PCHF)]
            nch = len(prev)
            for r in range(0, H, P2G):
                for half in range(2):
                    rs = slice(r, r + P2G)
                    blocks = [sbuf[c, 2 * half + j, rs, t * 128:(t + 1) * 128]
                              for j in (0, 1) for t in range(W // 128)]
                    blocks[0] = tie(prev[n % nch], blocks[0])
                    m = jnp.broadcast_to(
                        jnp.max(functools.reduce(jnp.maximum, blocks), axis=-1, keepdims=True), (P2G, 128))
                    if c < NC - 1:
                        l = functools.reduce(jnp.add, [jnp.exp2(t - m) for t in blocks])
                        cstat[0, c, half, rs, :] = m
                        cstat[1, c, half, rs, :] = l
                        prev[n % nch] = l
                    else:
                        ms = [cstat[0, cc, half, rs, :] for cc in range(NC - 1)]
                        m = functools.reduce(jnp.maximum, ms + [m])
                        l = functools.reduce(jnp.add, [jnp.exp2(t - m) for t in blocks]
                                             + [cstat[1, cc, half, rs, :] * jnp.exp2(ms[cc] - m) for cc in range(NC - 1)])
                        mp = m + jnp.log2(jnp.sum(l, axis=-1, keepdims=True))
                        mbuf[half, rs, :] = mp
                        prev[n % nch] = mp
                    n += 1

    def att_pv(i, side, unroll=False):
        b = i // NTB

        def trip(c, carry):
            mt = jnp.concatenate([mbuf[0]] * (W // 128), axis=1)
            mb = jnp.concatenate([mbuf[1]] * (W // 128), axis=1)
            ms = (mt, mt, mb, mb)
            a = _a_ops(*[jnp.exp2(sbuf[c, j] - ms[j]) for j in range(4)])
            kr = pl.ds(pl.multiple_of(c * W, W), W)
            O = _smm(lambda k: a[k], lambda k: vops[b, k, kr, :])
            for q in QORD:
                xr[qidx(i, q)] = xr[qidx(i, q)] + O[q]
            side(c)
            return carry

        if unroll:
            for c in range(NC):
                trip(c, 0)
        else:
            lax.fori_loop(0, NC, trip, 0)

    def front(hnops, wkv, xbuf, rawa, rawb, rawq, rawp1, rawp2, rawdw, xsem, wsem):
        def xcopy(t, slot):
            return pltpu.make_async_copy(x_hbm.at[pl.ds(pl.multiple_of(t * TM, 16), TM), :], xbuf.at[slot], xsem.at[slot])

        cp = [
            pltpu.make_async_copy(wq_h, rawq.at[0], wsem.at[0]),
            pltpu.make_async_copy(wk_h, rawq.at[1], wsem.at[1]),
            pltpu.make_async_copy(wv_h, rawq.at[2], wsem.at[2]),
            pltpu.make_async_copy(wo_h, rawq.at[3], wsem.at[3]),
            pltpu.make_async_copy(w1a_h, rawa, wsem.at[4]),
            pltpu.make_async_copy(w1b_h, rawb, wsem.at[5]),
            pltpu.make_async_copy(dw_h, rawdw, wsem.at[6]),
            pltpu.make_async_copy(wp1_h, rawp1, wsem.at[7]),
            pltpu.make_async_copy(wp2_h, rawp2, wsem.at[8]),
            pltpu.make_async_copy(w2a_h, rawa, wsem.at[9]),
            pltpu.make_async_copy(w2b_h, rawb, wsem.at[10]),
        ]
        CQ, CK, CV, CO, C1A, C1B, CDW, CP1, CP2, C2A, C2B = range(11)

        def stage_A(t, slot, chained=True):
            xs = t % 3

            def st(k, r, n, v):
                hnops[slot, k, r:r + n, :] = v
            return ln_chain(lambda r, n: xbuf[xs, r:r + n, :].astype(f32), st, chained=chained)[1]

        def stage_B2(i, U):
            d = ff_down(U)
            xs = i % 3
            for q in DQORD:
                r0, c0 = (q // 2) * H, (q % 2) * Dh
                xr[qidx(i, q)] = xbuf[xs, r0:r0 + H, c0:c0 + Dh].astype(f32) + d[q]

        def p1(i, carry, dma=True):
            if dma:
                @pl.when(i + 2 < NT)
                def _():
                    xcopy(i + 2, (i + 2) % 3).start()

                @pl.when(i + 1 < NT)
                def _():
                    xcopy(i + 1, (i + 1) % 3).wait()
            U = ff_up(hnops, i % 2)
            prev = stage_A(jnp.minimum(i + 1, NT - 1), (i + 1) % 2)
            hq, _ = stage_C1(i - 1, prev)
            stage_B2(i, U)
            stage_C2(wkv, i - 1, hq)
            return carry

        if ONLY == 'p1':
            lax.fori_loop(1, NT, lambda i, c: p1(i, c, False), 0)
            return
        if ONLY is not None:
            return
        cp[CQ].start()
        cp[CK].start()
        cp[C1A].start()
        xcopy(0, 0).start()
        cp[CV].start()
        cp[CO].start()
        cp[C1B].start()
        xcopy(1, 1).start()
        cp[CDW].start()
        xcopy(2, 2).start()
        cp[CP1].start()
        cp[CP2].start()

        for b in range(B):
            for k in range(7):
                kops[b, k, TH:, :] = jnp.zeros((TP - TH, Dh), bf16)
                vops[b, k, TH:, :] = jnp.zeros((TP - TH, Dh), bf16)

        cp[CQ].wait()
        cp[CK].wait()
        wf = _dot_nt(rawq[1], rawq[0])
        ops = _b_ops(wf[:Dh, :Dh], wf[:Dh, Dh:], wf[Dh:, :Dh], wf[Dh:, Dh:])
        for k in range(7):
            wkv[0, k] = ops[k]
        cp[C1A].wait()
        build_b_ops(rawa, wa, 0, Dh, 0, F, 0.5, chained=False)
        xcopy(0, 0).wait()
        stage_A(0, 0, chained=False)
        cp[CV].wait()
        cp[CO].wait()
        cp[C1B].wait()
        cp[CDW].wait()
        xcopy(1, 1).wait()
        with jax.named_scope("peel1"):
            wf = _dot(rawq[2], rawq[3])
            ops = _b_ops(wf[:Dh, :Dh], wf[:Dh, Dh:], wf[Dh:, :Dh], wf[Dh:, Dh:])
            for k in range(7):
                wkv[1, k] = ops[k]
            dwv = rawdw[...].astype(f32)
            for k in range(K):
                for cb in range(4):
                    dwb[k, cb] = jnp.broadcast_to(dwv[k:k + 1, cb * 128:(cb + 1) * 128], (8, 128))
            U = ff_up(hnops, 0)
            build_b_ops(rawb, wb, 0, F // 2, 0, D, 0.5)
            stage_A(1, 1)
            stage_B2(0, U)
        cp[C2A].start()
        cp[C2B].start()

        with jax.named_scope("p1loop"):
            lax.fori_loop(1, NT, p1, 0)

        cp[CP1].wait()
        cp[CP2].wait()
        cp[C2A].wait()
        cp[C2B].wait()

        def wops(c):
            q = Dh // NC
            r0 = c * q if isinstance(c, int) else pl.multiple_of(c * q, 16)
            r1 = c * (F // 2 // NC) if isinstance(c, int) else pl.multiple_of(c * (F // 2 // NC), 16)
            build_b_ops(rawp1, wp1.at[0], r0, q, 0, D, 0.5)
            build_b_ops(rawp1, wp1.at[1], r0, q, D, D, 0.5)
            build_b_ops(rawp2, wp2, r0, q, 0, D, 1.0)
            build_b_ops(rawa, wa, r0, q, 0, F, 0.5)
            build_b_ops(rawb, wb, r1, F // 2 // NC, 0, D, 0.5)

        with jax.named_scope("p2peel"):
            hq, _ = stage_C1(NT - 1)
            att_qk(0)
            stage_C2(wkv, NT - 1, hq)
            att_stats()
            att_pv(0, wops, unroll=PEEL_UNROLL)

    V = pltpu.VMEM
    with jax.named_scope("front"):
        pl.run_scoped(front, V((2, 7, H, Dh), bf16), V((2, 7, Dh, Dh), bf16), V((3, TM, D), bf16), V((D, F), bf16), V((F, D), bf16), V((4, D, D), bf16),
                      V((D, 2 * D), bf16), V((D, D), bf16), V((K, D), bf16),
                      pltpu.SemaphoreType.DMA((3,)), pltpu.SemaphoreType.DMA((11,)))

    def back(dc, stats):
        def attention(gbuf):
            def stage_D1(j, chained=True):
                return ln_chain(lambda r, n: xr[rows(j, r, n), :], chained=chained)[0]

            def stage_D2(j, a):
                ga = _smm(lambda k: a[k], lambda k: wp1[0, k])
                gb_ = _smm(lambda k: a[k], lambda k: wp1[1, k])
                g = [_hglu(u, v) for u, v in zip(ga, gb_)]
                slot = j % 4
                jb = j % NTB
                first = jb == 0
                last = jb == NTB - 1
                for q in QORD:
                    for t in range(2):
                        cb = 2 * (q % 2) + t
                        v = g[q][:, t * 128:(t + 1) * 128]
                        r0 = 8 + (q // 2) * H
                        gbuf[slot, cb, r0:r0 + H, :] = v
                        if q // 2 == 0:
                            gbuf[(j + 3) % 4, cb, 8 + TM:16 + TM, :] = jnp.where(first, 0.0, v[0:8])
                        else:
                            gbuf[(j + 1) % 4, cb, 0:8, :] = jnp.where(last, 0.0, v[H - 8:H])

            def stage_E(j, cb, nch):
                slot = j % 4
                w = [dwb[k, cb] for k in range(K)]
                prev = [None] * max(nch, 1)
                shift = s1 = s2 = None
                for n, r0 in enumerate(range(0, TM, 8)):
                    acc = None
                    for k in range(K):
                        t = gbuf[slot, cb, pl.ds(r0 + k + 8 - K // 2, 8), :] * w[k]
                        if acc is None:
                            acc = tie(prev[n % nch], t) if nch else t
                        else:
                            acc = acc + t
                    dc[cb, pl.ds(pl.multiple_of(j * TM + r0, 8), 8), :] = acc
                    if nch:
                        prev[n % nch] = acc
                    if shift is None:
                        shift = acc
                    else:
                        d = acc - shift
                        s1 = d if s1 is None else s1 + d
                        s2 = d * d if s2 is None else s2 + d * d
                ns = TM // 8
                js = pl.ds(pl.multiple_of(j * 8, 8), 8)
                stats[0, cb, js, :] = shift + s1 * (1.0 / ns)
                stats[1, cb, js, :] = s2 - s1 * s1 * (1.0 / ns)

            for cb in range(4):
                gbuf[0, cb, 0:8, :] = jnp.zeros((8, 128), f32)

            def p2(i, carry):
                je = jnp.maximum(i - ELAG, 0)
                a = stage_D1(i - 1)
                att_qk(i)
                stage_D2(i - 1, a)
                att_stats()
                att_pv(i, lambda c: stage_E(je, c, ECH))
                return carry

            if ONLY in ('p1', 'p4'):
                return
            with jax.named_scope("p2loop"):
                lax.fori_loop(1, NT, p2, 0)
            if ONLY is not None:
                return

            a = stage_D1(NT - 1, chained=False)
            stage_D2(NT - 1, a)
            for cb in range(4):
                gbuf[(NT - 1) % 4, cb, 8 + TM:16 + TM, :] = jnp.zeros((8, 128), f32)
            for j in range(NT - ELAG, NT):
                for cb in range(4):
                    stage_E(j, cb, EPI_CH if j < NT - 1 else EPI_LAST)

        pl.run_scoped(attention, V((4, 4, TM + 16, 128), f32))

        st0 = jnp.concatenate([stats[0, cb] for cb in range(4)], axis=1)
        st1 = jnp.concatenate([stats[1, cb] for cb in range(4)], axis=1)
        mu = jnp.sum(st0, axis=0, keepdims=True) * (1.0 / (8 * NT))
        dm = st0 - mu
        var = jnp.sum(st1 + (TM // 8) * dm * dm, axis=0, keepdims=True) * (1.0 / N)
        rsd = 0.5 * lax.rsqrt(var + EPS)

        def final(hnops, zops, obuf, osem):
            def ocopy(t, slot):
                return pltpu.make_async_copy(obuf.at[slot], out_hbm.at[pl.ds(pl.multiple_of(t * TM, 16), TM), :], osem.at[slot])

            def stage_F1(j, prev=None, chained=True):
                def zq(r0, n, hi):
                    d = jnp.concatenate([dc[2 * hi + t, rows(j, r0, n), :] for t in range(2)], axis=1)
                    return (d - mu[:, hi * Dh:(hi + 1) * Dh]) * rsd[:, hi * Dh:(hi + 1) * Dh]
                if not chained:
                    ops = _a_ops(*[_hsilu(zq(r0, H, hi)) for r0 in (0, H) for hi in (0, 1)])
                    for k in range(7):
                        zops[k] = ops[k]
                    return
                for r in range(0, H, 16):
                    z = []
                    for r0 in (0, H):
                        for hi in (0, 1):
                            t = _hsilu(tie0(prev, zq(r0 + r, 16, hi)))
                            prev = t[:, :128] + t[:, 128:]
                            z.append(t)
                    for k, o in enumerate(_a_ops(*z)):
                        zops[k, r:r + 16, :] = o

            def stage_F2(j):
                E = _smm(lambda k: zops[k], lambda k: wp2[k])
                for q in QORD:
                    xr[qidx(j, q)] = xr[qidx(j, q)] + E[q]

            def stage_F3(j, slot, prev=None, chained=True):
                def st(k, r, n, v):
                    hnops[slot, k, r:r + n, :] = v
                return ln_chain(lambda r, n: xr[rows(j, r, n), :], st, prev, chained=chained)[1]

            def stage_G2(i, U):
                d = ff_down(U)
                for q in DQORD:
                    xr[qidx(i, q)] = xr[qidx(i, q)] + d[q]

            def stage_Hh(j, chained=True):
                slot = j % 2
                if not chained:
                    obuf[slot, 0:H, :] = _ln(xr[rows(j), :]).astype(bf16)
                    obuf[slot, H:TM, :] = _ln(xr[rows(j, H), :]).astype(bf16)
                    return None
                prev = None
                for r in range(0, TM, HG):
                    y = _ln(tie0(prev, xr[rows(j, r, HG), :]))
                    prev = y[:, :128]
                    obuf[slot, r:r + HG, :] = y.astype(bf16)
                return prev

            if ONLY in ('p1', 'p2'):
                return
            if ONLY is None:
                stage_F1(0, chained=False)
                stage_F2(0)
                stage_F3(0, 0, chained=False)
                stage_F1(1, chained=False)

            def p4(i, carry):
                if ONLY is None:
                    @pl.when(i >= 3)
                    def _():
                        ocopy(i - 3, (i - 3) % 2).wait()
                stage_F2(i + 1)
                U = ff_up(hnops, i % 2)
                prev = stage_Hh(jnp.maximum(i - 1, 0))
                prev = stage_F3(i + 1, (i + 1) % 2, prev[0:16] if LINK & 1 else None)
                stage_F1(jnp.minimum(i + 2, NT - 1), prev if LINK & 2 else None)
                stage_G2(i, U)

                if ONLY is None:
                    @pl.when(i >= 1)
                    def _():
                        ocopy(i - 1, (i - 1) % 2).start()
                return carry

            with jax.named_scope("p4loop"):
                lax.fori_loop(0, NT - 1, p4, 0)
            if ONLY is not None:
                return

            ocopy(NT - 4, (NT - 4) % 2).wait()
            U = ff_up(hnops, (NT - 1) % 2)
            stage_Hh(NT - 2)
            stage_G2(NT - 1, U)
            ocopy(NT - 3, (NT - 3) % 2).wait()
            ocopy(NT - 2, (NT - 2) % 2).start()
            stage_Hh(NT - 1, chained=False)
            ocopy(NT - 1, (NT - 1) % 2).start()
            ocopy(NT - 2, (NT - 2) % 2).wait()
            ocopy(NT - 1, (NT - 1) % 2).wait()

        pl.run_scoped(final, V((2, 7, H, Dh), bf16), V((7, H, Dh), bf16), V((2, TM, D), bf16),
                      pltpu.SemaphoreType.DMA((2,)))

    with jax.named_scope("back"):
        pl.run_scoped(back, V((4, N, 128), f32), V((2, 4, 8 * NT, 128), f32))


@jax.jit
def pallas_standalone__conformer_family_conformer__speech_kernel(
    x, w_ff1_a, w_ff1_b, w_q, w_k, w_v, w_o, w_pw1, dw, w_pw2, w_ff2_a, w_ff2_b):
    B, T, D = x.shape
    K = dw.shape[0]
    F = w_ff1_a.shape[1]
    N = B * T
    TM = 2 * H
    NT = N // TM
    TP = (T // 2 + 127) // 128 * 128
    Dh = D // 2
    kern = functools.partial(_kernel, B=B, T=T, D=D, K=K, F=F)
    hbm = pl.BlockSpec(memory_space=pl.ANY)
    V = pltpu.VMEM
    out = pl.pallas_call(
        kern,
        out_shape=jax.ShapeDtypeStruct((N, D), x.dtype),
        in_specs=[hbm] * 12,
        out_specs=hbm,
        scratch_shapes=[
            V((N, D), f32),
            V((NT, 7, H, Dh), bf16),
            V((B, 7, TP, Dh), bf16),
            V((B, 7, TP, Dh), bf16),
            V((7, Dh, F // 2), bf16),
            V((7, F // 2, Dh), bf16),
            V((2, 7, Dh, Dh), bf16),
            V((7, Dh, Dh), bf16),
            V((K, 4, 8, 128), f32),
            V((TP // W, 4, H, W), f32),
            V((2, H, 128), f32),
            V((2, TP // W - 1, 2, H, 128), f32),
            V((8, 128), jnp.int32),
        ],
        compiler_params=pltpu.CompilerParams(vmem_limit_bytes=VMEM_LIMIT),
    )(x.reshape(N, D), w_ff1_a, w_ff1_b, w_q, w_k, w_v, w_o, w_pw1, dw, w_pw2, w_ff2_a, w_ff2_b)
    return out.reshape(B, T, D)
```

```python
import functools
import jax
import jax.numpy as jnp
from jax import lax
import jax.experimental.pallas as pl
import jax.experimental.pallas.tpu as pltpu

H = 400
W = 512
EPS = 1e-5
LOG2E = 1.4426950408889634
NEG = -1e30
ELAG = 2
UPO = (1, 2, 0, 5, 3, 4, 6)
DNO = (1, 3, 6, 0, 2, 4, 5)
DQORD = (2, 0, 1, 3)
PR = (40, 40, 40, 40)
P2G = 8
EPI_CH = 1
EPI_LAST = 2
HG = 32
LINK = 1
P2END = 10
PCHF = 8
PCH = 4
ECH = 1
PEEL_UNROLL = 2
PVU = 2
ONLY = None
VMEM_LIMIT = 127 * 1024 * 1024

bf16 = jnp.bfloat16
f32 = jnp.float32


def _ln(x):
    m = jnp.mean(x, axis=-1, keepdims=True)
    c = x - m
    v = jnp.mean(c * c, axis=-1, keepdims=True)
    return c * lax.rsqrt(v + EPS)


def _hsilu(h):
    return h * jnp.tanh(h) + h


def _hglu(a, b):
    return a * jnp.tanh(b) + a


def _dot(a, b):
    return jnp.dot(a, b, preferred_element_type=f32)


def _dot_nt(a, b):
    return lax.dot_general(a, b, (((1,), (1,)), ((), ())), preferred_element_type=f32)


def _a_sums(A11, A12, A21, A22):
    return [A11 + A22, A21 + A22, A11, A22, A11 + A12, A21 - A11, A12 - A22]


def _a_ops(*q):
    return [t.astype(bf16) for t in _a_sums(*q)]


def _b_ops(B11, B12, B21, B22):
    return [t.astype(bf16) for t in
            (B11 + B22, B11, B12 - B22, B21 - B11, B22, B11 + B12, B21 + B22)]


def _smm(a, w, order=UPO, dot=_dot):
    M = [None] * 7
    for k in order:
        M[k] = dot(a(k), w(k))
    return (M[0] + M[3] - M[4] + M[6], M[2] + M[4], M[1] + M[3], M[0] - M[1] + M[2] + M[5])


def _cat(a, b):
    return jnp.concatenate([a, b], axis=1)


def _kernel(x_hbm, w1a_h, w1b_h, wq_h, wk_h, wv_h, wo_h, wp1_h, dw_h, wp2_h, w2a_h, w2b_h, out_hbm,
            xr, hops, kops, vops, wa, wb, wp1, wp2, dwb, sbuf, mbuf, cstat, zref, *, B, T, D, K, F):
    N = B * T
    TM = 2 * H
    NTB = T // TM
    NT = B * NTB
    TH = T // 2
    TP = kops.shape[2]
    NC = TP // W
    Dh = D // 2
    cat = _cat
    ident = tuple(range(7))

    zref[...] = jnp.zeros_like(zref)

    def tie(prev, v):
        if prev is None:
            return v
        never = jnp.tile(zref[...], (v.shape[0] // 8, 1)) != 0
        return jnp.where(never, prev, v)

    def tie0(prev, v):
        return v if prev is None else cat(tie(prev, v[:, :128]), v[:, 128:])

    def rows(i, off=0, n=H):
        return pl.ds(pl.multiple_of(i * TM + off, 16), n)

    def ln_chain(load, store=None, prev=None, chained=True):
        if not chained:
            ht, hb = _ln(load(0, H)), _ln(load(H, H))
            ops = _a_ops(ht[:, :Dh], ht[:, Dh:], hb[:, :Dh], hb[:, Dh:])
            if store is not None:
                for k in range(7):
                    store(k, 0, H, ops[k])
            return ops, None
        outs = [[] for _ in range(7)]
        for r in range(0, H, 16):
            ht, hb = _ln(tie0(prev, load(r, 16))), _ln(load(H + r, 16))
            s = _a_sums(ht[:, :Dh], ht[:, Dh:], hb[:, :Dh], hb[:, Dh:])
            prev = s[0][:, :128]
            for k in range(7):
                o = s[k].astype(bf16)
                outs[k].append(o)
                if store is not None:
                    store(k, r, 16, o)
        return [jnp.concatenate(o, axis=0) for o in outs], prev

    def chained(fn, x, pr):
        if pr == 0:
            return fn(x)
        prev = None
        cols = []
        for t in range(x.shape[1] // 128):
            parts = []
            for r in range(0, x.shape[0], pr):
                prev = fn(tie(prev, x[r:r + pr, t * 128:(t + 1) * 128]))
                parts.append(prev)
            cols.append(jnp.concatenate(parts, axis=0))
        return jnp.concatenate(cols, axis=1)

    def build_b_ops(raw, dst, r0, nr, c0, n, scale, chained=True, prev=None):
        k = raw.shape[0] // 2
        nh = n // 2
        for r in range(0, nr, 16):
            for c in range(0, nh, 128):
                def blk(ro, co):
                    return raw[pl.ds(ro + r0 + r, 16), c0 + co + c:c0 + co + c + 128].astype(f32) * scale
                B11, B12, B21, B22 = tie(prev if chained else None, blk(0, 0)), blk(0, nh), blk(k, 0), blk(k, nh)
                prev = (B11 + B12) + (B21 + B22)
                ops = _b_ops(B11, B12, B21, B22)
                for i in range(7):
                    dst[i, pl.ds(r0 + r, 16), c:c + 128] = ops[i]
        return prev

    QORD = (3, 2, 1, 0)

    def qidx(i, q):
        return rows(i, (q // 2) * H), slice((q % 2) * Dh, (q % 2 + 1) * Dh)

    def ff_up(hnops, slot):
        C = _smm(lambda k: hnops[slot, k], lambda k: wa[k], UPO)
        return [chained(_hsilu, C[q], PR[q]) for q in range(4)]

    def ff_down(U):
        a = _a_ops(*U)
        return _smm(lambda k: a[k], lambda k: wb[k], DNO)

    def stage_C1(i, prev=None):
        def st(k, r, n, v):
            hops[i, k, r:r + n, :] = v
        return ln_chain(lambda r, n: xr[rows(i, r, n), :], st, prev)

    def stage_C2(wkv, i, a):
        b = i // NTB
        r = pl.ds(pl.multiple_of((i % NTB) * H, 16), H)
        c = D ** -0.5 * LOG2E
        ktl, kth, kbl, kbh = [t * c for t in _smm(lambda k: a[k], lambda k: wkv[0, k])]
        ops = _b_ops(ktl, kbl, kth, kbh)
        for k in range(7):
            kops[b, k, r, :] = ops[k]
        vtl, vth, vbl, vbh = _smm(lambda k: a[k], lambda k: wkv[1, k])
        ops = _b_ops(vtl, vth, vbl, vbh)
        for k in range(7):
            vops[b, k, r, :] = ops[k]

    def att_qk(i):
        b = i // NTB
        for c in range(NC):
            s = list(_smm(lambda k: hops[i, k], lambda k: kops[b, k, c * W:(c + 1) * W, :], ident, _dot_nt))
            nv = TH - c * W
            for j in range(4):
                t = s[j]
                if nv < W:
                    lo = nv // 128 * 128
                    col = lax.broadcasted_iota(jnp.int32, (H, W - lo), 1)
                    t = cat(t[:, :lo], jnp.where(col < nv - lo, t[:, lo:], NEG))
                sbuf[c, j] = t

    def att_stats():
        prev = [None] * PCH
        n = 0
        for c in range(NC):
            if c == NC - 1:
                prev = [prev[t % PCH] for t in range(PCHF)]
            nch = len(prev)
            for r in range(0, H, P2G):
                for half in range(2):
                    rs = slice(r, r + P2G)
                    blocks = [sbuf[c, 2 * half + j, rs, t * 128:(t + 1) * 128]
                              for j in (0, 1) for t in range(W // 128)]
                    blocks[0] = tie(prev[n % nch], blocks[0])
                    m = jnp.broadcast_to(
                        jnp.max(functools.reduce(jnp.maximum, blocks), axis=-1, keepdims=True), (P2G, 128))
                    if c < NC - 1:
                        l = functools.reduce(jnp.add, [jnp.exp2(t - m) for t in blocks])
                        cstat[0, c, half, rs, :] = m
                        cstat[1, c, half, rs, :] = l
                        prev[n % nch] = l
                    else:
                        ms = [cstat[0, cc, half, rs, :] for cc in range(NC - 1)]
                        m = functools.reduce(jnp.maximum, ms + [m])
                        l = functools.reduce(jnp.add, [jnp.exp2(t - m) for t in blocks]
                                             + [cstat[1, cc, half, rs, :] * jnp.exp2(ms[cc] - m) for cc in range(NC - 1)])
                        mp = m + jnp.log2(jnp.sum(l, axis=-1, keepdims=True))
                        mbuf[half, rs, :] = mp
                        prev[n % nch] = mp
                    n += 1

    def att_pv(i, side, unroll=1):
        b = i // NTB

        def trip(c, prev):
            mt = jnp.concatenate([mbuf[0]] * (W // 128), axis=1)
            mb = jnp.concatenate([mbuf[1]] * (W // 128), axis=1)
            ms = (mt, mt, mb, mb)
            a = _a_ops(*[jnp.exp2(sbuf[c, j] - ms[j]) for j in range(4)])
            kr = pl.ds(pl.multiple_of(c * W, W), W)
            O = _smm(lambda k: a[k], lambda k: vops[b, k, kr, :])
            for q in QORD:
                xr[qidx(i, q)] = xr[qidx(i, q)] + O[q]
            return side(c, prev)

        def rolled(t, carry):
            prev = None
            for u in range(unroll):
                prev = trip(t * unroll + u, prev)
            return carry

        if unroll >= NC:
            rolled(0, 0)
        else:
            lax.fori_loop(0, NC // unroll, rolled, 0)

    def front(hnops, wkv, xbuf, rawa, rawb, rawq, rawp1, rawp2, rawdw, xsem, wsem):
        def xcopy(t, slot):
            return pltpu.make_async_copy(x_hbm.at[pl.ds(pl.multiple_of(t * TM, 16), TM), :], xbuf.at[slot], xsem.at[slot])

        cp = [
            pltpu.make_async_copy(wq_h, rawq.at[0], wsem.at[0]),
            pltpu.make_async_copy(wk_h, rawq.at[1], wsem.at[1]),
            pltpu.make_async_copy(wv_h, rawq.at[2], wsem.at[2]),
            pltpu.make_async_copy(wo_h, rawq.at[3], wsem.at[3]),
            pltpu.make_async_copy(w1a_h, rawa, wsem.at[4]),
            pltpu.make_async_copy(w1b_h, rawb, wsem.at[5]),
            pltpu.make_async_copy(dw_h, rawdw, wsem.at[6]),
            pltpu.make_async_copy(wp1_h, rawp1, wsem.at[7]),
            pltpu.make_async_copy(wp2_h, rawp2, wsem.at[8]),
            pltpu.make_async_copy(w2a_h, rawa, wsem.at[9]),
            pltpu.make_async_copy(w2b_h, rawb, wsem.at[10]),
        ]
        CQ, CK, CV, CO, C1A, C1B, CDW, CP1, CP2, C2A, C2B = range(11)

        def stage_A(t, slot, chained=True):
            xs = t % 3

            def st(k, r, n, v):
                hnops[slot, k, r:r + n, :] = v
            return ln_chain(lambda r, n: xbuf[xs, r:r + n, :].astype(f32), st, chained=chained)[1]

        def stage_B2(i, U):
            d = ff_down(U)
            xs = i % 3
            for q in DQORD:
                r0, c0 = (q // 2) * H, (q % 2) * Dh
                xr[qidx(i, q)] = xbuf[xs, r0:r0 + H, c0:c0 + Dh].astype(f32) + d[q]

        def p1(i, carry, dma=True):
            if dma:
                @pl.when(i + 2 < NT)
                def _():
                    xcopy(i + 2, (i + 2) % 3).start()

                @pl.when(i + 1 < NT)
                def _():
                    xcopy(i + 1, (i + 1) % 3).wait()
            U = ff_up(hnops, i % 2)
            prev = stage_A(jnp.minimum(i + 1, NT - 1), (i + 1) % 2)
            hq, _ = stage_C1(i - 1, prev)
            stage_B2(i, U)
            stage_C2(wkv, i - 1, hq)
            return carry

        if ONLY == 'p1':
            lax.fori_loop(1, NT, lambda i, c: p1(i, c, False), 0)
            return
        if ONLY is not None:
            return
        cp[C1A].start()
        xcopy(0, 0).start()
        for b in range(B):
            for k in range(7):
                kops[b, k, TH:, :] = jnp.zeros((TP - TH, Dh), bf16)
                vops[b, k, TH:, :] = jnp.zeros((TP - TH, Dh), bf16)
        xcopy(0, 0).wait()
        cp[C1B].start()
        stage_A(0, 0, chained=False)
        cp[C1A].wait()
        for c_ in (cp[CQ], cp[CK], cp[CV], cp[CO], xcopy(1, 1), cp[CDW], xcopy(2, 2), cp[CP1], cp[CP2]):
            c_.start()
        build_b_ops(rawa, wa, 0, Dh, 0, F, 0.5, chained=False)
        U = ff_up(hnops, 0)
        cp[C1B].wait()
        build_b_ops(rawb, wb, 0, F // 2, 0, D, 0.5)
        cp[CQ].wait()
        cp[CK].wait()
        wf = _dot_nt(rawq[1], rawq[0])
        ops = _b_ops(wf[:Dh, :Dh], wf[:Dh, Dh:], wf[Dh:, :Dh], wf[Dh:, Dh:])
        for k in range(7):
            wkv[0, k] = ops[k]
        cp[CV].wait()
        cp[CO].wait()
        wf = _dot(rawq[2], rawq[3])
        ops = _b_ops(wf[:Dh, :Dh], wf[:Dh, Dh:], wf[Dh:, :Dh], wf[Dh:, Dh:])
        for k in range(7):
            wkv[1, k] = ops[k]
        xcopy(1, 1).wait()
        stage_A(1, 1)
        stage_B2(0, U)
        cp[CDW].wait()
        dwv = rawdw[...].astype(f32)
        for k in range(K):
            for cb in range(4):
                dwb[k, cb] = jnp.broadcast_to(dwv[k:k + 1, cb * 128:(cb + 1) * 128], (8, 128))
        cp[C2A].start()
        cp[C2B].start()

        with jax.named_scope("p1loop"):
            lax.fori_loop(1, NT, p1, 0)

        cp[CP1].wait()
        cp[CP2].wait()
        cp[C2A].wait()
        cp[C2B].wait()

        def wops(c, prev):
            q = Dh // NC
            r0 = c * q if isinstance(c, int) else pl.multiple_of(c * q, 16)
            r1 = c * (F // 2 // NC) if isinstance(c, int) else pl.multiple_of(c * (F // 2 // NC), 16)
            prev = build_b_ops(rawp1, wp1.at[0], r0, q, 0, D, 0.5, prev=prev)
            prev = build_b_ops(rawp1, wp1.at[1], r0, q, D, D, 0.5, prev=prev)
            prev = build_b_ops(rawp2, wp2, r0, q, 0, D, 1.0, prev=prev)
            prev = build_b_ops(rawa, wa, r0, q, 0, F, 0.5, prev=prev)
            return build_b_ops(rawb, wb, r1, F // 2 // NC, 0, D, 0.5, prev=prev)

        with jax.named_scope("p2peel"):
            hq, _ = stage_C1(NT - 1)
            att_qk(0)
            stage_C2(wkv, NT - 1, hq)
            att_stats()
            att_pv(0, wops, unroll=PEEL_UNROLL)

    V = pltpu.VMEM
    with jax.named_scope("front"):
        pl.run_scoped(front, V((2, 7, H, Dh), bf16), V((2, 7, Dh, Dh), bf16), V((3, TM, D), bf16), V((D, F), bf16), V((F, D), bf16), V((4, D, D), bf16),
                      V((D, 2 * D), bf16), V((D, D), bf16), V((K, D), bf16),
                      pltpu.SemaphoreType.DMA((3,)), pltpu.SemaphoreType.DMA((11,)))

    def back(dc, stats):
        def attention(gbuf):
            def stage_D1(j, chained=True):
                return ln_chain(lambda r, n: xr[rows(j, r, n), :], chained=chained)[0]

            def stage_D2(j, a):
                ga = _smm(lambda k: a[k], lambda k: wp1[0, k])
                gb_ = _smm(lambda k: a[k], lambda k: wp1[1, k])
                g = [_hglu(u, v) for u, v in zip(ga, gb_)]
                slot = j % 4
                jb = j % NTB
                first = jb == 0
                last = jb == NTB - 1
                for q in QORD:
                    for t in range(2):
                        cb = 2 * (q % 2) + t
                        v = g[q][:, t * 128:(t + 1) * 128]
                        r0 = 8 + (q // 2) * H
                        gbuf[slot, cb, r0:r0 + H, :] = v
                        if q // 2 == 0:
                            gbuf[(j + 3) % 4, cb, 8 + TM:16 + TM, :] = jnp.where(first, 0.0, v[0:8])
                        else:
                            gbuf[(j + 1) % 4, cb, 0:8, :] = jnp.where(last, 0.0, v[H - 8:H])

            def stage_E(j, cb, nch, head=None):
                slot = j % 4
                w = [dwb[k, cb] for k in range(K)]
                prev = [head] * max(nch, 1)
                shift = s1 = s2 = None
                for n, r0 in enumerate(range(0, TM, 8)):
                    acc = None
                    for k in range(K):
                        t = gbuf[slot, cb, pl.ds(r0 + k + 8 - K // 2, 8), :] * w[k]
                        if acc is None:
                            acc = tie(prev[n % nch], t) if nch else t
                        else:
                            acc = acc + t
                    dc[cb, pl.ds(pl.multiple_of(j * TM + r0, 8), 8), :] = acc
                    if nch:
                        prev[n % nch] = acc
                    if shift is None:
                        shift = acc
                    else:
                        d = acc - shift
                        s1 = d if s1 is None else s1 + d
                        s2 = d * d if s2 is None else s2 + d * d
                ns = TM // 8
                js = pl.ds(pl.multiple_of(j * 8, 8), 8)
                stats[0, cb, js, :] = shift + s1 * (1.0 / ns)
                stats[1, cb, js, :] = s2 - s1 * s1 * (1.0 / ns)
                return prev[-1]

            for cb in range(4):
                gbuf[0, cb, 0:8, :] = jnp.zeros((8, 128), f32)

            def p2(i, carry):
                je = jnp.maximum(i - ELAG, 0)
                a = stage_D1(i - 1)
                att_qk(i)
                stage_D2(i - 1, a)
                att_stats()
                att_pv(i, lambda c, prev: stage_E(je, c, ECH, prev), PVU)
                return carry

            if ONLY in ('p1', 'p4'):
                return
            with jax.named_scope("p2loop"):
                lax.fori_loop(1, P2END, p2, 0)
            if ONLY is not None:
                return

            a = stage_D1(NT - 1, chained=False)
            stage_D2(NT - 1, a)
            for cb in range(4):
                gbuf[(NT - 1) % 4, cb, 8 + TM:16 + TM, :] = jnp.zeros((8, 128), f32)
            for j in range(NT - ELAG, NT):
                for cb in range(4):
                    stage_E(j, cb, EPI_CH if j < NT - 1 else EPI_LAST)

        pl.run_scoped(attention, V((4, 4, TM + 16, 128), f32))

        st0 = jnp.concatenate([stats[0, cb] for cb in range(4)], axis=1)
        st1 = jnp.concatenate([stats[1, cb] for cb in range(4)], axis=1)
        mu = jnp.sum(st0, axis=0, keepdims=True) * (1.0 / (8 * NT))
        dm = st0 - mu
        var = jnp.sum(st1 + (TM // 8) * dm * dm, axis=0, keepdims=True) * (1.0 / N)
        rsd = 0.5 * lax.rsqrt(var + EPS)

        def final(hnops, zops, obuf, osem):
            def ocopy(t, slot):
                return pltpu.make_async_copy(obuf.at[slot], out_hbm.at[pl.ds(pl.multiple_of(t * TM, 16), TM), :], osem.at[slot])

            def stage_F1(j, prev=None, chained=True):
                def zq(r0, n, hi):
                    d = jnp.concatenate([dc[2 * hi + t, rows(j, r0, n), :] for t in range(2)], axis=1)
                    return (d - mu[:, hi * Dh:(hi + 1) * Dh]) * rsd[:, hi * Dh:(hi + 1) * Dh]
                if not chained:
                    ops = _a_ops(*[_hsilu(zq(r0, H, hi)) for r0 in (0, H) for hi in (0, 1)])
                    for k in range(7):
                        zops[k] = ops[k]
                    return
                for r in range(0, H, 16):
                    z = []
                    for r0 in (0, H):
                        for hi in (0, 1):
                            t = _hsilu(tie0(prev, zq(r0 + r, 16, hi)))
                            prev = t[:, :128] + t[:, 128:]
                            z.append(t)
                    for k, o in enumerate(_a_ops(*z)):
                        zops[k, r:r + 16, :] = o

            def stage_F2(j):
                E = _smm(lambda k: zops[k], lambda k: wp2[k])
                for q in QORD:
                    xr[qidx(j, q)] = xr[qidx(j, q)] + E[q]

            def stage_F3(j, slot, prev=None, chained=True):
                def st(k, r, n, v):
                    hnops[slot, k, r:r + n, :] = v
                return ln_chain(lambda r, n: xr[rows(j, r, n), :], st, prev, chained=chained)[1]

            def stage_G2(i, U):
                d = ff_down(U)
                for q in DQORD:
                    xr[qidx(i, q)] = xr[qidx(i, q)] + d[q]

            def stage_Hh(j, chained=True):
                slot = j % 2
                if not chained:
                    obuf[slot, 0:H, :] = _ln(xr[rows(j), :]).astype(bf16)
                    obuf[slot, H:TM, :] = _ln(xr[rows(j, H), :]).astype(bf16)
                    return None
                prev = None
                for r in range(0, TM, HG):
                    y = _ln(tie0(prev, xr[rows(j, r, HG), :]))
                    prev = y[:, :128]
                    obuf[slot, r:r + HG, :] = y.astype(bf16)
                return prev

            if ONLY in ('p1', 'p2'):
                return
            if ONLY is None:
                stage_F1(0, chained=False)
                stage_F2(0)
                stage_F3(0, 0, chained=False)
                stage_F1(1, chained=False)

            def p4(i, carry):
                if ONLY is None:
                    @pl.when(i >= 3)
                    def _():
                        ocopy(i - 3, (i - 3) % 2).wait()
                stage_F2(i + 1)
                U = ff_up(hnops, i % 2)
                prev = stage_Hh(jnp.maximum(i - 1, 0))
                prev = stage_F3(i + 1, (i + 1) % 2, prev[0:16] if LINK & 1 else None)
                stage_F1(jnp.minimum(i + 2, NT - 1), prev if LINK & 2 else None)
                stage_G2(i, U)

                if ONLY is None:
                    @pl.when(i >= 1)
                    def _():
                        ocopy(i - 1, (i - 1) % 2).start()
                return carry

            with jax.named_scope("p4loop"):
                lax.fori_loop(0, NT - 1, p4, 0)
            if ONLY is not None:
                return

            ocopy(NT - 4, (NT - 4) % 2).wait()
            U = ff_up(hnops, (NT - 1) % 2)
            stage_Hh(NT - 2)
            stage_G2(NT - 1, U)
            ocopy(NT - 3, (NT - 3) % 2).wait()
            ocopy(NT - 2, (NT - 2) % 2).start()
            stage_Hh(NT - 1, chained=False)
            ocopy(NT - 1, (NT - 1) % 2).start()
            ocopy(NT - 2, (NT - 2) % 2).wait()
            ocopy(NT - 1, (NT - 1) % 2).wait()

        pl.run_scoped(final, V((2, 7, H, Dh), bf16), V((7, H, Dh), bf16), V((2, TM, D), bf16),
                      pltpu.SemaphoreType.DMA((2,)))

    with jax.named_scope("back"):
        pl.run_scoped(back, V((4, N, 128), f32), V((2, 4, 8 * NT, 128), f32))


@jax.jit
def pallas_standalone__conformer_family_conformer__speech_kernel(
    x, w_ff1_a, w_ff1_b, w_q, w_k, w_v, w_o, w_pw1, dw, w_pw2, w_ff2_a, w_ff2_b):
    B, T, D = x.shape
    K = dw.shape[0]
    F = w_ff1_a.shape[1]
    N = B * T
    TM = 2 * H
    NT = N // TM
    TP = (T // 2 + 127) // 128 * 128
    Dh = D // 2
    kern = functools.partial(_kernel, B=B, T=T, D=D, K=K, F=F)
    hbm = pl.BlockSpec(memory_space=pl.ANY)
    V = pltpu.VMEM
    out = pl.pallas_call(
        kern,
        out_shape=jax.ShapeDtypeStruct((N, D), x.dtype),
        in_specs=[hbm] * 12,
        out_specs=hbm,
        scratch_shapes=[
            V((N, D), f32),
            V((NT, 7, H, Dh), bf16),
            V((B, 7, TP, Dh), bf16),
            V((B, 7, TP, Dh), bf16),
            V((7, Dh, F // 2), bf16),
            V((7, F // 2, Dh), bf16),
            V((2, 7, Dh, Dh), bf16),
            V((7, Dh, Dh), bf16),
            V((K, 4, 8, 128), f32),
            V((TP // W, 4, H, W), f32),
            V((2, H, 128), f32),
            V((2, TP // W - 1, 2, H, 128), f32),
            V((8, 128), jnp.int32),
        ],
        compiler_params=pltpu.CompilerParams(vmem_limit_bytes=VMEM_LIMIT),
    )(x.reshape(N, D), w_ff1_a, w_ff1_b, w_q, w_k, w_v, w_o, w_pw1, dw, w_pw2, w_ff2_a, w_ff2_b)
    return out.reshape(B, T, D)
```

```python
import functools
import jax
import jax.numpy as jnp
from jax import lax
import jax.experimental.pallas as pl
import jax.experimental.pallas.tpu as pltpu

H = 400
W = 512
EPS = 1e-5
LOG2E = 1.4426950408889634
NEG = -1e30
HALO = 16
UPO = (1, 2, 0, 5, 3, 4, 6)
DNO = (1, 3, 6, 0, 2, 4, 5)
DQORD = (2, 0, 1, 3)
PR = (40, 40, 40, 40)
P2G = 8
EPI_CH = 2
EPI_LAST = 0
EPI_LN = 9
LCH1 = 2
LCH4 = 2
HCH = 1
LCHD = 1
BLINK = 2
HG = 32
LINK = 1
ZDMA = True
ZN = 1
PADK = 1
P1END = 10
P4END = 9
P2END = 10
PCHF = 8
PCH = 4
ECH = 1
PEEL_UNROLL = 2
PEEL_PCH = 16
PEEL_ROLL = False
PVU = 2
ONLY = None
VMEM_LIMIT = 127 * 1024 * 1024

bf16 = jnp.bfloat16
f32 = jnp.float32


def _ln(x):
    m = jnp.mean(x, axis=-1, keepdims=True)
    c = x - m
    v = jnp.mean(c * c, axis=-1, keepdims=True)
    return c * lax.rsqrt(v + EPS)


def _hsilu(h):
    return h * jnp.tanh(h) + h


def _hglu(a, b):
    return a * jnp.tanh(b) + a


def _dot(a, b):
    return jnp.dot(a, b, preferred_element_type=f32)


def _dot_nt(a, b):
    return lax.dot_general(a, b, (((1,), (1,)), ((), ())), preferred_element_type=f32)


def _a_sums(A11, A12, A21, A22):
    return [A11 + A22, A21 + A22, A11, A22, A11 + A12, A21 - A11, A12 - A22]


def _a_ops(*q):
    return [t.astype(bf16) for t in _a_sums(*q)]


def _b_ops(B11, B12, B21, B22):
    return [t.astype(bf16) for t in
            (B11 + B22, B11, B12 - B22, B21 - B11, B22, B11 + B12, B21 + B22)]


def _smm(a, w, order=UPO, dot=_dot):
    M = [None] * 7
    for k in order:
        M[k] = dot(a(k), w(k))
    return (M[0] + M[3] - M[4] + M[6], M[2] + M[4], M[1] + M[3], M[0] - M[1] + M[2] + M[5])


def _cat(a, b):
    return jnp.concatenate([a, b], axis=1)


def _kernel(x_hbm, w1a_h, w1b_h, wq_h, wk_h, wv_h, wo_h, wp1_h, dw_h, wp2_h, w2a_h, w2b_h, out_hbm,
            xr, hops, kops, vops, wa, wb, wp1, wp2, dwb, sbuf, mbuf, cstat, zsrc, zref, padbuf, zsem, *, B, T, D, K, F):
    N = B * T
    TM = 2 * H
    NTB = T // TM
    NT = B * NTB
    TH = T // 2
    TP = kops.shape[2]
    NC = TP // W
    Dh = D // 2
    cat = _cat
    ident = tuple(range(7))

    if ZDMA:
        zsrc[...] = jnp.zeros_like(zsrc)
        zcopy = pltpu.make_async_copy(zsrc, zref, zsem)
        zcopy.start()
        zcopy.wait()
    else:
        zref[...] = jnp.zeros_like(zref)

    def tie(prev, v):
        if prev is None:
            return v
        never = jnp.tile(zref[0:8, :], (v.shape[0] // 8, 1)) != 0
        return jnp.where(never, prev, v)

    def tie0(prev, v):
        return v if prev is None else cat(tie(prev, v[:, :128]), v[:, 128:])

    def al16(v):
        return v if isinstance(v, int) else pl.multiple_of(v, 16)

    def rows(i, off=0, n=H):
        return pl.ds(al16(i * TM + off), n)

    def ln_chain(load, store=None, prev=None, chained=True, nch=1):
        if not chained:
            ht, hb = _ln(load(0, H)), _ln(load(H, H))
            ops = _a_ops(ht[:, :Dh], ht[:, Dh:], hb[:, :Dh], hb[:, Dh:])
            if store is not None:
                for k in range(7):
                    store(k, 0, H, ops[k])
            return ops, None
        outs = [[] for _ in range(7)]
        heads = [prev] * nch
        for n, r in enumerate(range(0, H, 16)):
            ht, hb = _ln(tie0(heads[n % nch], load(r, 16))), _ln(load(H + r, 16))
            s = _a_sums(ht[:, :Dh], ht[:, Dh:], hb[:, :Dh], hb[:, Dh:])
            prev = heads[n % nch] = s[0][:, :128]
            for k in range(7):
                o = s[k].astype(bf16)
                outs[k].append(o)
                if store is not None:
                    store(k, r, 16, o)
        return [jnp.concatenate(o, axis=0) for o in outs], prev

    def chained(fn, x, pr):
        if pr == 0:
            return fn(x)
        prev = None
        cols = []
        for t in range(x.shape[1] // 128):
            parts = []
            for r in range(0, x.shape[0], pr):
                prev = fn(tie(prev, x[r:r + pr, t * 128:(t + 1) * 128]))
                parts.append(prev)
            cols.append(jnp.concatenate(parts, axis=0))
        return jnp.concatenate(cols, axis=1)

    def build_b_ops(raw, dst, r0, nr, c0, n, scale, chained=True, prev=None):
        k = raw.shape[0] // 2
        nh = n // 2
        n_ = 0
        for r in range(0, nr, 16):
            for c in range(0, nh, 128):
                def blk(ro, co):
                    return raw[pl.ds(al16(ro + r0 + r), 16), c0 + co + c:c0 + co + c + 128].astype(f32) * scale
                B11, B12, B21, B22 = tie(prev if chained else None, blk(0, 0)), blk(0, nh), blk(k, 0), blk(k, nh)
                n_ += 1
                if n_ % BLINK == 0:
                    prev = jnp.broadcast_to(jnp.max((B11 + B12) + (B21 + B22), axis=-1, keepdims=True), (16, 128))
                ops = _b_ops(B11, B12, B21, B22)
                for i in range(7):
                    dst[i, pl.ds(al16(r0 + r), 16), c:c + 128] = ops[i]
        return prev

    QORD = (3, 2, 1, 0)

    def qidx(i, q):
        return rows(i, (q // 2) * H), slice((q % 2) * Dh, (q % 2 + 1) * Dh)

    def ff_up(hnops, slot):
        C = _smm(lambda k: hnops[slot, k], lambda k: wa[k], UPO)
        return [chained(_hsilu, C[q], PR[q]) for q in range(4)]

    def ff_down(U):
        a = _a_ops(*U)
        return _smm(lambda k: a[k], lambda k: wb[k], DNO)

    def stage_C1(i, prev=None, chained=True):
        def st(k, r, n, v):
            hops[i, k, r:r + n, :] = v
        return ln_chain(lambda r, n: xr[rows(i, r, n), :], st, prev, chained=chained, nch=LCH1)

    def stage_C2(wkv, i, a):
        b = i // NTB
        r = pl.ds(pl.multiple_of((i % NTB) * H, 16), H)
        c = D ** -0.5 * LOG2E
        ktl, kth, kbl, kbh = [t * c for t in _smm(lambda k: a[k], lambda k: wkv[0, k])]
        ops = _b_ops(ktl, kbl, kth, kbh)
        for k in range(7):
            kops[b, k, r, :] = ops[k]
        vtl, vth, vbl, vbh = _smm(lambda k: a[k], lambda k: wkv[1, k])
        ops = _b_ops(vtl, vth, vbl, vbh)
        for k in range(7):
            vops[b, k, r, :] = ops[k]

    def att_qk(i, rolled=False):
        b = i // NTB

        def chunk(c, carry=None):
            static = isinstance(c, int)
            kr = slice(c * W, (c + 1) * W) if static else pl.ds(pl.multiple_of(c * W, W), W)
            s = list(_smm(lambda k: hops[i, k], lambda k: kops[b, k, kr, :], ident, _dot_nt))
            nv = TH - c * W
            for j in range(4):
                t = s[j]
                if not static:
                    t = jnp.where(lax.broadcasted_iota(jnp.int32, (H, W), 1) < nv, t, NEG)
                elif nv < W:
                    lo = nv // 128 * 128
                    col = lax.broadcasted_iota(jnp.int32, (H, W - lo), 1)
                    t = cat(t[:, :lo], jnp.where(col < nv - lo, t[:, lo:], NEG))
                sbuf[c, j] = t
            return carry

        if rolled:
            lax.fori_loop(0, NC, chunk, 0)
        else:
            for c in range(NC):
                chunk(c)

    def att_stats(nch0=None, nchf=None):
        nch0, nchf = nch0 or PCH, nchf or PCHF
        prev = [None] * nch0
        n = 0
        for c in range(NC):
            if c == NC - 1:
                prev = [prev[t % nch0] for t in range(nchf)]
            nch = len(prev)
            for r in range(0, H, P2G):
                for half in range(2):
                    rs = slice(r, r + P2G)
                    blocks = [sbuf[c, 2 * half + j, rs, t * 128:(t + 1) * 128]
                              for j in (0, 1) for t in range(W // 128)]
                    blocks[0] = tie(prev[n % nch], blocks[0])
                    m = jnp.broadcast_to(
                        jnp.max(functools.reduce(jnp.maximum, blocks), axis=-1, keepdims=True), (P2G, 128))
                    if c < NC - 1:
                        l = functools.reduce(jnp.add, [jnp.exp2(t - m) for t in blocks])
                        cstat[0, c, half, rs, :] = m
                        cstat[1, c, half, rs, :] = l
                        prev[n % nch] = l
                    else:
                        ms = [cstat[0, cc, half, rs, :] for cc in range(NC - 1)]
                        m = functools.reduce(jnp.maximum, ms + [m])
                        l = functools.reduce(jnp.add, [jnp.exp2(t - m) for t in blocks]
                                             + [cstat[1, cc, half, rs, :] * jnp.exp2(ms[cc] - m) for cc in range(NC - 1)])
                        mp = m + jnp.log2(jnp.sum(l, axis=-1, keepdims=True))
                        mbuf[half, rs, :] = mp
                        prev[n % nch] = mp
                    n += 1

    def att_pv(i, side, unroll=1):
        b = i // NTB

        def trip(c, prev):
            mt = jnp.concatenate([mbuf[0]] * (W // 128), axis=1)
            mb = jnp.concatenate([mbuf[1]] * (W // 128), axis=1)
            ms = (mt, mt, mb, mb)
            a = _a_ops(*[jnp.exp2(sbuf[c, j] - ms[j]) for j in range(4)])
            kr = pl.ds(pl.multiple_of(c * W, W), W)
            O = _smm(lambda k: a[k], lambda k: vops[b, k, kr, :])
            for q in QORD:
                xr[qidx(i, q)] = xr[qidx(i, q)] + O[q]
            return side(c, prev)

        def rolled(t, carry):
            prev = None
            for u in range(unroll):
                prev = trip(t * unroll + u, prev)
            return carry

        if unroll >= NC:
            rolled(0, 0)
        else:
            lax.fori_loop(0, NC // unroll, rolled, 0)

    def front(hnops, wkv, xbuf, rawa, rawb, rawq, rawp1, rawp2, rawdw, xsem, wsem):
        def xcopy(t, slot):
            return pltpu.make_async_copy(x_hbm.at[pl.ds(pl.multiple_of(t * TM, 16), TM), :], xbuf.at[slot], xsem.at[slot])

        cp = [
            pltpu.make_async_copy(wq_h, rawq.at[0], wsem.at[0]),
            pltpu.make_async_copy(wk_h, rawq.at[1], wsem.at[1]),
            pltpu.make_async_copy(wv_h, rawq.at[2], wsem.at[2]),
            pltpu.make_async_copy(wo_h, rawq.at[3], wsem.at[3]),
            pltpu.make_async_copy(w1a_h, rawa, wsem.at[4]),
            pltpu.make_async_copy(w1b_h, rawb, wsem.at[5]),
            pltpu.make_async_copy(dw_h, rawdw, wsem.at[6]),
            pltpu.make_async_copy(wp1_h, rawp1, wsem.at[7]),
            pltpu.make_async_copy(wp2_h, rawp2, wsem.at[8]),
            pltpu.make_async_copy(w2a_h, rawa, wsem.at[9]),
            pltpu.make_async_copy(w2b_h, rawb, wsem.at[10]),
        ]
        CQ, CK, CV, CO, C1A, C1B, CDW, CP1, CP2, C2A, C2B = range(11)

        def stage_A(t, slot, chained=True):
            xs = t % 3

            def st(k, r, n, v):
                hnops[slot, k, r:r + n, :] = v
            return ln_chain(lambda r, n: xbuf[xs, r:r + n, :].astype(f32), st, chained=chained, nch=LCH1)[1]

        def stage_B2(i, U):
            d = ff_down(U)
            xs = i % 3
            for q in DQORD:
                r0, c0 = (q // 2) * H, (q % 2) * Dh
                xr[qidx(i, q)] = xbuf[xs, r0:r0 + H, c0:c0 + Dh].astype(f32) + d[q]

        def p1(i, carry, dma=True):
            if dma:
                @pl.when(i + 2 < NT)
                def _():
                    xcopy(i + 2, (i + 2) % 3).start()

                @pl.when(i + 1 < NT)
                def _():
                    xcopy(i + 1, (i + 1) % 3).wait()
            U = ff_up(hnops, i % 2)
            prev = stage_A(jnp.minimum(i + 1, NT - 1), (i + 1) % 2)
            hq, _ = stage_C1(i - 1, prev)
            stage_B2(i, U)
            stage_C2(wkv, i - 1, hq)
            return carry

        if ONLY == 'p1':
            lax.fori_loop(1, NT, lambda i, c: p1(i, c, False), 0)
            return
        if ONLY not in (None, 'f0'):
            return
        cp[C1A].start()
        xcopy(0, 0).start()
        for b in range(B):
            for k in range(7):
                kops[b, k, TH:, :] = jnp.zeros((TP - TH, Dh), bf16)
                vops[b, k, TH:, :] = jnp.zeros((TP - TH, Dh), bf16)
        xcopy(0, 0).wait()
        cp[C1B].start()
        stage_A(0, 0, chained=False)
        cp[C1A].wait()
        for c_ in (cp[CQ], cp[CK], cp[CV], cp[CO], xcopy(1, 1), cp[CDW], xcopy(2, 2), cp[CP1], cp[CP2]):
            c_.start()
        build_b_ops(rawa, wa, 0, Dh, 0, F, 0.5, chained=False)
        cp[C1B].wait()
        U = ff_up(hnops, 0)
        build_b_ops(rawb, wb, 0, F // 2, 0, D, 0.5)
        for c_ in (cp[CQ], cp[CK], cp[CV], cp[CO], xcopy(1, 1), cp[CDW]):
            c_.wait()
        wf = _dot_nt(rawq[1], rawq[0])
        ops = _b_ops(wf[:Dh, :Dh], wf[:Dh, Dh:], wf[Dh:, :Dh], wf[Dh:, Dh:])
        for k in range(7):
            wkv[0, k] = ops[k]
        wf = _dot(rawq[2], rawq[3])
        ops = _b_ops(wf[:Dh, :Dh], wf[:Dh, Dh:], wf[Dh:, :Dh], wf[Dh:, Dh:])
        for k in range(7):
            wkv[1, k] = ops[k]
        stage_A(1, 1)
        stage_B2(0, U)
        dwv = rawdw[...].astype(f32)
        for k in range(K):
            for cb in range(4):
                dwb[k, cb] = jnp.broadcast_to(dwv[k:k + 1, cb * 128:(cb + 1) * 128], (8, 128))
        cp[C2A].start()
        cp[C2B].start()

        if ONLY == 'f0':
            for c_ in (xcopy(2, 2), cp[CP1], cp[CP2], cp[C2A], cp[C2B]):
                c_.wait()
            return
        with jax.named_scope("p1loop"):
            lax.fori_loop(1, P1END, p1, 0)

        cp[CP1].wait()
        cp[CP2].wait()
        cp[C2A].wait()
        cp[C2B].wait()

        def wops(c, prev):
            q = Dh // NC
            r0 = c * q if isinstance(c, int) else pl.multiple_of(c * q, 16)
            r1 = c * (F // 2 // NC) if isinstance(c, int) else pl.multiple_of(c * (F // 2 // NC), 16)
            prev = build_b_ops(rawp1, wp1.at[0], r0, q, 0, D, 0.5, prev=prev)
            prev = build_b_ops(rawp1, wp1.at[1], r0, q, D, D, 0.5, prev=prev)
            prev = build_b_ops(rawp2, wp2, r0, q, 0, D, 1.0, prev=prev)
            prev = build_b_ops(rawa, wa, r0, q, 0, F, 0.5, prev=prev)
            return build_b_ops(rawb, wb, r1, F // 2 // NC, 0, D, 0.5, prev=prev)

        with jax.named_scope("p2peel"):
            if PEEL_ROLL:
                att_qk(0, rolled=True)
                hq, _ = stage_C1(NT - 1, chained=False)
                stage_C2(wkv, NT - 1, hq)
                att_stats(PEEL_PCH, PEEL_PCH)
            else:
                hq, _ = stage_C1(NT - 1)
                att_qk(0)
                stage_C2(wkv, NT - 1, hq)
                att_stats()
            att_pv(0, wops, unroll=PEEL_UNROLL)

    V = pltpu.VMEM
    with jax.named_scope("front"):
        pl.run_scoped(front, V((2, 7, H, Dh), bf16), V((2, 7, Dh, Dh), bf16), V((3, TM, D), bf16), V((D, F), bf16), V((F, D), bf16), V((4, D, D), bf16),
                      V((D, 2 * D), bf16), V((D, D), bf16), V((K, D), bf16),
                      pltpu.SemaphoreType.DMA((3,)), pltpu.SemaphoreType.DMA((11,)))

    def back(dc, stats):
        def attention(gbuf):
            def stage_D1(j, chained=True):
                return ln_chain(lambda r, n: xr[rows(j, r, n), :], chained=chained, nch=LCHD)[0]

            def stage_D2(j, a):
                ga = _smm(lambda k: a[k], lambda k: wp1[0, k])
                gb_ = _smm(lambda k: a[k], lambda k: wp1[1, k])
                g = [_hglu(u, v) for u, v in zip(ga, gb_)]
                for q in QORD:
                    for t in range(2):
                        cb = 2 * (q % 2) + t
                        v = g[q][:, t * 128:(t + 1) * 128]
                        r0 = HALO + (q // 2) * H
                        gbuf[j % 2, cb, r0:r0 + H, :] = v
                        if q // 2 == 1:
                            gbuf[(j + 1) % 2, cb, 0:HALO, :] = v[H - HALO:H]

            class Conv:
                def __init__(self, j, cb, nch, head=None):
                    self.j, self.cb, self.nch = j, cb, nch
                    self.w = [dwb[k, cb] for k in range(K)]
                    self.prev = [head] * max(nch, 1)
                    self.shift = self.s1 = self.s2 = None
                    first = j % NTB == 0
                    self.lim = (jnp.where(first, HALO, 2 * HALO), jnp.where(first, HALO, 0))

                def step(self, n):
                    j, cb = self.j, self.cb
                    sub = lax.broadcasted_iota(jnp.int32, (8, 128), 0)
                    acc = None
                    for k in range(K):
                        i0 = 8 * n + k + 1
                        t = gbuf[j % 2, cb, pl.ds(i0, 8), :]
                        if n == 0 and i0 + 7 >= HALO:
                            t = jnp.where(sub + i0 < self.lim[0], t, 0.0)
                        if n == 1 and i0 < HALO:
                            t = jnp.where(sub + i0 >= self.lim[1], t, 0.0)
                        t = t * self.w[k]
                        if acc is None:
                            acc = tie(self.prev[n % self.nch], t) if self.nch else t
                        else:
                            acc = acc + t
                    dc[cb, pl.ds(pl.multiple_of(j * TM + 8 * n, 8), 8), :] = acc
                    if self.nch:
                        self.prev[n % self.nch] = acc
                    return acc

                def run(self):
                    j, cb = self.j, self.cb
                    ns = TM // 8
                    shift = self.step(1)
                    s1 = s2 = None
                    for n in [0] + list(range(2, ns)):
                        d = self.step(n) - shift
                        if n == 0:
                            d = jnp.where(j > 0, d, 0.0)
                        s1 = d if s1 is None else s1 + d
                        s2 = d * d if s2 is None else s2 + d * d
                    inv = jnp.where(j > 0, 1.0 / ns, 1.0 / (ns - 1))
                    js = pl.ds(pl.multiple_of(j * 8, 8), 8)
                    stats[0, cb, js, :] = shift + s1 * inv
                    stats[1, cb, js, :] = s2 - s1 * s1 * inv
                    return self.prev[-1]

            for cb in range(4):
                gbuf[0, cb, 0:HALO, :] = jnp.zeros((HALO, 128), f32)
                gbuf[1, cb, HALO:2 * HALO, :] = jnp.zeros((HALO, 128), f32)

            def p2(i, carry):
                a = stage_D1(i - 1)
                att_qk(i)
                stage_D2(i - 1, a)
                att_stats()
                att_pv(i, lambda c, prev: Conv(i - 1, c, ECH, prev).run(), PVU)
                return carry

            if ONLY in ('p1', 'p4', 'f0', 't0'):
                return
            if ONLY != 'e0':
                with jax.named_scope("p2loop"):
                    lax.fori_loop(1, P2END, p2, 0)
            if ONLY not in (None, 'e0'):
                return

            stage_D2(NT - 1, stage_D1(NT - 1, chained=False))
            for cb in range(4):
                Conv(NT - 1, cb, EPI_LAST).run()
                acc = Conv(NT, cb, 0).step(0)
                stats[0, cb, 8 * NT:8 * NT + 8, :] = acc
                stats[1, cb, 8 * NT:8 * NT + 8, :] = jnp.zeros((8, 128), f32)

        pl.run_scoped(attention, V((2, 4, TM + HALO, 128), f32))

        st0 = jnp.concatenate([stats[0, cb] for cb in range(4)], axis=1)
        st1 = jnp.concatenate([stats[1, cb] for cb in range(4)], axis=1)
        grow = lax.broadcasted_iota(jnp.int32, st0.shape, 0)
        cnt = jnp.where(grow < 8, TM // 8 - 1, jnp.where(grow < 8 * NT, TM // 8, 1)).astype(f32)
        mu = jnp.sum(cnt * st0, axis=0, keepdims=True) * (1.0 / N)
        dm = st0 - mu
        var = jnp.sum(st1 + cnt * dm * dm, axis=0, keepdims=True) * (1.0 / N)
        rsd = 0.5 * lax.rsqrt(var + EPS)

        def final(hnops, zops, obuf, osem):
            def ocopy(t, slot):
                return pltpu.make_async_copy(obuf.at[slot], out_hbm.at[pl.ds(pl.multiple_of(t * TM, 16), TM), :], osem.at[slot])

            def stage_F1(j, prev=None, chained=True):
                def zq(r0, n, hi):
                    rr = pl.ds(pl.multiple_of(j * TM + 8 + r0, 8), n)
                    d = jnp.concatenate([dc[2 * hi + t, rr, :] for t in range(2)], axis=1)
                    return (d - mu[:, hi * Dh:(hi + 1) * Dh]) * rsd[:, hi * Dh:(hi + 1) * Dh]
                if not chained:
                    return _a_ops(*[_hsilu(zq(r0, H, hi)) for r0 in (0, H) for hi in (0, 1)])
                for r in range(0, H, 16):
                    z = []
                    for r0 in (0, H):
                        for hi in (0, 1):
                            t = _hsilu(tie0(prev, zq(r0 + r, 16, hi)))
                            prev = t[:, :128] + t[:, 128:]
                            z.append(t)
                    for k, o in enumerate(_a_ops(*z)):
                        zops[k, r:r + 16, :] = o
                return prev

            def stage_F2(j, a=None):
                E = _smm((lambda k: zops[k]) if a is None else (lambda k: a[k]), lambda k: wp2[k])
                for q in QORD:
                    xr[qidx(j, q)] = xr[qidx(j, q)] + E[q]

            def stage_F3(j, slot, prev=None, nch=None):
                def st(k, r, n, v):
                    hnops[slot, k, r:r + n, :] = v
                return ln_chain(lambda r, n: xr[rows(j, r, n), :], st, prev, nch=nch or LCH4)[1]

            def stage_G2(i, U):
                d = ff_down(U)
                for q in DQORD:
                    xr[qidx(i, q)] = xr[qidx(i, q)] + d[q]

            def stage_Hh(j, chained=True):
                slot = j % 2
                if not chained:
                    obuf[slot, 0:H, :] = _ln(xr[rows(j), :]).astype(bf16)
                    obuf[slot, H:TM, :] = _ln(xr[rows(j, H), :]).astype(bf16)
                    return None
                heads = [None] * HCH
                for n, r in enumerate(range(0, TM, HG)):
                    y = _ln(tie0(heads[n % HCH], xr[rows(j, r, HG), :]))
                    prev = heads[n % HCH] = y[:, :128]
                    obuf[slot, r:r + HG, :] = y.astype(bf16)
                return prev

            if ONLY in ('p1', 'p2', 'f0'):
                return
            if ONLY in (None, 'e0'):
                stage_F2(0, stage_F1(0, chained=False))
                stage_F3(0, 0, stage_F1(1), nch=EPI_LN)

            def p4(i, carry):
                if ONLY is None:
                    @pl.when(i >= 3)
                    def _():
                        ocopy(i - 3, (i - 3) % 2).wait()
                stage_F2(i + 1)
                U = ff_up(hnops, i % 2)
                prev = stage_Hh(jnp.maximum(i - 1, 0))
                prev = stage_F3(i + 1, (i + 1) % 2, prev[0:16] if LINK & 1 else None)
                stage_F1(jnp.minimum(i + 2, NT - 1), prev if LINK & 2 else None)
                stage_G2(i, U)

                if ONLY is None:
                    @pl.when(i >= 1)
                    def _():
                        ocopy(i - 1, (i - 1) % 2).start()
                return carry

            if ONLY == 'e0':
                return
            if ONLY != 't0':
                with jax.named_scope("p4loop"):
                    lax.fori_loop(0, P4END, p4, 0)
            if ONLY not in (None, 't0'):
                return

            ocopy(NT - 4, (NT - 4) % 2).wait()
            ocopy(NT - 3, (NT - 3) % 2).wait()
            U = ff_up(hnops, (NT - 1) % 2)
            stage_Hh(NT - 2)
            d = ff_down(U)
            slot = (NT - 1) % 2
            last = [ocopy(NT - 2, (NT - 2) % 2)]
            for half in range(2):
                x4 = cat(*[xr[qidx(NT - 1, 2 * half + t)] + d[2 * half + t] for t in range(2)])
                obuf[slot, half * H:(half + 1) * H, :] = _ln(x4).astype(bf16)
                last.append(pltpu.make_async_copy(obuf.at[slot, half * H:(half + 1) * H, :],
                                                  out_hbm.at[pl.ds((NT - 1) * TM + half * H, H), :], osem.at[1 + half]))
                if half == 0:
                    last[0].start()
                last[-1].start()
            for c_ in last:
                c_.wait()

        pl.run_scoped(final, V((2, 7, H, Dh), bf16), V((7, H, Dh), bf16), V((2, TM, D), bf16),
                      pltpu.SemaphoreType.DMA((3,)))

    with jax.named_scope("back"):
        pl.run_scoped(back, V((4, N + 8, 128), f32), V((2, 4, 8 * NT + 8, 128), f32))


@jax.jit
def pallas_standalone__conformer_family_conformer__speech_kernel(
    x, w_ff1_a, w_ff1_b, w_q, w_k, w_v, w_o, w_pw1, dw, w_pw2, w_ff2_a, w_ff2_b):
    B, T, D = x.shape
    K = dw.shape[0]
    F = w_ff1_a.shape[1]
    N = B * T
    TM = 2 * H
    NT = N // TM
    TP = (T // 2 + 127) // 128 * 128
    Dh = D // 2
    kern = functools.partial(_kernel, B=B, T=T, D=D, K=K, F=F)
    hbm = pl.BlockSpec(memory_space=pl.ANY)
    V = pltpu.VMEM
    out = pl.pallas_call(
        kern,
        out_shape=jax.ShapeDtypeStruct((N, D), x.dtype),
        in_specs=[hbm] * 12,
        out_specs=hbm,
        scratch_shapes=[
            V((N, D), f32),
            V((NT, 7, H, Dh), bf16),
            V((B, 7, TP, Dh), bf16),
            V((B, 7, TP, Dh), bf16),
            V((7, Dh, F // 2), bf16),
            V((7, F // 2, Dh), bf16),
            V((2, 7, Dh, Dh), bf16),
            V((7, Dh, Dh), bf16),
            V((K, 4, 8, 128), f32),
            V((TP // W, 4, H, W), f32),
            V((2, H, 128), f32),
            V((2, TP // W - 1, 2, H, 128), f32),
            V((8 * ZN, 128), jnp.int32),
            V((8 * ZN, 128), jnp.int32),
            V((8 * PADK, 128), jnp.int32),
            pltpu.SemaphoreType.DMA(()),
        ],
        compiler_params=pltpu.CompilerParams(vmem_limit_bytes=VMEM_LIMIT),
    )(x.reshape(N, D), w_ff1_a, w_ff1_b, w_q, w_k, w_v, w_o, w_pw1, dw, w_pw2, w_ff2_a, w_ff2_b)
    return out.reshape(B, T, D)
```

```python
import functools
import jax
import jax.numpy as jnp
from jax import lax
import jax.experimental.pallas as pl
import jax.experimental.pallas.tpu as pltpu

H = 400
W = 512
EPS = 1e-5
LOG2E = 1.4426950408889634
NEG = -1e30
HALO = 16
UPO = (1, 2, 0, 5, 3, 4, 6)
DNO = (1, 3, 6, 0, 2, 4, 5)
DQORD = (2, 0, 1, 3)
PR = (40, 40, 40, 40)
P2G = 8
EPI_CH = 2
EPI_LAST = 0
EPI_LN = 9
LCH1 = 2
LCH4 = 2
HCH = 1
LCHD = 1
MIDUP = 2
BLINK = 2
HG = 32
LINK = 1
ZDMA = True
ZN = 1
PADK = 1
P1END = 10
P4END = 9
P2END = 10
PCHF = 8
PCH = 4
ECH = 1
PEEL_UNROLL = 2
PEEL_PCH = 16
PEEL_ROLL = False
PVU = 2
ONLY = None
VMEM_LIMIT = 127 * 1024 * 1024

bf16 = jnp.bfloat16
f32 = jnp.float32


def _ln(x):
    m = jnp.mean(x, axis=-1, keepdims=True)
    c = x - m
    v = jnp.mean(c * c, axis=-1, keepdims=True)
    return c * lax.rsqrt(v + EPS)


def _hsilu(h):
    return h * jnp.tanh(h) + h


def _hglu(a, b):
    return a * jnp.tanh(b) + a


def _dot(a, b):
    return jnp.dot(a, b, preferred_element_type=f32)


def _dot_nt(a, b):
    return lax.dot_general(a, b, (((1,), (1,)), ((), ())), preferred_element_type=f32)


def _a_sums(A11, A12, A21, A22):
    return [A11 + A22, A21 + A22, A11, A22, A11 + A12, A21 - A11, A12 - A22]


def _a_ops(*q):
    return [t.astype(bf16) for t in _a_sums(*q)]


def _b_ops(B11, B12, B21, B22):
    return [t.astype(bf16) for t in
            (B11 + B22, B11, B12 - B22, B21 - B11, B22, B11 + B12, B21 + B22)]


def _smm(a, w, order=UPO, dot=_dot, mid=None):
    M = [None] * 7
    for n, k in enumerate(order):
        if mid is not None and n == mid[0]:
            mid[1]()
        M[k] = dot(a(k), w(k))
    return (M[0] + M[3] - M[4] + M[6], M[2] + M[4], M[1] + M[3], M[0] - M[1] + M[2] + M[5])


def _cat(a, b):
    return jnp.concatenate([a, b], axis=1)


def _kernel(x_hbm, w1a_h, w1b_h, wq_h, wk_h, wv_h, wo_h, wp1_h, dw_h, wp2_h, w2a_h, w2b_h, out_hbm,
            xr, hops, kops, vops, wa, wb, wp1, wp2, dwb, sbuf, mbuf, cstat, zsrc, zref, padbuf, zsem, *, B, T, D, K, F):
    N = B * T
    TM = 2 * H
    NTB = T // TM
    NT = B * NTB
    TH = T // 2
    TP = kops.shape[2]
    NC = TP // W
    Dh = D // 2
    cat = _cat
    ident = tuple(range(7))

    if ZDMA:
        zsrc[...] = jnp.zeros_like(zsrc)
        zcopy = pltpu.make_async_copy(zsrc, zref, zsem)
        zcopy.start()
        zcopy.wait()
    else:
        zref[...] = jnp.zeros_like(zref)

    def tie(prev, v):
        if prev is None:
            return v
        never = jnp.tile(zref[0:8, :], (v.shape[0] // 8, 1)) != 0
        return jnp.where(never, prev, v)

    def tie0(prev, v):
        return v if prev is None else cat(tie(prev, v[:, :128]), v[:, 128:])

    def al16(v):
        return v if isinstance(v, int) else pl.multiple_of(v, 16)

    def rows(i, off=0, n=H):
        return pl.ds(al16(i * TM + off), n)

    def ln_chain(load, store=None, prev=None, chained=True, nch=1):
        if not chained:
            ht, hb = _ln(load(0, H)), _ln(load(H, H))
            ops = _a_ops(ht[:, :Dh], ht[:, Dh:], hb[:, :Dh], hb[:, Dh:])
            if store is not None:
                for k in range(7):
                    store(k, 0, H, ops[k])
            return ops, None
        outs = [[] for _ in range(7)]
        heads = [prev] * nch
        for n, r in enumerate(range(0, H, 16)):
            ht, hb = _ln(tie0(heads[n % nch], load(r, 16))), _ln(load(H + r, 16))
            s = _a_sums(ht[:, :Dh], ht[:, Dh:], hb[:, :Dh], hb[:, Dh:])
            prev = heads[n % nch] = s[0][:, :128]
            for k in range(7):
                o = s[k].astype(bf16)
                outs[k].append(o)
                if store is not None:
                    store(k, r, 16, o)
        return [jnp.concatenate(o, axis=0) for o in outs], prev

    def chained(fn, x, pr):
        if pr == 0:
            return fn(x)
        prev = None
        cols = []
        for t in range(x.shape[1] // 128):
            parts = []
            for r in range(0, x.shape[0], pr):
                prev = fn(tie(prev, x[r:r + pr, t * 128:(t + 1) * 128]))
                parts.append(prev)
            cols.append(jnp.concatenate(parts, axis=0))
        return jnp.concatenate(cols, axis=1)

    def build_b_ops(raw, dst, r0, nr, c0, n, scale, chained=True, prev=None):
        k = raw.shape[0] // 2
        nh = n // 2
        n_ = 0
        for r in range(0, nr, 16):
            for c in range(0, nh, 128):
                def blk(ro, co):
                    return raw[pl.ds(al16(ro + r0 + r), 16), c0 + co + c:c0 + co + c + 128].astype(f32) * scale
                B11, B12, B21, B22 = tie(prev if chained else None, blk(0, 0)), blk(0, nh), blk(k, 0), blk(k, nh)
                n_ += 1
                if n_ % BLINK == 0:
                    prev = jnp.broadcast_to(jnp.max((B11 + B12) + (B21 + B22), axis=-1, keepdims=True), (16, 128))
                ops = _b_ops(B11, B12, B21, B22)
                for i in range(7):
                    dst[i, pl.ds(al16(r0 + r), 16), c:c + 128] = ops[i]
        return prev

    QORD = (3, 2, 1, 0)

    def qidx(i, q):
        return rows(i, (q // 2) * H), slice((q % 2) * Dh, (q % 2 + 1) * Dh)

    def ff_up(hnops, slot, mid=None):
        C = _smm(lambda k: hnops[slot, k], lambda k: wa[k], UPO, mid=mid)
        return [chained(_hsilu, C[q], PR[q]) for q in range(4)]

    def ff_down(U):
        a = _a_ops(*U)
        return _smm(lambda k: a[k], lambda k: wb[k], DNO)

    def stage_C1(i, prev=None, chained=True):
        def st(k, r, n, v):
            hops[i, k, r:r + n, :] = v
        return ln_chain(lambda r, n: xr[rows(i, r, n), :], st, prev, chained=chained, nch=LCH1)

    def stage_C2(wkv, i, a):
        b = i // NTB
        r = pl.ds(pl.multiple_of((i % NTB) * H, 16), H)
        c = D ** -0.5 * LOG2E
        ktl, kth, kbl, kbh = [t * c for t in _smm(lambda k: a[k], lambda k: wkv[0, k])]
        ops = _b_ops(ktl, kbl, kth, kbh)
        for k in range(7):
            kops[b, k, r, :] = ops[k]
        vtl, vth, vbl, vbh = _smm(lambda k: a[k], lambda k: wkv[1, k])
        ops = _b_ops(vtl, vth, vbl, vbh)
        for k in range(7):
            vops[b, k, r, :] = ops[k]

    def att_qk(i, rolled=False):
        b = i // NTB

        def chunk(c, carry=None):
            static = isinstance(c, int)
            kr = slice(c * W, (c + 1) * W) if static else pl.ds(pl.multiple_of(c * W, W), W)
            s = list(_smm(lambda k: hops[i, k], lambda k: kops[b, k, kr, :], ident, _dot_nt))
            nv = TH - c * W
            for j in range(4):
                t = s[j]
                if not static:
                    t = jnp.where(lax.broadcasted_iota(jnp.int32, (H, W), 1) < nv, t, NEG)
                elif nv < W:
                    lo = nv // 128 * 128
                    col = lax.broadcasted_iota(jnp.int32, (H, W - lo), 1)
                    t = cat(t[:, :lo], jnp.where(col < nv - lo, t[:, lo:], NEG))
                sbuf[c, j] = t
            return carry

        if rolled:
            lax.fori_loop(0, NC, chunk, 0)
        else:
            for c in range(NC):
                chunk(c)

    def att_stats(nch0=None, nchf=None):
        nch0, nchf = nch0 or PCH, nchf or PCHF
        prev = [None] * nch0
        n = 0
        for c in range(NC):
            if c == NC - 1:
                prev = [prev[t % nch0] for t in range(nchf)]
            nch = len(prev)
            for r in range(0, H, P2G):
                for half in range(2):
                    rs = slice(r, r + P2G)
                    blocks = [sbuf[c, 2 * half + j, rs, t * 128:(t + 1) * 128]
                              for j in (0, 1) for t in range(W // 128)]
                    blocks[0] = tie(prev[n % nch], blocks[0])
                    m = jnp.broadcast_to(
                        jnp.max(functools.reduce(jnp.maximum, blocks), axis=-1, keepdims=True), (P2G, 128))
                    if c < NC - 1:
                        l = functools.reduce(jnp.add, [jnp.exp2(t - m) for t in blocks])
                        cstat[0, c, half, rs, :] = m
                        cstat[1, c, half, rs, :] = l
                        prev[n % nch] = l
                    else:
                        ms = [cstat[0, cc, half, rs, :] for cc in range(NC - 1)]
                        m = functools.reduce(jnp.maximum, ms + [m])
                        l = functools.reduce(jnp.add, [jnp.exp2(t - m) for t in blocks]
                                             + [cstat[1, cc, half, rs, :] * jnp.exp2(ms[cc] - m) for cc in range(NC - 1)])
                        mp = m + jnp.log2(jnp.sum(l, axis=-1, keepdims=True))
                        mbuf[half, rs, :] = mp
                        prev[n % nch] = mp
                    n += 1

    def att_pv(i, side, unroll=1):
        b = i // NTB

        def trip(c, prev):
            mt = jnp.concatenate([mbuf[0]] * (W // 128), axis=1)
            mb = jnp.concatenate([mbuf[1]] * (W // 128), axis=1)
            ms = (mt, mt, mb, mb)
            a = _a_ops(*[jnp.exp2(sbuf[c, j] - ms[j]) for j in range(4)])
            kr = pl.ds(pl.multiple_of(c * W, W), W)
            O = _smm(lambda k: a[k], lambda k: vops[b, k, kr, :])
            for q in QORD:
                xr[qidx(i, q)] = xr[qidx(i, q)] + O[q]
            return side(c, prev)

        def rolled(t, carry):
            prev = None
            for u in range(unroll):
                prev = trip(t * unroll + u, prev)
            return carry

        if unroll >= NC:
            rolled(0, 0)
        else:
            lax.fori_loop(0, NC // unroll, rolled, 0)

    def front(hnops, wkv, xbuf, rawa, rawb, rawq, rawp1, rawp2, rawdw, xsem, wsem):
        def xcopy(t, slot):
            return pltpu.make_async_copy(x_hbm.at[pl.ds(pl.multiple_of(t * TM, 16), TM), :], xbuf.at[slot], xsem.at[slot])

        cp = [
            pltpu.make_async_copy(wq_h, rawq.at[0], wsem.at[0]),
            pltpu.make_async_copy(wk_h, rawq.at[1], wsem.at[1]),
            pltpu.make_async_copy(wv_h, rawq.at[2], wsem.at[2]),
            pltpu.make_async_copy(wo_h, rawq.at[3], wsem.at[3]),
            pltpu.make_async_copy(w1a_h, rawa, wsem.at[4]),
            pltpu.make_async_copy(w1b_h, rawb, wsem.at[5]),
            pltpu.make_async_copy(dw_h, rawdw, wsem.at[6]),
            pltpu.make_async_copy(wp1_h, rawp1, wsem.at[7]),
            pltpu.make_async_copy(wp2_h, rawp2, wsem.at[8]),
            pltpu.make_async_copy(w2a_h, rawa, wsem.at[9]),
            pltpu.make_async_copy(w2b_h, rawb, wsem.at[10]),
        ]
        CQ, CK, CV, CO, C1A, C1B, CDW, CP1, CP2, C2A, C2B = range(11)

        def stage_A(t, slot, chained=True):
            xs = t % 3

            def st(k, r, n, v):
                hnops[slot, k, r:r + n, :] = v
            return ln_chain(lambda r, n: xbuf[xs, r:r + n, :].astype(f32), st, chained=chained, nch=LCH1)[1]

        def stage_B2(i, U):
            d = ff_down(U)
            xs = i % 3
            for q in DQORD:
                r0, c0 = (q // 2) * H, (q % 2) * Dh
                xr[qidx(i, q)] = xbuf[xs, r0:r0 + H, c0:c0 + Dh].astype(f32) + d[q]

        def p1(i, carry, dma=True):
            if dma:
                @pl.when(i + 2 < NT)
                def _():
                    xcopy(i + 2, (i + 2) % 3).start()

                @pl.when(i + 1 < NT)
                def _():
                    xcopy(i + 1, (i + 1) % 3).wait()
            U = ff_up(hnops, i % 2)
            prev = stage_A(jnp.minimum(i + 1, NT - 1), (i + 1) % 2)
            hq, _ = stage_C1(i - 1, prev)
            stage_B2(i, U)
            stage_C2(wkv, i - 1, hq)
            return carry

        if ONLY == 'p1':
            lax.fori_loop(1, NT, lambda i, c: p1(i, c, False), 0)
            return
        if ONLY not in (None, 'f0'):
            return
        cp[C1A].start()
        xcopy(0, 0).start()
        for b in range(B):
            for k in range(7):
                kops[b, k, TH:, :] = jnp.zeros((TP - TH, Dh), bf16)
                vops[b, k, TH:, :] = jnp.zeros((TP - TH, Dh), bf16)
        xcopy(0, 0).wait()
        cp[C1B].start()
        stage_A(0, 0, chained=False)
        cp[C1A].wait()
        build_b_ops(rawa, wa, 0, Dh, 0, F, 0.5, chained=False)
        early = (cp[CQ], cp[CK], cp[CV], cp[CO], xcopy(1, 1), cp[CDW])

        def mid_up():
            cp[C1B].wait()
            for c_ in early:
                c_.start()
            build_b_ops(rawb, wb, 0, F // 2, 0, D, 0.5)

        U = ff_up(hnops, 0, mid=(MIDUP, mid_up))
        for c_ in early:
            c_.wait()
        for c_ in (xcopy(2, 2), cp[CP1], cp[CP2]):
            c_.start()
        wf = _dot_nt(rawq[1], rawq[0])
        ops = _b_ops(wf[:Dh, :Dh], wf[:Dh, Dh:], wf[Dh:, :Dh], wf[Dh:, Dh:])
        for k in range(7):
            wkv[0, k] = ops[k]
        wf = _dot(rawq[2], rawq[3])
        ops = _b_ops(wf[:Dh, :Dh], wf[:Dh, Dh:], wf[Dh:, :Dh], wf[Dh:, Dh:])
        for k in range(7):
            wkv[1, k] = ops[k]
        stage_A(1, 1)
        stage_B2(0, U)
        dwv = rawdw[...].astype(f32)
        for k in range(K):
            for cb in range(4):
                dwb[k, cb] = jnp.broadcast_to(dwv[k:k + 1, cb * 128:(cb + 1) * 128], (8, 128))
        cp[C2A].start()
        cp[C2B].start()

        if ONLY == 'f0':
            for c_ in (xcopy(2, 2), cp[CP1], cp[CP2], cp[C2A], cp[C2B]):
                c_.wait()
            return
        with jax.named_scope("p1loop"):
            lax.fori_loop(1, P1END, p1, 0)

        cp[CP1].wait()
        cp[CP2].wait()
        cp[C2A].wait()
        cp[C2B].wait()

        def wops(c, prev):
            q = Dh // NC
            r0 = c * q if isinstance(c, int) else pl.multiple_of(c * q, 16)
            r1 = c * (F // 2 // NC) if isinstance(c, int) else pl.multiple_of(c * (F // 2 // NC), 16)
            prev = build_b_ops(rawp1, wp1.at[0], r0, q, 0, D, 0.5, prev=prev)
            prev = build_b_ops(rawp1, wp1.at[1], r0, q, D, D, 0.5, prev=prev)
            prev = build_b_ops(rawp2, wp2, r0, q, 0, D, 1.0, prev=prev)
            prev = build_b_ops(rawa, wa, r0, q, 0, F, 0.5, prev=prev)
            return build_b_ops(rawb, wb, r1, F // 2 // NC, 0, D, 0.5, prev=prev)

        with jax.named_scope("p2peel"):
            if PEEL_ROLL:
                att_qk(0, rolled=True)
                hq, _ = stage_C1(NT - 1, chained=False)
                stage_C2(wkv, NT - 1, hq)
                att_stats(PEEL_PCH, PEEL_PCH)
            else:
                hq, _ = stage_C1(NT - 1)
                att_qk(0)
                stage_C2(wkv, NT - 1, hq)
                att_stats()
            att_pv(0, wops, unroll=PEEL_UNROLL)

    V = pltpu.VMEM
    with jax.named_scope("front"):
        pl.run_scoped(front, V((2, 7, H, Dh), bf16), V((2, 7, Dh, Dh), bf16), V((3, TM, D), bf16), V((D, F), bf16), V((F, D), bf16), V((4, D, D), bf16),
                      V((D, 2 * D), bf16), V((D, D), bf16), V((K, D), bf16),
                      pltpu.SemaphoreType.DMA((3,)), pltpu.SemaphoreType.DMA((11,)))

    def back(dc, stats):
        def attention(gbuf):
            def stage_D1(j, chained=True):
                return ln_chain(lambda r, n: xr[rows(j, r, n), :], chained=chained, nch=LCHD)[0]

            def stage_D2(j, a):
                ga = _smm(lambda k: a[k], lambda k: wp1[0, k])
                gb_ = _smm(lambda k: a[k], lambda k: wp1[1, k])
                g = [_hglu(u, v) for u, v in zip(ga, gb_)]
                for q in QORD:
                    for t in range(2):
                        cb = 2 * (q % 2) + t
                        v = g[q][:, t * 128:(t + 1) * 128]
                        r0 = HALO + (q // 2) * H
                        gbuf[j % 2, cb, r0:r0 + H, :] = v
                        if q // 2 == 1:
                            gbuf[(j + 1) % 2, cb, 0:HALO, :] = v[H - HALO:H]

            class Conv:
                def __init__(self, j, cb, nch, head=None):
                    self.j, self.cb, self.nch = j, cb, nch
                    self.w = [dwb[k, cb] for k in range(K)]
                    self.prev = [head] * max(nch, 1)
                    self.shift = self.s1 = self.s2 = None
                    first = j % NTB == 0
                    self.lim = (jnp.where(first, HALO, 2 * HALO), jnp.where(first, HALO, 0))

                def step(self, n):
                    j, cb = self.j, self.cb
                    sub = lax.broadcasted_iota(jnp.int32, (8, 128), 0)
                    acc = None
                    for k in range(K):
                        i0 = 8 * n + k + 1
                        t = gbuf[j % 2, cb, pl.ds(i0, 8), :]
                        if n == 0 and i0 + 7 >= HALO:
                            t = jnp.where(sub + i0 < self.lim[0], t, 0.0)
                        if n == 1 and i0 < HALO:
                            t = jnp.where(sub + i0 >= self.lim[1], t, 0.0)
                        t = t * self.w[k]
                        if acc is None:
                            acc = tie(self.prev[n % self.nch], t) if self.nch else t
                        else:
                            acc = acc + t
                    dc[cb, pl.ds(pl.multiple_of(j * TM + 8 * n, 8), 8), :] = acc
                    if self.nch:
                        self.prev[n % self.nch] = acc
                    return acc

                def run(self):
                    j, cb = self.j, self.cb
                    ns = TM // 8
                    shift = self.step(1)
                    s1 = s2 = None
                    for n in [0] + list(range(2, ns)):
                        d = self.step(n) - shift
                        if n == 0:
                            d = jnp.where(j > 0, d, 0.0)
                        s1 = d if s1 is None else s1 + d
                        s2 = d * d if s2 is None else s2 + d * d
                    inv = jnp.where(j > 0, 1.0 / ns, 1.0 / (ns - 1))
                    js = pl.ds(pl.multiple_of(j * 8, 8), 8)
                    stats[0, cb, js, :] = shift + s1 * inv
                    stats[1, cb, js, :] = s2 - s1 * s1 * inv
                    return self.prev[-1]

            for cb in range(4):
                gbuf[0, cb, 0:HALO, :] = jnp.zeros((HALO, 128), f32)
                gbuf[1, cb, HALO:2 * HALO, :] = jnp.zeros((HALO, 128), f32)

            def p2(i, carry):
                a = stage_D1(i - 1)
                att_qk(i)
                stage_D2(i - 1, a)
                att_stats()
                att_pv(i, lambda c, prev: Conv(i - 1, c, ECH, prev).run(), PVU)
                return carry

            if ONLY in ('p1', 'p4', 'f0', 't0'):
                return
            if ONLY != 'e0':
                with jax.named_scope("p2loop"):
                    lax.fori_loop(1, P2END, p2, 0)
            if ONLY not in (None, 'e0'):
                return

            stage_D2(NT - 1, stage_D1(NT - 1, chained=False))
            for cb in range(4):
                Conv(NT - 1, cb, EPI_LAST).run()
                acc = Conv(NT, cb, 0).step(0)
                stats[0, cb, 8 * NT:8 * NT + 8, :] = acc
                stats[1, cb, 8 * NT:8 * NT + 8, :] = jnp.zeros((8, 128), f32)

        pl.run_scoped(attention, V((2, 4, TM + HALO, 128), f32))

        st0 = jnp.concatenate([stats[0, cb] for cb in range(4)], axis=1)
        st1 = jnp.concatenate([stats[1, cb] for cb in range(4)], axis=1)
        grow = lax.broadcasted_iota(jnp.int32, st0.shape, 0)
        cnt = jnp.where(grow < 8, TM // 8 - 1, jnp.where(grow < 8 * NT, TM // 8, 1)).astype(f32)
        mu = jnp.sum(cnt * st0, axis=0, keepdims=True) * (1.0 / N)
        dm = st0 - mu
        var = jnp.sum(st1 + cnt * dm * dm, axis=0, keepdims=True) * (1.0 / N)
        rsd = 0.5 * lax.rsqrt(var + EPS)

        def final(hnops, zops, obuf, osem):
            def ocopy(t, slot):
                return pltpu.make_async_copy(obuf.at[slot], out_hbm.at[pl.ds(pl.multiple_of(t * TM, 16), TM), :], osem.at[slot])

            def stage_F1(j, prev=None, chained=True):
                def zq(r0, n, hi):
                    rr = pl.ds(pl.multiple_of(j * TM + 8 + r0, 8), n)
                    d = jnp.concatenate([dc[2 * hi + t, rr, :] for t in range(2)], axis=1)
                    return (d - mu[:, hi * Dh:(hi + 1) * Dh]) * rsd[:, hi * Dh:(hi + 1) * Dh]
                if not chained:
                    return _a_ops(*[_hsilu(zq(r0, H, hi)) for r0 in (0, H) for hi in (0, 1)])
                for r in range(0, H, 16):
                    z = []
                    for r0 in (0, H):
                        for hi in (0, 1):
                            t = _hsilu(tie0(prev, zq(r0 + r, 16, hi)))
                            prev = t[:, :128] + t[:, 128:]
                            z.append(t)
                    for k, o in enumerate(_a_ops(*z)):
                        zops[k, r:r + 16, :] = o
                return prev

            def stage_F2(j, a=None):
                E = _smm((lambda k: zops[k]) if a is None else (lambda k: a[k]), lambda k: wp2[k])
                for q in QORD:
                    xr[qidx(j, q)] = xr[qidx(j, q)] + E[q]

            def stage_F3(j, slot, prev=None, nch=None):
                def st(k, r, n, v):
                    hnops[slot, k, r:r + n, :] = v
                return ln_chain(lambda r, n: xr[rows(j, r, n), :], st, prev, nch=nch or LCH4)[1]

            def stage_G2(i, U):
                d = ff_down(U)
                for q in DQORD:
                    xr[qidx(i, q)] = xr[qidx(i, q)] + d[q]

            def stage_Hh(j, chained=True):
                slot = j % 2
                if not chained:
                    obuf[slot, 0:H, :] = _ln(xr[rows(j), :]).astype(bf16)
                    obuf[slot, H:TM, :] = _ln(xr[rows(j, H), :]).astype(bf16)
                    return None
                heads = [None] * HCH
                for n, r in enumerate(range(0, TM, HG)):
                    y = _ln(tie0(heads[n % HCH], xr[rows(j, r, HG), :]))
                    prev = heads[n % HCH] = y[:, :128]
                    obuf[slot, r:r + HG, :] = y.astype(bf16)
                return prev

            if ONLY in ('p1', 'p2', 'f0'):
                return
            if ONLY in (None, 'e0'):
                stage_F2(0, stage_F1(0, chained=False))
                stage_F3(0, 0, stage_F1(1), nch=EPI_LN)

            def p4(i, carry):
                if ONLY is None:
                    @pl.when(i >= 3)
                    def _():
                        ocopy(i - 3, (i - 3) % 2).wait()
                stage_F2(i + 1)
                U = ff_up(hnops, i % 2)
                prev = stage_Hh(jnp.maximum(i - 1, 0))
                prev = stage_F3(i + 1, (i + 1) % 2, prev[0:16] if LINK & 1 else None)
                stage_F1(jnp.minimum(i + 2, NT - 1), prev if LINK & 2 else None)
                stage_G2(i, U)

                if ONLY is None:
                    @pl.when(i >= 1)
                    def _():
                        ocopy(i - 1, (i - 1) % 2).start()
                return carry

            if ONLY == 'e0':
                return
            if ONLY != 't0':
                with jax.named_scope("p4loop"):
                    lax.fori_loop(0, P4END, p4, 0)
            if ONLY not in (None, 't0'):
                return

            ocopy(NT - 4, (NT - 4) % 2).wait()
            ocopy(NT - 3, (NT - 3) % 2).wait()
            U = ff_up(hnops, (NT - 1) % 2)
            stage_Hh(NT - 2)
            d = ff_down(U)
            slot = (NT - 1) % 2
            last = [ocopy(NT - 2, (NT - 2) % 2)]
            for half in range(2):
                x4 = cat(*[xr[qidx(NT - 1, 2 * half + t)] + d[2 * half + t] for t in range(2)])
                obuf[slot, half * H:(half + 1) * H, :] = _ln(x4).astype(bf16)
                last.append(pltpu.make_async_copy(obuf.at[slot, half * H:(half + 1) * H, :],
                                                  out_hbm.at[pl.ds((NT - 1) * TM + half * H, H), :], osem.at[1 + half]))
                if half == 0:
                    last[0].start()
                last[-1].start()
            for c_ in last:
                c_.wait()

        pl.run_scoped(final, V((2, 7, H, Dh), bf16), V((7, H, Dh), bf16), V((2, TM, D), bf16),
                      pltpu.SemaphoreType.DMA((3,)))

    with jax.named_scope("back"):
        pl.run_scoped(back, V((4, N + 8, 128), f32), V((2, 4, 8 * NT + 8, 128), f32))


@jax.jit
def pallas_standalone__conformer_family_conformer__speech_kernel(
    x, w_ff1_a, w_ff1_b, w_q, w_k, w_v, w_o, w_pw1, dw, w_pw2, w_ff2_a, w_ff2_b):
    B, T, D = x.shape
    K = dw.shape[0]
    F = w_ff1_a.shape[1]
    N = B * T
    TM = 2 * H
    NT = N // TM
    TP = (T // 2 + 127) // 128 * 128
    Dh = D // 2
    kern = functools.partial(_kernel, B=B, T=T, D=D, K=K, F=F)
    hbm = pl.BlockSpec(memory_space=pl.ANY)
    V = pltpu.VMEM
    out = pl.pallas_call(
        kern,
        out_shape=jax.ShapeDtypeStruct((N, D), x.dtype),
        in_specs=[hbm] * 12,
        out_specs=hbm,
        scratch_shapes=[
            V((N, D), f32),
            V((NT, 7, H, Dh), bf16),
            V((B, 7, TP, Dh), bf16),
            V((B, 7, TP, Dh), bf16),
            V((7, Dh, F // 2), bf16),
            V((7, F // 2, Dh), bf16),
            V((2, 7, Dh, Dh), bf16),
            V((7, Dh, Dh), bf16),
            V((K, 4, 8, 128), f32),
            V((TP // W, 4, H, W), f32),
            V((2, H, 128), f32),
            V((2, TP // W - 1, 2, H, 128), f32),
            V((8 * ZN, 128), jnp.int32),
            V((8 * ZN, 128), jnp.int32),
            V((8 * PADK, 128), jnp.int32),
            pltpu.SemaphoreType.DMA(()),
        ],
        compiler_params=pltpu.CompilerParams(vmem_limit_bytes=VMEM_LIMIT),
    )(x.reshape(N, D), w_ff1_a, w_ff1_b, w_q, w_k, w_v, w_o, w_pw1, dw, w_pw2, w_ff2_a, w_ff2_b)
    return out.reshape(B, T, D)
```

```python
import functools
import jax
import jax.numpy as jnp
from jax import lax
import jax.experimental.pallas as pl
import jax.experimental.pallas.tpu as pltpu

H = 400
W = 512
EPS = 1e-5
LOG2E = 1.4426950408889634
NEG = -1e30
HALO = 16
UPO = (1, 2, 0, 5, 3, 4, 6)
DNO = (1, 3, 6, 0, 2, 4, 5)
DQORD = (2, 0, 1, 3)
PR = (40, 40, 40, 40)
P2G = 8
EPI_CH = 2
EPI_LAST = 0
EPI_LN = 9
LCH1 = 2
LCH4 = 2
HCH = 1
LCHD = 1
MIDUP = 2
BLINK = 2
HG = 32
LINK = 1
PADS = (0, 0, 2, 0, 3, 0)
P1END = 10
P4END = 9
P2END = 10
PCHF = 8
PCH = 4
ECH = 1
PEEL_UNROLL = 2
PEEL_PCH = 16
PEEL_ROLL = False
PVU = 2
ONLY = None
VMEM_LIMIT = 127 * 1024 * 1024

bf16 = jnp.bfloat16
f32 = jnp.float32


def _ln(x):
    m = jnp.mean(x, axis=-1, keepdims=True)
    c = x - m
    v = jnp.mean(c * c, axis=-1, keepdims=True)
    return c * lax.rsqrt(v + EPS)


def _hsilu(h):
    return h * jnp.tanh(h) + h


def _hglu(a, b):
    return a * jnp.tanh(b) + a


def _dot(a, b):
    return jnp.dot(a, b, preferred_element_type=f32)


def _dot_nt(a, b):
    return lax.dot_general(a, b, (((1,), (1,)), ((), ())), preferred_element_type=f32)


def _a_sums(A11, A12, A21, A22):
    return [A11 + A22, A21 + A22, A11, A22, A11 + A12, A21 - A11, A12 - A22]


def _a_ops(*q):
    return [t.astype(bf16) for t in _a_sums(*q)]


def _b_ops(B11, B12, B21, B22):
    return [t.astype(bf16) for t in
            (B11 + B22, B11, B12 - B22, B21 - B11, B22, B11 + B12, B21 + B22)]


def _smm(a, w, order=UPO, dot=_dot, mid=None):
    M = [None] * 7
    for n, k in enumerate(order):
        if mid is not None and n == mid[0]:
            mid[1]()
        M[k] = dot(a(k), w(k))
    return (M[0] + M[3] - M[4] + M[6], M[2] + M[4], M[1] + M[3], M[0] - M[1] + M[2] + M[5])


def _cat(a, b):
    return jnp.concatenate([a, b], axis=1)


def _kernel(x_hbm, w1a_h, w1b_h, wq_h, wk_h, wv_h, wo_h, wp1_h, dw_h, wp2_h, w2a_h, w2b_h, out_hbm,
            xr, hops, kops, vops, wa, wb, wp1, wp2, dwb, sbuf, mbuf, cstat, zsrc, zref, zsem, *, B, T, D, K, F):
    N = B * T
    TM = 2 * H
    NTB = T // TM
    NT = B * NTB
    TH = T // 2
    TP = kops.shape[2]
    NC = TP // W
    Dh = D // 2
    cat = _cat
    ident = tuple(range(7))

    def fill_zref(src):
        src[0:8, :] = jnp.zeros((8, 128), jnp.int32)
        zcopy = pltpu.make_async_copy(src.at[0:8, :], zref, zsem)
        zcopy.start()
        zcopy.wait()

    fill_zref(zsrc)

    def tie(prev, v):
        if prev is None:
            return v
        never = jnp.tile(zref[0:8, :], (v.shape[0] // 8, 1)) != 0
        return jnp.where(never, prev, v)

    def tie0(prev, v):
        return v if prev is None else cat(tie(prev, v[:, :128]), v[:, 128:])

    def al16(v):
        return v if isinstance(v, int) else pl.multiple_of(v, 16)

    def rows(i, off=0, n=H):
        return pl.ds(al16(i * TM + off), n)

    def ln_chain(load, store=None, prev=None, chained=True, nch=1):
        if not chained:
            ht, hb = _ln(load(0, H)), _ln(load(H, H))
            ops = _a_ops(ht[:, :Dh], ht[:, Dh:], hb[:, :Dh], hb[:, Dh:])
            if store is not None:
                for k in range(7):
                    store(k, 0, H, ops[k])
            return ops, None
        outs = [[] for _ in range(7)]
        heads = [prev] * nch
        for n, r in enumerate(range(0, H, 16)):
            ht, hb = _ln(tie0(heads[n % nch], load(r, 16))), _ln(load(H + r, 16))
            s = _a_sums(ht[:, :Dh], ht[:, Dh:], hb[:, :Dh], hb[:, Dh:])
            prev = heads[n % nch] = s[0][:, :128]
            for k in range(7):
                o = s[k].astype(bf16)
                outs[k].append(o)
                if store is not None:
                    store(k, r, 16, o)
        return [jnp.concatenate(o, axis=0) for o in outs], prev

    def chained(fn, x, pr):
        if pr == 0:
            return fn(x)
        prev = None
        cols = []
        for t in range(x.shape[1] // 128):
            parts = []
            for r in range(0, x.shape[0], pr):
                prev = fn(tie(prev, x[r:r + pr, t * 128:(t + 1) * 128]))
                parts.append(prev)
            cols.append(jnp.concatenate(parts, axis=0))
        return jnp.concatenate(cols, axis=1)

    def build_b_ops(raw, dst, r0, nr, c0, n, scale, chained=True, prev=None):
        k = raw.shape[0] // 2
        nh = n // 2
        n_ = 0
        for r in range(0, nr, 16):
            for c in range(0, nh, 128):
                def blk(ro, co):
                    return raw[pl.ds(al16(ro + r0 + r), 16), c0 + co + c:c0 + co + c + 128].astype(f32) * scale
                B11, B12, B21, B22 = tie(prev if chained else None, blk(0, 0)), blk(0, nh), blk(k, 0), blk(k, nh)
                n_ += 1
                if n_ % BLINK == 0:
                    prev = jnp.broadcast_to(jnp.max((B11 + B12) + (B21 + B22), axis=-1, keepdims=True), (16, 128))
                ops = _b_ops(B11, B12, B21, B22)
                for i in range(7):
                    dst[i, pl.ds(al16(r0 + r), 16), c:c + 128] = ops[i]
        return prev

    QORD = (3, 2, 1, 0)

    def qidx(i, q):
        return rows(i, (q // 2) * H), slice((q % 2) * Dh, (q % 2 + 1) * Dh)

    def ff_up(hnops, slot, mid=None):
        C = _smm(lambda k: hnops[slot, k], lambda k: wa[k], UPO, mid=mid)
        return [chained(_hsilu, C[q], PR[q]) for q in range(4)]

    def ff_down(U):
        a = _a_ops(*U)
        return _smm(lambda k: a[k], lambda k: wb[k], DNO)

    def stage_C1(i, prev=None, chained=True):
        def st(k, r, n, v):
            hops[i, k, r:r + n, :] = v
        return ln_chain(lambda r, n: xr[rows(i, r, n), :], st, prev, chained=chained, nch=LCH1)

    def stage_C2(wkv, i, a):
        b = i // NTB
        r = pl.ds(pl.multiple_of((i % NTB) * H, 16), H)
        c = D ** -0.5 * LOG2E
        ktl, kth, kbl, kbh = [t * c for t in _smm(lambda k: a[k], lambda k: wkv[0, k])]
        ops = _b_ops(ktl, kbl, kth, kbh)
        for k in range(7):
            kops[b, k, r, :] = ops[k]
        vtl, vth, vbl, vbh = _smm(lambda k: a[k], lambda k: wkv[1, k])
        ops = _b_ops(vtl, vth, vbl, vbh)
        for k in range(7):
            vops[b, k, r, :] = ops[k]

    def att_qk(i, rolled=False):
        b = i // NTB

        def chunk(c, carry=None):
            static = isinstance(c, int)
            kr = slice(c * W, (c + 1) * W) if static else pl.ds(pl.multiple_of(c * W, W), W)
            s = list(_smm(lambda k: hops[i, k], lambda k: kops[b, k, kr, :], ident, _dot_nt))
            nv = TH - c * W
            for j in range(4):
                t = s[j]
                if not static:
                    t = jnp.where(lax.broadcasted_iota(jnp.int32, (H, W), 1) < nv, t, NEG)
                elif nv < W:
                    lo = nv // 128 * 128
                    col = lax.broadcasted_iota(jnp.int32, (H, W - lo), 1)
                    t = cat(t[:, :lo], jnp.where(col < nv - lo, t[:, lo:], NEG))
                sbuf[c, j] = t
            return carry

        if rolled:
            lax.fori_loop(0, NC, chunk, 0)
        else:
            for c in range(NC):
                chunk(c)

    def att_stats(nch0=None, nchf=None):
        nch0, nchf = nch0 or PCH, nchf or PCHF
        prev = [None] * nch0
        n = 0
        for c in range(NC):
            if c == NC - 1:
                prev = [prev[t % nch0] for t in range(nchf)]
            nch = len(prev)
            for r in range(0, H, P2G):
                for half in range(2):
                    rs = slice(r, r + P2G)
                    blocks = [sbuf[c, 2 * half + j, rs, t * 128:(t + 1) * 128]
                              for j in (0, 1) for t in range(W // 128)]
                    blocks[0] = tie(prev[n % nch], blocks[0])
                    m = jnp.broadcast_to(
                        jnp.max(functools.reduce(jnp.maximum, blocks), axis=-1, keepdims=True), (P2G, 128))
                    if c < NC - 1:
                        l = functools.reduce(jnp.add, [jnp.exp2(t - m) for t in blocks])
                        cstat[0, c, half, rs, :] = m
                        cstat[1, c, half, rs, :] = l
                        prev[n % nch] = l
                    else:
                        ms = [cstat[0, cc, half, rs, :] for cc in range(NC - 1)]
                        m = functools.reduce(jnp.maximum, ms + [m])
                        l = functools.reduce(jnp.add, [jnp.exp2(t - m) for t in blocks]
                                             + [cstat[1, cc, half, rs, :] * jnp.exp2(ms[cc] - m) for cc in range(NC - 1)])
                        mp = m + jnp.log2(jnp.sum(l, axis=-1, keepdims=True))
                        mbuf[half, rs, :] = mp
                        prev[n % nch] = mp
                    n += 1

    def att_pv(i, side, unroll=1):
        b = i // NTB

        def trip(c, prev):
            mt = jnp.concatenate([mbuf[0]] * (W // 128), axis=1)
            mb = jnp.concatenate([mbuf[1]] * (W // 128), axis=1)
            ms = (mt, mt, mb, mb)
            a = _a_ops(*[jnp.exp2(sbuf[c, j] - ms[j]) for j in range(4)])
            kr = pl.ds(pl.multiple_of(c * W, W), W)
            O = _smm(lambda k: a[k], lambda k: vops[b, k, kr, :])
            for q in QORD:
                xr[qidx(i, q)] = xr[qidx(i, q)] + O[q]
            return side(c, prev)

        def rolled(t, carry):
            prev = None
            for u in range(unroll):
                prev = trip(t * unroll + u, prev)
            return carry

        if unroll >= NC:
            rolled(0, 0)
        else:
            lax.fori_loop(0, NC // unroll, rolled, 0)

    def front(padF, hnops, wkv, xbuf, rawa, rawb, rawq, rawp1, rawp2, rawdw, xsem, wsem):
        fill_zref(padF)

        def xcopy(t, slot):
            return pltpu.make_async_copy(x_hbm.at[pl.ds(pl.multiple_of(t * TM, 16), TM), :], xbuf.at[slot], xsem.at[slot])

        cp = [
            pltpu.make_async_copy(wq_h, rawq.at[0], wsem.at[0]),
            pltpu.make_async_copy(wk_h, rawq.at[1], wsem.at[1]),
            pltpu.make_async_copy(wv_h, rawq.at[2], wsem.at[2]),
            pltpu.make_async_copy(wo_h, rawq.at[3], wsem.at[3]),
            pltpu.make_async_copy(w1a_h, rawa, wsem.at[4]),
            pltpu.make_async_copy(w1b_h, rawb, wsem.at[5]),
            pltpu.make_async_copy(dw_h, rawdw, wsem.at[6]),
            pltpu.make_async_copy(wp1_h, rawp1, wsem.at[7]),
            pltpu.make_async_copy(wp2_h, rawp2, wsem.at[8]),
            pltpu.make_async_copy(w2a_h, rawa, wsem.at[9]),
            pltpu.make_async_copy(w2b_h, rawb, wsem.at[10]),
        ]
        CQ, CK, CV, CO, C1A, C1B, CDW, CP1, CP2, C2A, C2B = range(11)

        def stage_A(t, slot, chained=True):
            xs = t % 3

            def st(k, r, n, v):
                hnops[slot, k, r:r + n, :] = v
            return ln_chain(lambda r, n: xbuf[xs, r:r + n, :].astype(f32), st, chained=chained, nch=LCH1)[1]

        def stage_B2(i, U):
            d = ff_down(U)
            xs = i % 3
            for q in DQORD:
                r0, c0 = (q // 2) * H, (q % 2) * Dh
                xr[qidx(i, q)] = xbuf[xs, r0:r0 + H, c0:c0 + Dh].astype(f32) + d[q]

        def p1(i, carry, dma=True):
            if dma:
                @pl.when(i + 2 < NT)
                def _():
                    xcopy(i + 2, (i + 2) % 3).start()

                @pl.when(i + 1 < NT)
                def _():
                    xcopy(i + 1, (i + 1) % 3).wait()
            U = ff_up(hnops, i % 2)
            prev = stage_A(jnp.minimum(i + 1, NT - 1), (i + 1) % 2)
            hq, _ = stage_C1(i - 1, prev)
            stage_B2(i, U)
            stage_C2(wkv, i - 1, hq)
            return carry

        if ONLY == 'p1':
            lax.fori_loop(1, NT, lambda i, c: p1(i, c, False), 0)
            return
        if ONLY not in (None, 'f0'):
            return
        cp[C1A].start()
        xcopy(0, 0).start()
        for b in range(B):
            for k in range(7):
                kops[b, k, TH:, :] = jnp.zeros((TP - TH, Dh), bf16)
                vops[b, k, TH:, :] = jnp.zeros((TP - TH, Dh), bf16)
        xcopy(0, 0).wait()
        cp[C1B].start()
        stage_A(0, 0, chained=False)
        cp[C1A].wait()
        build_b_ops(rawa, wa, 0, Dh, 0, F, 0.5, chained=False)
        early = (cp[CQ], cp[CK], cp[CV], cp[CO], xcopy(1, 1), cp[CDW])

        def mid_up():
            cp[C1B].wait()
            for c_ in early:
                c_.start()
            build_b_ops(rawb, wb, 0, F // 2, 0, D, 0.5)

        U = ff_up(hnops, 0, mid=(MIDUP, mid_up))
        for c_ in early:
            c_.wait()
        for c_ in (xcopy(2, 2), cp[CP1], cp[CP2]):
            c_.start()
        wf = _dot_nt(rawq[1], rawq[0])
        ops = _b_ops(wf[:Dh, :Dh], wf[:Dh, Dh:], wf[Dh:, :Dh], wf[Dh:, Dh:])
        for k in range(7):
            wkv[0, k] = ops[k]
        wf = _dot(rawq[2], rawq[3])
        ops = _b_ops(wf[:Dh, :Dh], wf[:Dh, Dh:], wf[Dh:, :Dh], wf[Dh:, Dh:])
        for k in range(7):
            wkv[1, k] = ops[k]
        stage_A(1, 1)
        stage_B2(0, U)
        dwv = rawdw[...].astype(f32)
        for k in range(K):
            for cb in range(4):
                dwb[k, cb] = jnp.broadcast_to(dwv[k:k + 1, cb * 128:(cb + 1) * 128], (8, 128))
        cp[C2A].start()
        cp[C2B].start()

        if ONLY == 'f0':
            for c_ in (xcopy(2, 2), cp[CP1], cp[CP2], cp[C2A], cp[C2B]):
                c_.wait()
            return
        with jax.named_scope("p1loop"):
            lax.fori_loop(1, P1END, p1, 0)

        cp[CP1].wait()
        cp[CP2].wait()
        cp[C2A].wait()
        cp[C2B].wait()

        def wops(c, prev):
            q = Dh // NC
            r0 = c * q if isinstance(c, int) else pl.multiple_of(c * q, 16)
            r1 = c * (F // 2 // NC) if isinstance(c, int) else pl.multiple_of(c * (F // 2 // NC), 16)
            prev = build_b_ops(rawp1, wp1.at[0], r0, q, 0, D, 0.5, prev=prev)
            prev = build_b_ops(rawp1, wp1.at[1], r0, q, D, D, 0.5, prev=prev)
            prev = build_b_ops(rawp2, wp2, r0, q, 0, D, 1.0, prev=prev)
            prev = build_b_ops(rawa, wa, r0, q, 0, F, 0.5, prev=prev)
            return build_b_ops(rawb, wb, r1, F // 2 // NC, 0, D, 0.5, prev=prev)

        with jax.named_scope("p2peel"):
            if PEEL_ROLL:
                att_qk(0, rolled=True)
                hq, _ = stage_C1(NT - 1, chained=False)
                stage_C2(wkv, NT - 1, hq)
                att_stats(PEEL_PCH, PEEL_PCH)
            else:
                hq, _ = stage_C1(NT - 1)
                att_qk(0)
                stage_C2(wkv, NT - 1, hq)
                att_stats()
            att_pv(0, wops, unroll=PEEL_UNROLL)

    V = pltpu.VMEM
    PADT = lambda t: V((8 + 8 * PADS[t], 128), jnp.int32)
    with jax.named_scope("front"):
        pl.run_scoped(front, PADT(4), V((2, 7, H, Dh), bf16), V((2, 7, Dh, Dh), bf16), V((3, TM, D), bf16), V((D, F), bf16), V((F, D), bf16), V((4, D, D), bf16),
                      V((D, 2 * D), bf16), V((D, D), bf16), V((K, D), bf16),
                      pltpu.SemaphoreType.DMA((3,)), pltpu.SemaphoreType.DMA((11,)))

    def back(dc, padA, stats):
        def attention(padB, gbuf, padC):
            for p_ in (padA, padB, padC):
                fill_zref(p_)

            def stage_D1(j, chained=True):
                return ln_chain(lambda r, n: xr[rows(j, r, n), :], chained=chained, nch=LCHD)[0]

            def stage_D2(j, a):
                ga = _smm(lambda k: a[k], lambda k: wp1[0, k])
                gb_ = _smm(lambda k: a[k], lambda k: wp1[1, k])
                g = [_hglu(u, v) for u, v in zip(ga, gb_)]
                for q in QORD:
                    for t in range(2):
                        cb = 2 * (q % 2) + t
                        v = g[q][:, t * 128:(t + 1) * 128]
                        r0 = HALO + (q // 2) * H
                        gbuf[j % 2, cb, r0:r0 + H, :] = v
                        if q // 2 == 1:
                            gbuf[(j + 1) % 2, cb, 0:HALO, :] = v[H - HALO:H]

            class Conv:
                def __init__(self, j, cb, nch, head=None):
                    self.j, self.cb, self.nch = j, cb, nch
                    self.w = [dwb[k, cb] for k in range(K)]
                    self.prev = [head] * max(nch, 1)
                    self.shift = self.s1 = self.s2 = None
                    first = j % NTB == 0
                    self.lim = (jnp.where(first, HALO, 2 * HALO), jnp.where(first, HALO, 0))

                def step(self, n):
                    j, cb = self.j, self.cb
                    sub = lax.broadcasted_iota(jnp.int32, (8, 128), 0)
                    acc = None
                    for k in range(K):
                        i0 = 8 * n + k + 1
                        t = gbuf[j % 2, cb, pl.ds(i0, 8), :]
                        if n == 0 and i0 + 7 >= HALO:
                            t = jnp.where(sub + i0 < self.lim[0], t, 0.0)
                        if n == 1 and i0 < HALO:
                            t = jnp.where(sub + i0 >= self.lim[1], t, 0.0)
                        t = t * self.w[k]
                        if acc is None:
                            acc = tie(self.prev[n % self.nch], t) if self.nch else t
                        else:
                            acc = acc + t
                    dc[cb, pl.ds(pl.multiple_of(j * TM + 8 * n, 8), 8), :] = acc
                    if self.nch:
                        self.prev[n % self.nch] = acc
                    return acc

                def run(self):
                    j, cb = self.j, self.cb
                    ns = TM // 8
                    shift = self.step(1)
                    s1 = s2 = None
                    for n in [0] + list(range(2, ns)):
                        d = self.step(n) - shift
                        if n == 0:
                            d = jnp.where(j > 0, d, 0.0)
                        s1 = d if s1 is None else s1 + d
                        s2 = d * d if s2 is None else s2 + d * d
                    inv = jnp.where(j > 0, 1.0 / ns, 1.0 / (ns - 1))
                    js = pl.ds(pl.multiple_of(j * 8, 8), 8)
                    stats[0, cb, js, :] = shift + s1 * inv
                    stats[1, cb, js, :] = s2 - s1 * s1 * inv
                    return self.prev[-1]

            for cb in range(4):
                gbuf[0, cb, 0:HALO, :] = jnp.zeros((HALO, 128), f32)
                gbuf[1, cb, HALO:2 * HALO, :] = jnp.zeros((HALO, 128), f32)

            def p2(i, carry):
                a = stage_D1(i - 1)
                att_qk(i)
                stage_D2(i - 1, a)
                att_stats()
                att_pv(i, lambda c, prev: Conv(i - 1, c, ECH, prev).run(), PVU)
                return carry

            if ONLY in ('p1', 'p4', 'f0', 't0'):
                return
            if ONLY != 'e0':
                with jax.named_scope("p2loop"):
                    lax.fori_loop(1, P2END, p2, 0)
            if ONLY not in (None, 'e0'):
                return

            stage_D2(NT - 1, stage_D1(NT - 1, chained=False))
            for cb in range(4):
                Conv(NT - 1, cb, EPI_LAST).run()
                acc = Conv(NT, cb, 0).step(0)
                stats[0, cb, 8 * NT:8 * NT + 8, :] = acc
                stats[1, cb, 8 * NT:8 * NT + 8, :] = jnp.zeros((8, 128), f32)

        pl.run_scoped(attention, PADT(2), V((2, 4, TM + HALO, 128), f32), PADT(3))

        st0 = jnp.concatenate([stats[0, cb] for cb in range(4)], axis=1)
        st1 = jnp.concatenate([stats[1, cb] for cb in range(4)], axis=1)
        grow = lax.broadcasted_iota(jnp.int32, st0.shape, 0)
        cnt = jnp.where(grow < 8, TM // 8 - 1, jnp.where(grow < 8 * NT, TM // 8, 1)).astype(f32)
        mu = jnp.sum(cnt * st0, axis=0, keepdims=True) * (1.0 / N)
        dm = st0 - mu
        var = jnp.sum(st1 + cnt * dm * dm, axis=0, keepdims=True) * (1.0 / N)
        rsd = 0.5 * lax.rsqrt(var + EPS)

        def final(padG, hnops, zops, obuf, osem):
            fill_zref(padG)

            def ocopy(t, slot):
                return pltpu.make_async_copy(obuf.at[slot], out_hbm.at[pl.ds(pl.multiple_of(t * TM, 16), TM), :], osem.at[slot])

            def stage_F1(j, prev=None, chained=True):
                def zq(r0, n, hi):
                    rr = pl.ds(pl.multiple_of(j * TM + 8 + r0, 8), n)
                    d = jnp.concatenate([dc[2 * hi + t, rr, :] for t in range(2)], axis=1)
                    return (d - mu[:, hi * Dh:(hi + 1) * Dh]) * rsd[:, hi * Dh:(hi + 1) * Dh]
                if not chained:
                    return _a_ops(*[_hsilu(zq(r0, H, hi)) for r0 in (0, H) for hi in (0, 1)])
                for r in range(0, H, 16):
                    z = []
                    for r0 in (0, H):
                        for hi in (0, 1):
                            t = _hsilu(tie0(prev, zq(r0 + r, 16, hi)))
                            prev = t[:, :128] + t[:, 128:]
                            z.append(t)
                    for k, o in enumerate(_a_ops(*z)):
                        zops[k, r:r + 16, :] = o
                return prev

            def stage_F2(j, a=None):
                E = _smm((lambda k: zops[k]) if a is None else (lambda k: a[k]), lambda k: wp2[k])
                for q in QORD:
                    xr[qidx(j, q)] = xr[qidx(j, q)] + E[q]

            def stage_F3(j, slot, prev=None, nch=None):
                def st(k, r, n, v):
                    hnops[slot, k, r:r + n, :] = v
                return ln_chain(lambda r, n: xr[rows(j, r, n), :], st, prev, nch=nch or LCH4)[1]

            def stage_G2(i, U):
                d = ff_down(U)
                for q in DQORD:
                    xr[qidx(i, q)] = xr[qidx(i, q)] + d[q]

            def stage_Hh(j, chained=True):
                slot = j % 2
                if not chained:
                    obuf[slot, 0:H, :] = _ln(xr[rows(j), :]).astype(bf16)
                    obuf[slot, H:TM, :] = _ln(xr[rows(j, H), :]).astype(bf16)
                    return None
                heads = [None] * HCH
                for n, r in enumerate(range(0, TM, HG)):
                    y = _ln(tie0(heads[n % HCH], xr[rows(j, r, HG), :]))
                    prev = heads[n % HCH] = y[:, :128]
                    obuf[slot, r:r + HG, :] = y.astype(bf16)
                return prev

            if ONLY in ('p1', 'p2', 'f0'):
                return
            if ONLY in (None, 'e0'):
                stage_F2(0, stage_F1(0, chained=False))
                stage_F3(0, 0, stage_F1(1), nch=EPI_LN)

            def p4(i, carry):
                if ONLY is None:
                    @pl.when(i >= 3)
                    def _():
                        ocopy(i - 3, (i - 3) % 2).wait()
                stage_F2(i + 1)
                U = ff_up(hnops, i % 2)
                prev = stage_Hh(jnp.maximum(i - 1, 0))
                prev = stage_F3(i + 1, (i + 1) % 2, prev[0:16] if LINK & 1 else None)
                stage_F1(jnp.minimum(i + 2, NT - 1), prev if LINK & 2 else None)
                stage_G2(i, U)

                if ONLY is None:
                    @pl.when(i >= 1)
                    def _():
                        ocopy(i - 1, (i - 1) % 2).start()
                return carry

            if ONLY == 'e0':
                return
            if ONLY != 't0':
                with jax.named_scope("p4loop"):
                    lax.fori_loop(0, P4END, p4, 0)
            if ONLY not in (None, 't0'):
                return

            ocopy(NT - 4, (NT - 4) % 2).wait()
            ocopy(NT - 3, (NT - 3) % 2).wait()
            U = ff_up(hnops, (NT - 1) % 2)
            stage_Hh(NT - 2)
            d = ff_down(U)
            slot = (NT - 1) % 2
            last = [ocopy(NT - 2, (NT - 2) % 2)]
            for half in range(2):
                x4 = cat(*[xr[qidx(NT - 1, 2 * half + t)] + d[2 * half + t] for t in range(2)])
                obuf[slot, half * H:(half + 1) * H, :] = _ln(x4).astype(bf16)
                last.append(pltpu.make_async_copy(obuf.at[slot, half * H:(half + 1) * H, :],
                                                  out_hbm.at[pl.ds((NT - 1) * TM + half * H, H), :], osem.at[1 + half]))
                if half == 0:
                    last[0].start()
                last[-1].start()
            for c_ in last:
                c_.wait()

        pl.run_scoped(final, PADT(5), V((2, 7, H, Dh), bf16), V((7, H, Dh), bf16), V((2, TM, D), bf16),
                      pltpu.SemaphoreType.DMA((3,)))

    with jax.named_scope("back"):
        pl.run_scoped(back, V((4, N + 8, 128), f32), PADT(1), V((2, 4, 8 * NT + 8, 128), f32))


@jax.jit
def pallas_standalone__conformer_family_conformer__speech_kernel(
    x, w_ff1_a, w_ff1_b, w_q, w_k, w_v, w_o, w_pw1, dw, w_pw2, w_ff2_a, w_ff2_b):
    B, T, D = x.shape
    K = dw.shape[0]
    F = w_ff1_a.shape[1]
    N = B * T
    TM = 2 * H
    NT = N // TM
    TP = (T // 2 + 127) // 128 * 128
    Dh = D // 2
    kern = functools.partial(_kernel, B=B, T=T, D=D, K=K, F=F)
    hbm = pl.BlockSpec(memory_space=pl.ANY)
    V = pltpu.VMEM
    out = pl.pallas_call(
        kern,
        out_shape=jax.ShapeDtypeStruct((N, D), x.dtype),
        in_specs=[hbm] * 12,
        out_specs=hbm,
        scratch_shapes=[
            V((N, D), f32),
            V((NT, 7, H, Dh), bf16),
            V((B, 7, TP, Dh), bf16),
            V((B, 7, TP, Dh), bf16),
            V((7, Dh, F // 2), bf16),
            V((7, F // 2, Dh), bf16),
            V((2, 7, Dh, Dh), bf16),
            V((7, Dh, Dh), bf16),
            V((K, 4, 8, 128), f32),
            V((TP // W, 4, H, W), f32),
            V((2, H, 128), f32),
            V((2, TP // W - 1, 2, H, 128), f32),
            V((8 + 8 * PADS[0], 128), jnp.int32),
            V((8, 128), jnp.int32),
            pltpu.SemaphoreType.DMA(()),
        ],
        compiler_params=pltpu.CompilerParams(vmem_limit_bytes=VMEM_LIMIT),
    )(x.reshape(N, D), w_ff1_a, w_ff1_b, w_q, w_k, w_v, w_o, w_pw1, dw, w_pw2, w_ff2_a, w_ff2_b)
    return out.reshape(B, T, D)
```

```python
import functools
import jax
import jax.numpy as jnp
from jax import lax
import jax.experimental.pallas as pl
import jax.experimental.pallas.tpu as pltpu

H = 400
W = 512
EPS = 1e-5
LOG2E = 1.4426950408889634
NEG = -1e30
HALO = 16
UPO = (1, 2, 0, 5, 3, 4, 6)
DNO = (1, 3, 6, 0, 2, 4, 5)
DQORD = (2, 0, 1, 3)
PR = (40, 40, 40, 40)
P2G = 8
EPI_CH = 2
EPI_LAST = 0
EPI_LN = 9
LCH1 = 2
LCH4 = 2
HCH = 1
LCHD = 1
PVO = (1, 3, 6, 0, 2, 4, 5)
PVQ = (2, 0, 1, 3)
PKF = False
MIDUP = 2
BLINK = 2
HG = 32
LINK = 1
P1END = 10
P4END = 9
P2END = 10
PCHF = 8
PCH = 4
ECH = 1
PEEL_UNROLL = 2
PEEL_PCH = 16
PEEL_ROLL = False
PVU = 2
ONLY = None
VMEM_LIMIT = 127 * 1024 * 1024

bf16 = jnp.bfloat16
f32 = jnp.float32
u32 = jnp.uint32


def _ln(x):
    m = jnp.mean(x, axis=-1, keepdims=True)
    c = x - m
    v = jnp.mean(c * c, axis=-1, keepdims=True)
    return c * lax.rsqrt(v + EPS)


def _hsilu(h):
    return h * jnp.tanh(h) + h


def _hglu(a, b):
    return a * jnp.tanh(b) + a


def _dot(a, b):
    return jnp.dot(a, b, preferred_element_type=f32)


def _dot_nt(a, b):
    return lax.dot_general(a, b, (((1,), (1,)), ((), ())), preferred_element_type=f32)


def _a_sums(A11, A12, A21, A22):
    return [A11 + A22, A21 + A22, A11, A22, A11 + A12, A21 - A11, A12 - A22]


def _a_ops(*q):
    return [t.astype(bf16) for t in _a_sums(*q)]


def _b_ops(B11, B12, B21, B22):
    return [t.astype(bf16) for t in
            (B11 + B22, B11, B12 - B22, B21 - B11, B22, B11 + B12, B21 + B22)]


def _smm(a, w, order=UPO, dot=_dot, mid=None):
    M = [None] * 7
    for n, k in enumerate(order):
        if mid is not None and n == mid[0]:
            mid[1]()
        M[k] = dot(a(k), w(k))
    return _comb(M)


def _comb(M):
    return (M[0] + M[3] - M[4] + M[6], M[2] + M[4], M[1] + M[3], M[0] - M[1] + M[2] + M[5])


def _pk(v):
    return pltpu.bitcast(v, jnp.uint32)


def _un(v):
    return pltpu.bitcast(v, bf16)


def _hr(r0, n):
    h = r0 // 2
    return pl.ds(h if isinstance(h, int) else pl.multiple_of(h, 8), n // 2)


def _pkf(v):
    return _pk(v) if PKF else v


def _unf(v):
    return _un(v) if PKF else v


def _hrf(r0, n):
    return _hr(r0, n) if PKF else pl.ds(r0 if isinstance(r0, int) else pl.multiple_of(r0, 16), n)


def VF(shape):
    return pltpu.VMEM(shape[:-2] + (shape[-2] // 2, shape[-1]), u32) if PKF else pltpu.VMEM(shape, bf16)


def _cat(a, b):
    return jnp.concatenate([a, b], axis=1)


def _kernel(x_hbm, w1a_h, w1b_h, wq_h, wk_h, wv_h, wo_h, wp1_h, dw_h, wp2_h, w2a_h, w2b_h, out_hbm,
            xr, hops, kops, vops, wa, wb, wp1, wp2, dwb, sbuf, mbuf, cstat, zsrc, zref, zsem, *, B, T, D, K, F):
    N = B * T
    TM = 2 * H
    NTB = T // TM
    NT = B * NTB
    TH = T // 2
    TP = 2 * kops.shape[2]
    NC = TP // W
    Dh = D // 2
    cat = _cat
    ident = tuple(range(7))

    zsrc[...] = jnp.zeros_like(zsrc)
    zcopy = pltpu.make_async_copy(zsrc, zref, zsem)
    zcopy.start()
    zcopy.wait()

    def tie(prev, v):
        if prev is None:
            return v
        never = jnp.tile(zref[0:8, :], (v.shape[0] // 8, 1)) != 0
        return jnp.where(never, prev, v)

    def tie0(prev, v):
        return v if prev is None else cat(tie(prev, v[:, :128]), v[:, 128:])

    def al16(v):
        return v if isinstance(v, int) else pl.multiple_of(v, 16)

    def rows(i, off=0, n=H):
        return pl.ds(al16(i * TM + off), n)

    def ln_chain(load, store=None, prev=None, chained=True, nch=1):
        if not chained:
            ht, hb = _ln(load(0, H)), _ln(load(H, H))
            ops = _a_ops(ht[:, :Dh], ht[:, Dh:], hb[:, :Dh], hb[:, Dh:])
            if store is not None:
                for k in range(7):
                    store(k, 0, H, ops[k])
            return ops, None
        outs = [[] for _ in range(7)]
        heads = [prev] * nch
        for n, r in enumerate(range(0, H, 16)):
            ht, hb = _ln(tie0(heads[n % nch], load(r, 16))), _ln(load(H + r, 16))
            s = _a_sums(ht[:, :Dh], ht[:, Dh:], hb[:, :Dh], hb[:, Dh:])
            prev = heads[n % nch] = s[0][:, :128]
            for k in range(7):
                o = s[k].astype(bf16)
                outs[k].append(o)
                if store is not None:
                    store(k, r, 16, o)
        return [jnp.concatenate(o, axis=0) for o in outs], prev

    def chained(fn, x, pr):
        if pr == 0:
            return fn(x)
        prev = None
        cols = []
        for t in range(x.shape[1] // 128):
            parts = []
            for r in range(0, x.shape[0], pr):
                prev = fn(tie(prev, x[r:r + pr, t * 128:(t + 1) * 128]))
                parts.append(prev)
            cols.append(jnp.concatenate(parts, axis=0))
        return jnp.concatenate(cols, axis=1)

    def build_b_ops(raw, dst, r0, nr, c0, n, scale, chained=True, prev=None):
        k = raw.shape[0] // 2
        nh = n // 2
        n_ = 0
        for r in range(0, nr, 16):
            for c in range(0, nh, 128):
                def blk(ro, co):
                    return raw[pl.ds(al16(ro + r0 + r), 16), c0 + co + c:c0 + co + c + 128].astype(f32) * scale
                B11, B12, B21, B22 = tie(prev if chained else None, blk(0, 0)), blk(0, nh), blk(k, 0), blk(k, nh)
                n_ += 1
                if n_ % BLINK == 0:
                    prev = jnp.broadcast_to(jnp.max((B11 + B12) + (B21 + B22), axis=-1, keepdims=True), (16, 128))
                ops = _b_ops(B11, B12, B21, B22)
                for i in range(7):
                    if dst.dtype == u32:
                        dst[i, _hr(r0 + r, 16), c:c + 128] = _pk(ops[i])
                    else:
                        dst[i, pl.ds(al16(r0 + r), 16), c:c + 128] = ops[i]
        return prev

    QORD = (3, 2, 1, 0)

    def qidx(i, q):
        return rows(i, (q // 2) * H), slice((q % 2) * Dh, (q % 2 + 1) * Dh)

    def ff_up(hnops, slot, mid=None):
        C = _smm(lambda k: _unf(hnops[slot, k]), lambda k: _unf(wa[k]), UPO, mid=mid)
        return [chained(_hsilu, C[q], PR[q]) for q in range(4)]

    def ff_down(U):
        a = _a_ops(*U)
        return _smm(lambda k: a[k], lambda k: _unf(wb[k]), DNO)

    def stage_C1(i, prev=None, chained=True):
        def st(k, r, n, v):
            hops[i, k, _hr(r, n), :] = _pk(v)
        return ln_chain(lambda r, n: xr[rows(i, r, n), :], st, prev, chained=chained, nch=LCH1)

    def stage_C2(wkv, i, a):
        b = i // NTB
        r = _hr((i % NTB) * H, H)
        c = D ** -0.5 * LOG2E
        ktl, kth, kbl, kbh = [t * c for t in _smm(lambda k: a[k], lambda k: _unf(wkv[0, k]))]
        ops = _b_ops(ktl, kbl, kth, kbh)
        for k in range(7):
            kops[b, k, r, :] = _pk(ops[k])
        vtl, vth, vbl, vbh = _smm(lambda k: a[k], lambda k: _unf(wkv[1, k]))
        ops = _b_ops(vtl, vth, vbl, vbh)
        for k in range(7):
            vops[b, k, r, :] = _pk(ops[k])

    def att_qk(i, rolled=False):
        b = i // NTB

        def chunk(c, carry=None):
            static = isinstance(c, int)
            kr = _hr(c * W, W)
            s = list(_smm(lambda k: _un(hops[i, k]), lambda k: _un(kops[b, k, kr, :]), ident, _dot_nt))
            nv = TH - c * W
            for j in range(4):
                t = s[j]
                if not static:
                    t = jnp.where(lax.broadcasted_iota(jnp.int32, (H, W), 1) < nv, t, NEG)
                elif nv < W:
                    lo = nv // 128 * 128
                    col = lax.broadcasted_iota(jnp.int32, (H, W - lo), 1)
                    t = cat(t[:, :lo], jnp.where(col < nv - lo, t[:, lo:], NEG))
                sbuf[c, j] = t
            return carry

        if rolled:
            lax.fori_loop(0, NC, chunk, 0)
        else:
            for c in range(NC):
                chunk(c)

    def att_stats(nch0=None, nchf=None):
        nch0, nchf = nch0 or PCH, nchf or PCHF
        prev = [None] * nch0
        n = 0
        for c in range(NC):
            if c == NC - 1:
                prev = [prev[t % nch0] for t in range(nchf)]
            nch = len(prev)
            for r in range(0, H, P2G):
                for half in range(2):
                    rs = slice(r, r + P2G)
                    blocks = [sbuf[c, 2 * half + j, rs, t * 128:(t + 1) * 128]
                              for j in (0, 1) for t in range(W // 128)]
                    blocks[0] = tie(prev[n % nch], blocks[0])
                    m = jnp.broadcast_to(
                        jnp.max(functools.reduce(jnp.maximum, blocks), axis=-1, keepdims=True), (P2G, 128))
                    if c < NC - 1:
                        l = functools.reduce(jnp.add, [jnp.exp2(t - m) for t in blocks])
                        cstat[0, c, half, rs, :] = m
                        cstat[1, c, half, rs, :] = l
                        prev[n % nch] = l
                    else:
                        ms = [cstat[0, cc, half, rs, :] for cc in range(NC - 1)]
                        m = functools.reduce(jnp.maximum, ms + [m])
                        l = functools.reduce(jnp.add, [jnp.exp2(t - m) for t in blocks]
                                             + [cstat[1, cc, half, rs, :] * jnp.exp2(ms[cc] - m) for cc in range(NC - 1)])
                        mp = m + jnp.log2(jnp.sum(l, axis=-1, keepdims=True))
                        mbuf[half, rs, :] = mp
                        prev[n % nch] = mp
                    n += 1

    def att_pv(i, side, unroll=1):
        b = i // NTB

        def operands(c):
            mt = jnp.concatenate([mbuf[0]] * (W // 128), axis=1)
            mb = jnp.concatenate([mbuf[1]] * (W // 128), axis=1)
            ms = (mt, mt, mb, mb)
            a = _a_ops(*[jnp.exp2(sbuf[c, j] - ms[j]) for j in range(4)])
            return a, _hr(c * W, W)

        def rolled(t, carry):
            prev = None
            acc = [None] * 7
            for u in range(unroll):
                c = t * unroll + u
                a, kr = operands(c)
                for k in PVO:
                    m = _dot(a[k], _un(vops[b, k, kr, :]))
                    acc[k] = m if acc[k] is None else acc[k] + m
                prev = side(c, prev)
            O = _comb(acc)
            for q in PVQ:
                xr[qidx(i, q)] = xr[qidx(i, q)] + O[q]
            return carry

        if unroll >= NC:
            rolled(0, 0)
        else:
            lax.fori_loop(0, NC // unroll, rolled, 0)

    def front(hnops, wkv, xbuf, rawa, rawb, rawq, rawp1, rawp2, rawdw, xsem, wsem):
        def xcopy(t, slot):
            return pltpu.make_async_copy(x_hbm.at[pl.ds(pl.multiple_of(t * TM, 16), TM), :], xbuf.at[slot], xsem.at[slot])

        cp = [
            pltpu.make_async_copy(wq_h, rawq.at[0], wsem.at[0]),
            pltpu.make_async_copy(wk_h, rawq.at[1], wsem.at[1]),
            pltpu.make_async_copy(wv_h, rawq.at[2], wsem.at[2]),
            pltpu.make_async_copy(wo_h, rawq.at[3], wsem.at[3]),
            pltpu.make_async_copy(w1a_h, rawa, wsem.at[4]),
            pltpu.make_async_copy(w1b_h, rawb, wsem.at[5]),
            pltpu.make_async_copy(dw_h, rawdw, wsem.at[6]),
            pltpu.make_async_copy(wp1_h, rawp1, wsem.at[7]),
            pltpu.make_async_copy(wp2_h, rawp2, wsem.at[8]),
            pltpu.make_async_copy(w2a_h, rawa, wsem.at[9]),
            pltpu.make_async_copy(w2b_h, rawb, wsem.at[10]),
        ]
        CQ, CK, CV, CO, C1A, C1B, CDW, CP1, CP2, C2A, C2B = range(11)

        def stage_A(t, slot, chained=True):
            xs = t % 3

            def st(k, r, n, v):
                hnops[slot, k, _hrf(r, n), :] = _pkf(v)
            return ln_chain(lambda r, n: xbuf[xs, r:r + n, :].astype(f32), st, chained=chained, nch=LCH1)[1]

        def stage_B2(i, U):
            d = ff_down(U)
            xs = i % 3
            for q in DQORD:
                r0, c0 = (q // 2) * H, (q % 2) * Dh
                xr[qidx(i, q)] = xbuf[xs, r0:r0 + H, c0:c0 + Dh].astype(f32) + d[q]

        def p1(i, carry, dma=True):
            if dma:
                @pl.when(i + 2 < NT)
                def _():
                    xcopy(i + 2, (i + 2) % 3).start()

                @pl.when(i + 1 < NT)
                def _():
                    xcopy(i + 1, (i + 1) % 3).wait()
            U = ff_up(hnops, i % 2)
            prev = stage_A(jnp.minimum(i + 1, NT - 1), (i + 1) % 2)
            hq, _ = stage_C1(i - 1, prev)
            stage_B2(i, U)
            stage_C2(wkv, i - 1, hq)
            return carry

        if ONLY == 'p1':
            lax.fori_loop(1, NT, lambda i, c: p1(i, c, False), 0)
            return
        if ONLY not in (None, 'f0'):
            return
        cp[C1A].start()
        xcopy(0, 0).start()
        for b in range(B):
            for k in range(7):
                kops[b, k, TH // 2:, :] = jnp.zeros(((TP - TH) // 2, Dh), jnp.uint32)
                vops[b, k, TH // 2:, :] = jnp.zeros(((TP - TH) // 2, Dh), jnp.uint32)
        xcopy(0, 0).wait()
        cp[C1B].start()
        stage_A(0, 0, chained=False)
        cp[C1A].wait()
        build_b_ops(rawa, wa, 0, Dh, 0, F, 0.5, chained=False)
        early = (cp[CQ], cp[CK], cp[CV], cp[CO], xcopy(1, 1), cp[CDW])

        def mid_up():
            cp[C1B].wait()
            for c_ in early:
                c_.start()
            build_b_ops(rawb, wb, 0, F // 2, 0, D, 0.5)

        U = ff_up(hnops, 0, mid=(MIDUP, mid_up))
        for c_ in early:
            c_.wait()
        for c_ in (xcopy(2, 2), cp[CP1], cp[CP2]):
            c_.start()
        wf = _dot_nt(rawq[1], rawq[0])
        ops = _b_ops(wf[:Dh, :Dh], wf[:Dh, Dh:], wf[Dh:, :Dh], wf[Dh:, Dh:])
        for k in range(7):
            wkv[0, k] = _pkf(ops[k])
        wf = _dot(rawq[2], rawq[3])
        ops = _b_ops(wf[:Dh, :Dh], wf[:Dh, Dh:], wf[Dh:, :Dh], wf[Dh:, Dh:])
        for k in range(7):
            wkv[1, k] = _pkf(ops[k])
        stage_A(1, 1)
        stage_B2(0, U)
        dwv = rawdw[...].astype(f32)
        for k in range(K):
            for cb in range(4):
                dwb[k, cb] = jnp.broadcast_to(dwv[k:k + 1, cb * 128:(cb + 1) * 128], (8, 128))
        cp[C2A].start()
        cp[C2B].start()

        if ONLY == 'f0':
            for c_ in (xcopy(2, 2), cp[CP1], cp[CP2], cp[C2A], cp[C2B]):
                c_.wait()
            return
        with jax.named_scope("p1loop"):
            lax.fori_loop(1, P1END, p1, 0)

        cp[CP1].wait()
        cp[CP2].wait()
        cp[C2A].wait()
        cp[C2B].wait()

        def wops(c, prev):
            q = Dh // NC
            r0 = c * q if isinstance(c, int) else pl.multiple_of(c * q, 16)
            r1 = c * (F // 2 // NC) if isinstance(c, int) else pl.multiple_of(c * (F // 2 // NC), 16)
            prev = build_b_ops(rawp1, wp1.at[0], r0, q, 0, D, 0.5, prev=prev)
            prev = build_b_ops(rawp1, wp1.at[1], r0, q, D, D, 0.5, prev=prev)
            prev = build_b_ops(rawp2, wp2, r0, q, 0, D, 1.0, prev=prev)
            prev = build_b_ops(rawa, wa, r0, q, 0, F, 0.5, prev=prev)
            return build_b_ops(rawb, wb, r1, F // 2 // NC, 0, D, 0.5, prev=prev)

        with jax.named_scope("p2peel"):
            if PEEL_ROLL:
                att_qk(0, rolled=True)
                hq, _ = stage_C1(NT - 1, chained=False)
                stage_C2(wkv, NT - 1, hq)
                att_stats(PEEL_PCH, PEEL_PCH)
            else:
                hq, _ = stage_C1(NT - 1)
                att_qk(0)
                stage_C2(wkv, NT - 1, hq)
                att_stats()
            att_pv(0, wops, unroll=PEEL_UNROLL)

    V = pltpu.VMEM
    with jax.named_scope("front"):
        pl.run_scoped(front, VF((2, 7, H, Dh)), VF((2, 7, Dh, Dh)), V((3, TM, D), bf16), V((D, F), bf16), V((F, D), bf16), V((4, D, D), bf16),
                      V((D, 2 * D), bf16), V((D, D), bf16), V((K, D), bf16),
                      pltpu.SemaphoreType.DMA((3,)), pltpu.SemaphoreType.DMA((11,)))

    def back(dc, stats):
        def attention(gbuf):
            def stage_D1(j, chained=True):
                return ln_chain(lambda r, n: xr[rows(j, r, n), :], chained=chained, nch=LCHD)[0]

            def stage_D2(j, a):
                ga = _smm(lambda k: a[k], lambda k: _un(wp1[0, k]))
                gb_ = _smm(lambda k: a[k], lambda k: _un(wp1[1, k]))
                g = [_hglu(u, v) for u, v in zip(ga, gb_)]
                for q in QORD:
                    for t in range(2):
                        cb = 2 * (q % 2) + t
                        v = g[q][:, t * 128:(t + 1) * 128]
                        r0 = HALO + (q // 2) * H
                        gbuf[j % 2, cb, r0:r0 + H, :] = v
                        if q // 2 == 1:
                            gbuf[(j + 1) % 2, cb, 0:HALO, :] = v[H - HALO:H]

            class Conv:
                def __init__(self, j, cb, nch, head=None):
                    self.j, self.cb, self.nch = j, cb, nch
                    self.w = [dwb[k, cb] for k in range(K)]
                    self.prev = [head] * max(nch, 1)
                    self.shift = self.s1 = self.s2 = None
                    first = j % NTB == 0
                    self.lim = (jnp.where(first, HALO, 2 * HALO), jnp.where(first, HALO, 0))

                def step(self, n):
                    j, cb = self.j, self.cb
                    sub = lax.broadcasted_iota(jnp.int32, (8, 128), 0)
                    acc = None
                    for k in range(K):
                        i0 = 8 * n + k + 1
                        t = gbuf[j % 2, cb, pl.ds(i0, 8), :]
                        if n == 0 and i0 + 7 >= HALO:
                            t = jnp.where(sub + i0 < self.lim[0], t, 0.0)
                        if n == 1 and i0 < HALO:
                            t = jnp.where(sub + i0 >= self.lim[1], t, 0.0)
                        t = t * self.w[k]
                        if acc is None:
                            acc = tie(self.prev[n % self.nch], t) if self.nch else t
                        else:
                            acc = acc + t
                    dc[cb, pl.ds(pl.multiple_of(j * TM + 8 * n, 8), 8), :] = acc
                    if self.nch:
                        self.prev[n % self.nch] = acc
                    return acc

                def run(self):
                    j, cb = self.j, self.cb
                    ns = TM // 8
                    shift = self.step(1)
                    s1 = s2 = None
                    for n in [0] + list(range(2, ns)):
                        d = self.step(n) - shift
                        if n == 0:
                            d = jnp.where(j > 0, d, 0.0)
                        s1 = d if s1 is None else s1 + d
                        s2 = d * d if s2 is None else s2 + d * d
                    inv = jnp.where(j > 0, 1.0 / ns, 1.0 / (ns - 1))
                    js = pl.ds(pl.multiple_of(j * 8, 8), 8)
                    stats[0, cb, js, :] = shift + s1 * inv
                    stats[1, cb, js, :] = s2 - s1 * s1 * inv
                    return self.prev[-1]

            for cb in range(4):
                gbuf[0, cb, 0:HALO, :] = jnp.zeros((HALO, 128), f32)
                gbuf[1, cb, HALO:2 * HALO, :] = jnp.zeros((HALO, 128), f32)

            def p2(i, carry):
                a = stage_D1(i - 1)
                att_qk(i)
                stage_D2(i - 1, a)
                att_stats()
                att_pv(i, lambda c, prev: Conv(i - 1, c, ECH, prev).run(), PVU)
                return carry

            if ONLY in ('p1', 'p4', 'f0', 't0'):
                return
            if ONLY != 'e0':
                with jax.named_scope("p2loop"):
                    lax.fori_loop(1, P2END, p2, 0)
            if ONLY not in (None, 'e0'):
                return

            stage_D2(NT - 1, stage_D1(NT - 1, chained=False))
            for cb in range(4):
                Conv(NT - 1, cb, EPI_LAST).run()
                acc = Conv(NT, cb, 0).step(0)
                stats[0, cb, 8 * NT:8 * NT + 8, :] = acc
                stats[1, cb, 8 * NT:8 * NT + 8, :] = jnp.zeros((8, 128), f32)

        pl.run_scoped(attention, V((2, 4, TM + HALO, 128), f32))

        st0 = jnp.concatenate([stats[0, cb] for cb in range(4)], axis=1)
        st1 = jnp.concatenate([stats[1, cb] for cb in range(4)], axis=1)
        grow = lax.broadcasted_iota(jnp.int32, st0.shape, 0)
        cnt = jnp.where(grow < 8, TM // 8 - 1, jnp.where(grow < 8 * NT, TM // 8, 1)).astype(f32)
        mu = jnp.sum(cnt * st0, axis=0, keepdims=True) * (1.0 / N)
        dm = st0 - mu
        var = jnp.sum(st1 + cnt * dm * dm, axis=0, keepdims=True) * (1.0 / N)
        rsd = 0.5 * lax.rsqrt(var + EPS)

        def final(hnops, zops, obuf, osem):
            def ocopy(t, slot):
                return pltpu.make_async_copy(obuf.at[slot], out_hbm.at[pl.ds(pl.multiple_of(t * TM, 16), TM), :], osem.at[slot])

            def stage_F1(j, prev=None, chained=True):
                def zq(r0, n, hi):
                    rr = pl.ds(pl.multiple_of(j * TM + 8 + r0, 8), n)
                    d = jnp.concatenate([dc[2 * hi + t, rr, :] for t in range(2)], axis=1)
                    return (d - mu[:, hi * Dh:(hi + 1) * Dh]) * rsd[:, hi * Dh:(hi + 1) * Dh]
                if not chained:
                    return _a_ops(*[_hsilu(zq(r0, H, hi)) for r0 in (0, H) for hi in (0, 1)])
                for r in range(0, H, 16):
                    z = []
                    for r0 in (0, H):
                        for hi in (0, 1):
                            t = _hsilu(tie0(prev, zq(r0 + r, 16, hi)))
                            prev = t[:, :128] + t[:, 128:]
                            z.append(t)
                    for k, o in enumerate(_a_ops(*z)):
                        zops[k, _hrf(r, 16), :] = _pkf(o)
                return prev

            def stage_F2(j, a=None):
                E = _smm((lambda k: _unf(zops[k])) if a is None else (lambda k: a[k]), lambda k: _unf(wp2[k]))
                for q in QORD:
                    xr[qidx(j, q)] = xr[qidx(j, q)] + E[q]

            def stage_F3(j, slot, prev=None, nch=None):
                def st(k, r, n, v):
                    hnops[slot, k, _hrf(r, n), :] = _pkf(v)
                return ln_chain(lambda r, n: xr[rows(j, r, n), :], st, prev, nch=nch or LCH4)[1]

            def stage_G2(i, U):
                d = ff_down(U)
                for q in DQORD:
                    xr[qidx(i, q)] = xr[qidx(i, q)] + d[q]

            def stage_Hh(j, chained=True):
                slot = j % 2
                if not chained:
                    obuf[slot, 0:H, :] = _ln(xr[rows(j), :]).astype(bf16)
                    obuf[slot, H:TM, :] = _ln(xr[rows(j, H), :]).astype(bf16)
                    return None
                heads = [None] * HCH
                for n, r in enumerate(range(0, TM, HG)):
                    y = _ln(tie0(heads[n % HCH], xr[rows(j, r, HG), :]))
                    prev = heads[n % HCH] = y[:, :128]
                    obuf[slot, r:r + HG, :] = y.astype(bf16)
                return prev

            if ONLY in ('p1', 'p2', 'f0'):
                return
            if ONLY in (None, 'e0'):
                stage_F2(0, stage_F1(0, chained=False))
                stage_F3(0, 0, stage_F1(1), nch=EPI_LN)

            def p4(i, carry):
                if ONLY is None:
                    @pl.when(i >= 3)
                    def _():
                        ocopy(i - 3, (i - 3) % 2).wait()
                stage_F2(i + 1)
                U = ff_up(hnops, i % 2)
                prev = stage_Hh(jnp.maximum(i - 1, 0))
                prev = stage_F3(i + 1, (i + 1) % 2, prev[0:16] if LINK & 1 else None)
                stage_F1(jnp.minimum(i + 2, NT - 1), prev if LINK & 2 else None)
                stage_G2(i, U)

                if ONLY is None:
                    @pl.when(i >= 1)
                    def _():
                        ocopy(i - 1, (i - 1) % 2).start()
                return carry

            if ONLY == 'e0':
                return
            if ONLY != 't0':
                with jax.named_scope("p4loop"):
                    lax.fori_loop(0, P4END, p4, 0)
            if ONLY not in (None, 't0'):
                return

            ocopy(NT - 4, (NT - 4) % 2).wait()
            ocopy(NT - 3, (NT - 3) % 2).wait()
            U = ff_up(hnops, (NT - 1) % 2)
            stage_Hh(NT - 2)
            d = ff_down(U)
            slot = (NT - 1) % 2
            last = [ocopy(NT - 2, (NT - 2) % 2)]
            for half in range(2):
                x4 = cat(*[xr[qidx(NT - 1, 2 * half + t)] + d[2 * half + t] for t in range(2)])
                obuf[slot, half * H:(half + 1) * H, :] = _ln(x4).astype(bf16)
                last.append(pltpu.make_async_copy(obuf.at[slot, half * H:(half + 1) * H, :],
                                                  out_hbm.at[pl.ds((NT - 1) * TM + half * H, H), :], osem.at[1 + half]))
                if half == 0:
                    last[0].start()
                last[-1].start()
            for c_ in last:
                c_.wait()

        pl.run_scoped(final, VF((2, 7, H, Dh)), VF((7, H, Dh)), V((2, TM, D), bf16),
                      pltpu.SemaphoreType.DMA((3,)))

    with jax.named_scope("back"):
        pl.run_scoped(back, V((4, N + 8, 128), f32), V((2, 4, 8 * NT + 8, 128), f32))


@jax.jit
def pallas_standalone__conformer_family_conformer__speech_kernel(
    x, w_ff1_a, w_ff1_b, w_q, w_k, w_v, w_o, w_pw1, dw, w_pw2, w_ff2_a, w_ff2_b):
    B, T, D = x.shape
    K = dw.shape[0]
    F = w_ff1_a.shape[1]
    N = B * T
    TM = 2 * H
    NT = N // TM
    TP = (T // 2 + 127) // 128 * 128
    Dh = D // 2
    kern = functools.partial(_kernel, B=B, T=T, D=D, K=K, F=F)
    hbm = pl.BlockSpec(memory_space=pl.ANY)
    V = pltpu.VMEM
    out = pl.pallas_call(
        kern,
        out_shape=jax.ShapeDtypeStruct((N, D), x.dtype),
        in_specs=[hbm] * 12,
        out_specs=hbm,
        scratch_shapes=[
            V((N, D), f32),
            V((NT, 7, H // 2, Dh), u32),
            V((B, 7, TP // 2, Dh), u32),
            V((B, 7, TP // 2, Dh), u32),
            VF((7, Dh, F // 2)),
            VF((7, F // 2, Dh)),
            V((2, 7, Dh // 2, Dh), u32),
            VF((7, Dh, Dh)),
            V((K, 4, 8, 128), f32),
            V((TP // W, 4, H, W), f32),
            V((2, H, 128), f32),
            V((2, TP // W - 1, 2, H, 128), f32),
            V((8, 128), jnp.int32),
            V((8, 128), jnp.int32),
            pltpu.SemaphoreType.DMA(()),
        ],
        compiler_params=pltpu.CompilerParams(vmem_limit_bytes=VMEM_LIMIT),
    )(x.reshape(N, D), w_ff1_a, w_ff1_b, w_q, w_k, w_v, w_o, w_pw1, dw, w_pw2, w_ff2_a, w_ff2_b)
    return out.reshape(B, T, D)
```

```python
import functools
import jax
import jax.numpy as jnp
from jax import lax
import jax.experimental.pallas as pl
import jax.experimental.pallas.tpu as pltpu

H = 400
W = 512
EPS = 1e-5
LOG2E = 1.4426950408889634
NEG = -1e30
HALO = 16
UPO = (1, 2, 0, 5, 3, 4, 6)
DNO = (1, 3, 6, 0, 2, 4, 5)
DQORD = (2, 0, 1, 3)
PR = (40, 40, 40, 40)
P2G = 8
EPI_CH = 2
EPI_LAST = 0
EPI_LN = 25
LCH1 = 2
LCH4 = 2
HCH = 1
LCHD = 1
PVO = (1, 3, 6, 0, 2, 4, 5)
PVQ = (2, 0, 1, 3)
PKF = False
EPI_F1 = 4
MIDUP = 2
BLINK = 2
HG = 32
LINK = 1
P1END = 10
P4END = 9
P2END = 10
PCHF = 8
PCH = 4
ECH = 1
PEEL_UNROLL = 2
PEEL_PCH = 16
PEEL_ROLL = False
PVU = 2
ONLY = None
VMEM_LIMIT = 127 * 1024 * 1024

bf16 = jnp.bfloat16
f32 = jnp.float32
u32 = jnp.uint32


def _ln(x):
    m = jnp.mean(x, axis=-1, keepdims=True)
    c = x - m
    v = jnp.mean(c * c, axis=-1, keepdims=True)
    return c * lax.rsqrt(v + EPS)


def _hsilu(h):
    return h * jnp.tanh(h) + h


def _hglu(a, b):
    return a * jnp.tanh(b) + a


def _dot(a, b):
    return jnp.dot(a, b, preferred_element_type=f32)


def _dot_nt(a, b):
    return lax.dot_general(a, b, (((1,), (1,)), ((), ())), preferred_element_type=f32)


def _a_sums(A11, A12, A21, A22):
    return [A11 + A22, A21 + A22, A11, A22, A11 + A12, A21 - A11, A12 - A22]


def _a_ops(*q):
    return [t.astype(bf16) for t in _a_sums(*q)]


def _b_ops(B11, B12, B21, B22):
    return [t.astype(bf16) for t in
            (B11 + B22, B11, B12 - B22, B21 - B11, B22, B11 + B12, B21 + B22)]


def _smm(a, w, order=UPO, dot=_dot, mid=None):
    M = [None] * 7
    for n, k in enumerate(order):
        if mid is not None and n == mid[0]:
            mid[1]()
        M[k] = dot(a(k), w(k))
    return _comb(M)


def _comb(M):
    return (M[0] + M[3] - M[4] + M[6], M[2] + M[4], M[1] + M[3], M[0] - M[1] + M[2] + M[5])


def _pk(v):
    return pltpu.bitcast(v, jnp.uint32)


def _un(v):
    return pltpu.bitcast(v, bf16)


def _hr(r0, n):
    h = r0 // 2
    return pl.ds(h if isinstance(h, int) else pl.multiple_of(h, 8), n // 2)


def _pkf(v):
    return _pk(v) if PKF else v


def _unf(v):
    return _un(v) if PKF else v


def _hrf(r0, n):
    return _hr(r0, n) if PKF else pl.ds(r0 if isinstance(r0, int) else pl.multiple_of(r0, 16), n)


def VF(shape):
    return pltpu.VMEM(shape[:-2] + (shape[-2] // 2, shape[-1]), u32) if PKF else pltpu.VMEM(shape, bf16)


def _cat(a, b):
    return jnp.concatenate([a, b], axis=1)


def _kernel(x_hbm, w1a_h, w1b_h, wq_h, wk_h, wv_h, wo_h, wp1_h, dw_h, wp2_h, w2a_h, w2b_h, out_hbm,
            xr, hops, kops, vops, wa, wb, wp1, wp2, dwb, sbuf, mbuf, cstat, zsrc, zref, zsem, *, B, T, D, K, F):
    N = B * T
    TM = 2 * H
    NTB = T // TM
    NT = B * NTB
    TH = T // 2
    TP = 2 * kops.shape[2]
    NC = TP // W
    Dh = D // 2
    cat = _cat
    ident = tuple(range(7))

    zsrc[...] = jnp.zeros_like(zsrc)
    zcopy = pltpu.make_async_copy(zsrc, zref, zsem)
    zcopy.start()
    zcopy.wait()

    def tie(prev, v):
        if prev is None:
            return v
        never = jnp.tile(zref[0:8, :], (v.shape[0] // 8, 1)) != 0
        return jnp.where(never, prev, v)

    def tie0(prev, v):
        return v if prev is None else cat(tie(prev, v[:, :128]), v[:, 128:])

    def al16(v):
        return v if isinstance(v, int) else pl.multiple_of(v, 16)

    def rows(i, off=0, n=H):
        return pl.ds(al16(i * TM + off), n)

    def ln_chain(load, store=None, prev=None, chained=True, nch=1):
        if not chained:
            ht, hb = _ln(load(0, H)), _ln(load(H, H))
            ops = _a_ops(ht[:, :Dh], ht[:, Dh:], hb[:, :Dh], hb[:, Dh:])
            if store is not None:
                for k in range(7):
                    store(k, 0, H, ops[k])
            return ops, None
        outs = [[] for _ in range(7)]
        heads = [prev] * nch
        for n, r in enumerate(range(0, H, 16)):
            ht, hb = _ln(tie0(heads[n % nch], load(r, 16))), _ln(load(H + r, 16))
            s = _a_sums(ht[:, :Dh], ht[:, Dh:], hb[:, :Dh], hb[:, Dh:])
            prev = heads[n % nch] = s[0][:, :128]
            for k in range(7):
                o = s[k].astype(bf16)
                outs[k].append(o)
                if store is not None:
                    store(k, r, 16, o)
        return [jnp.concatenate(o, axis=0) for o in outs], prev

    def chained(fn, x, pr):
        if pr == 0:
            return fn(x)
        prev = None
        cols = []
        for t in range(x.shape[1] // 128):
            parts = []
            for r in range(0, x.shape[0], pr):
                prev = fn(tie(prev, x[r:r + pr, t * 128:(t + 1) * 128]))
                parts.append(prev)
            cols.append(jnp.concatenate(parts, axis=0))
        return jnp.concatenate(cols, axis=1)

    def build_b_ops(raw, dst, r0, nr, c0, n, scale, chained=True, prev=None):
        k = raw.shape[0] // 2
        nh = n // 2
        n_ = 0
        for r in range(0, nr, 16):
            for c in range(0, nh, 128):
                def blk(ro, co):
                    return raw[pl.ds(al16(ro + r0 + r), 16), c0 + co + c:c0 + co + c + 128].astype(f32) * scale
                B11, B12, B21, B22 = tie(prev if chained else None, blk(0, 0)), blk(0, nh), blk(k, 0), blk(k, nh)
                n_ += 1
                if n_ % BLINK == 0:
                    prev = jnp.broadcast_to(jnp.max((B11 + B12) + (B21 + B22), axis=-1, keepdims=True), (16, 128))
                ops = _b_ops(B11, B12, B21, B22)
                for i in range(7):
                    if dst.dtype == u32:
                        dst[i, _hr(r0 + r, 16), c:c + 128] = _pk(ops[i])
                    else:
                        dst[i, pl.ds(al16(r0 + r), 16), c:c + 128] = ops[i]
        return prev

    QORD = (3, 2, 1, 0)

    def qidx(i, q):
        return rows(i, (q // 2) * H), slice((q % 2) * Dh, (q % 2 + 1) * Dh)

    def ff_up(hnops, slot, mid=None):
        C = _smm(lambda k: _unf(hnops[slot, k]), lambda k: _unf(wa[k]), UPO, mid=mid)
        return [chained(_hsilu, C[q], PR[q]) for q in range(4)]

    def ff_down(U):
        a = _a_ops(*U)
        return _smm(lambda k: a[k], lambda k: _unf(wb[k]), DNO)

    def stage_C1(i, prev=None, chained=True):
        def st(k, r, n, v):
            hops[i, k, _hr(r, n), :] = _pk(v)
        return ln_chain(lambda r, n: xr[rows(i, r, n), :], st, prev, chained=chained, nch=LCH1)

    def stage_C2(wkv, i, a):
        b = i // NTB
        r = _hr((i % NTB) * H, H)
        c = D ** -0.5 * LOG2E
        ktl, kth, kbl, kbh = [t * c for t in _smm(lambda k: a[k], lambda k: _unf(wkv[0, k]))]
        ops = _b_ops(ktl, kbl, kth, kbh)
        for k in range(7):
            kops[b, k, r, :] = _pk(ops[k])
        vtl, vth, vbl, vbh = _smm(lambda k: a[k], lambda k: _unf(wkv[1, k]))
        ops = _b_ops(vtl, vth, vbl, vbh)
        for k in range(7):
            vops[b, k, r, :] = _pk(ops[k])

    def att_qk(i, rolled=False):
        b = i // NTB

        def chunk(c, carry=None):
            static = isinstance(c, int)
            kr = _hr(c * W, W)
            s = list(_smm(lambda k: _un(hops[i, k]), lambda k: _un(kops[b, k, kr, :]), ident, _dot_nt))
            nv = TH - c * W
            for j in range(4):
                t = s[j]
                if not static:
                    t = jnp.where(lax.broadcasted_iota(jnp.int32, (H, W), 1) < nv, t, NEG)
                elif nv < W:
                    lo = nv // 128 * 128
                    col = lax.broadcasted_iota(jnp.int32, (H, W - lo), 1)
                    t = cat(t[:, :lo], jnp.where(col < nv - lo, t[:, lo:], NEG))
                sbuf[c, j] = t
            return carry

        if rolled:
            lax.fori_loop(0, NC, chunk, 0)
        else:
            for c in range(NC):
                chunk(c)

    def att_stats(nch0=None, nchf=None):
        nch0, nchf = nch0 or PCH, nchf or PCHF
        prev = [None] * nch0
        n = 0
        for c in range(NC):
            if c == NC - 1:
                prev = [prev[t % nch0] for t in range(nchf)]
            nch = len(prev)
            for r in range(0, H, P2G):
                for half in range(2):
                    rs = slice(r, r + P2G)
                    blocks = [sbuf[c, 2 * half + j, rs, t * 128:(t + 1) * 128]
                              for j in (0, 1) for t in range(W // 128)]
                    blocks[0] = tie(prev[n % nch], blocks[0])
                    m = jnp.broadcast_to(
                        jnp.max(functools.reduce(jnp.maximum, blocks), axis=-1, keepdims=True), (P2G, 128))
                    if c < NC - 1:
                        l = functools.reduce(jnp.add, [jnp.exp2(t - m) for t in blocks])
                        cstat[0, c, half, rs, :] = m
                        cstat[1, c, half, rs, :] = l
                        prev[n % nch] = l
                    else:
                        ms = [cstat[0, cc, half, rs, :] for cc in range(NC - 1)]
                        m = functools.reduce(jnp.maximum, ms + [m])
                        l = functools.reduce(jnp.add, [jnp.exp2(t - m) for t in blocks]
                                             + [cstat[1, cc, half, rs, :] * jnp.exp2(ms[cc] - m) for cc in range(NC - 1)])
                        mp = m + jnp.log2(jnp.sum(l, axis=-1, keepdims=True))
                        mbuf[half, rs, :] = mp
                        prev[n % nch] = mp
                    n += 1

    def att_pv(i, side, unroll=1):
        b = i // NTB

        def operands(c):
            mt = jnp.concatenate([mbuf[0]] * (W // 128), axis=1)
            mb = jnp.concatenate([mbuf[1]] * (W // 128), axis=1)
            ms = (mt, mt, mb, mb)
            a = _a_ops(*[jnp.exp2(sbuf[c, j] - ms[j]) for j in range(4)])
            return a, _hr(c * W, W)

        def rolled(t, carry):
            prev = None
            acc = [None] * 7
            for u in range(unroll):
                c = t * unroll + u
                a, kr = operands(c)
                for k in PVO:
                    m = _dot(a[k], _un(vops[b, k, kr, :]))
                    acc[k] = m if acc[k] is None else acc[k] + m
                prev = side(c, prev)
            O = _comb(acc)
            for q in PVQ:
                xr[qidx(i, q)] = xr[qidx(i, q)] + O[q]
            return carry

        if unroll >= NC:
            rolled(0, 0)
        else:
            lax.fori_loop(0, NC // unroll, rolled, 0)

    def front(hnops, wkv, xbuf, rawa, rawb, rawq, rawp1, rawp2, rawdw, xsem, wsem):
        def xcopy(t, slot):
            return pltpu.make_async_copy(x_hbm.at[pl.ds(pl.multiple_of(t * TM, 16), TM), :], xbuf.at[slot], xsem.at[slot])

        cp = [
            pltpu.make_async_copy(wq_h, rawq.at[0], wsem.at[0]),
            pltpu.make_async_copy(wk_h, rawq.at[1], wsem.at[1]),
            pltpu.make_async_copy(wv_h, rawq.at[2], wsem.at[2]),
            pltpu.make_async_copy(wo_h, rawq.at[3], wsem.at[3]),
            pltpu.make_async_copy(w1a_h, rawa, wsem.at[4]),
            pltpu.make_async_copy(w1b_h, rawb, wsem.at[5]),
            pltpu.make_async_copy(dw_h, rawdw, wsem.at[6]),
            pltpu.make_async_copy(wp1_h, rawp1, wsem.at[7]),
            pltpu.make_async_copy(wp2_h, rawp2, wsem.at[8]),
            pltpu.make_async_copy(w2a_h, rawa, wsem.at[9]),
            pltpu.make_async_copy(w2b_h, rawb, wsem.at[10]),
        ]
        CQ, CK, CV, CO, C1A, C1B, CDW, CP1, CP2, C2A, C2B = range(11)

        def stage_A(t, slot, chained=True):
            xs = t % 3

            def st(k, r, n, v):
                hnops[slot, k, _hrf(r, n), :] = _pkf(v)
            return ln_chain(lambda r, n: xbuf[xs, r:r + n, :].astype(f32), st, chained=chained, nch=LCH1)[1]

        def stage_B2(i, U):
            d = ff_down(U)
            xs = i % 3
            for q in DQORD:
                r0, c0 = (q // 2) * H, (q % 2) * Dh
                xr[qidx(i, q)] = xbuf[xs, r0:r0 + H, c0:c0 + Dh].astype(f32) + d[q]

        def p1(i, carry, dma=True):
            if dma:
                @pl.when(i + 1 < NT)
                def _():
                    xcopy(i + 1, (i + 1) % 3).wait()

                    @pl.when(i + 2 < NT)
                    def _():
                        xcopy(i + 2, (i + 2) % 3).start()
            U = ff_up(hnops, i % 2)
            prev = stage_A(jnp.minimum(i + 1, NT - 1), (i + 1) % 2)
            hq, _ = stage_C1(i - 1, prev)
            stage_B2(i, U)
            stage_C2(wkv, i - 1, hq)
            return carry

        if ONLY == 'p1':
            lax.fori_loop(1, NT, lambda i, c: p1(i, c, False), 0)
            return
        if ONLY not in (None, 'f0'):
            return
        cp[C1A].start()
        xcopy(0, 0).start()
        for b in range(B):
            for k in range(7):
                kops[b, k, TH // 2:, :] = jnp.zeros(((TP - TH) // 2, Dh), jnp.uint32)
                vops[b, k, TH // 2:, :] = jnp.zeros(((TP - TH) // 2, Dh), jnp.uint32)
        xcopy(0, 0).wait()
        cp[C1B].start()
        stage_A(0, 0, chained=False)
        cp[C1A].wait()
        build_b_ops(rawa, wa, 0, Dh, 0, F, 0.5, chained=False)
        early = (cp[CQ], cp[CK], cp[CV], cp[CO], xcopy(1, 1), cp[CDW])

        def mid_up():
            cp[C1B].wait()
            for c_ in early:
                c_.start()
            build_b_ops(rawb, wb, 0, F // 2, 0, D, 0.5)

        U = ff_up(hnops, 0, mid=(MIDUP, mid_up))
        for c_ in early:
            c_.wait()
        for c_ in (xcopy(2, 2), cp[CP1], cp[CP2]):
            c_.start()
        wf = _dot_nt(rawq[1], rawq[0])
        ops = _b_ops(wf[:Dh, :Dh], wf[:Dh, Dh:], wf[Dh:, :Dh], wf[Dh:, Dh:])
        for k in range(7):
            wkv[0, k] = _pkf(ops[k])
        wf = _dot(rawq[2], rawq[3])
        ops = _b_ops(wf[:Dh, :Dh], wf[:Dh, Dh:], wf[Dh:, :Dh], wf[Dh:, Dh:])
        for k in range(7):
            wkv[1, k] = _pkf(ops[k])
        stage_A(1, 1)
        stage_B2(0, U)
        dwv = rawdw[...].astype(f32)
        for k in range(K):
            for cb in range(4):
                dwb[k, cb] = jnp.broadcast_to(dwv[k:k + 1, cb * 128:(cb + 1) * 128], (8, 128))
        cp[C2A].start()
        cp[C2B].start()

        if ONLY == 'f0':
            for c_ in (xcopy(2, 2), cp[CP1], cp[CP2], cp[C2A], cp[C2B]):
                c_.wait()
            return
        with jax.named_scope("p1loop"):
            lax.fori_loop(1, P1END, p1, 0)

        cp[CP1].wait()
        cp[CP2].wait()
        cp[C2A].wait()
        cp[C2B].wait()

        def wops(c, prev):
            q = Dh // NC
            r0 = c * q if isinstance(c, int) else pl.multiple_of(c * q, 16)
            r1 = c * (F // 2 // NC) if isinstance(c, int) else pl.multiple_of(c * (F // 2 // NC), 16)
            prev = build_b_ops(rawp1, wp1.at[0], r0, q, 0, D, 0.5, prev=prev)
            prev = build_b_ops(rawp1, wp1.at[1], r0, q, D, D, 0.5, prev=prev)
            prev = build_b_ops(rawp2, wp2, r0, q, 0, D, 1.0, prev=prev)
            prev = build_b_ops(rawa, wa, r0, q, 0, F, 0.5, prev=prev)
            return build_b_ops(rawb, wb, r1, F // 2 // NC, 0, D, 0.5, prev=prev)

        with jax.named_scope("p2peel"):
            if PEEL_ROLL:
                att_qk(0, rolled=True)
                hq, _ = stage_C1(NT - 1, chained=False)
                stage_C2(wkv, NT - 1, hq)
                att_stats(PEEL_PCH, PEEL_PCH)
            else:
                hq, _ = stage_C1(NT - 1)
                att_qk(0)
                stage_C2(wkv, NT - 1, hq)
                att_stats()
            att_pv(0, wops, unroll=PEEL_UNROLL)

    V = pltpu.VMEM
    with jax.named_scope("front"):
        pl.run_scoped(front, VF((2, 7, H, Dh)), VF((2, 7, Dh, Dh)), V((3, TM, D), bf16), V((D, F), bf16), V((F, D), bf16), V((4, D, D), bf16),
                      V((D, 2 * D), bf16), V((D, D), bf16), V((K, D), bf16),
                      pltpu.SemaphoreType.DMA((3,)), pltpu.SemaphoreType.DMA((11,)))

    def back(dc, stats):
        def attention(gbuf):
            def stage_D1(j, chained=True):
                return ln_chain(lambda r, n: xr[rows(j, r, n), :], chained=chained, nch=LCHD)[0]

            def stage_D2(j, a):
                ga = _smm(lambda k: a[k], lambda k: _un(wp1[0, k]))
                gb_ = _smm(lambda k: a[k], lambda k: _un(wp1[1, k]))
                g = [_hglu(u, v) for u, v in zip(ga, gb_)]
                for q in QORD:
                    for t in range(2):
                        cb = 2 * (q % 2) + t
                        v = g[q][:, t * 128:(t + 1) * 128]
                        r0 = HALO + (q // 2) * H
                        gbuf[j % 2, cb, r0:r0 + H, :] = v
                        if q // 2 == 1:
                            gbuf[(j + 1) % 2, cb, 0:HALO, :] = v[H - HALO:H]

            class Conv:
                def __init__(self, j, cb, nch, head=None):
                    self.j, self.cb, self.nch = j, cb, nch
                    self.w = [dwb[k, cb] for k in range(K)]
                    self.prev = [head] * max(nch, 1)
                    self.shift = self.s1 = self.s2 = None
                    first = j % NTB == 0
                    self.lim = (jnp.where(first, HALO, 2 * HALO), jnp.where(first, HALO, 0))

                def step(self, n):
                    j, cb = self.j, self.cb
                    sub = lax.broadcasted_iota(jnp.int32, (8, 128), 0)
                    acc = None
                    for k in range(K):
                        i0 = 8 * n + k + 1
                        t = gbuf[j % 2, cb, pl.ds(i0, 8), :]
                        if n == 0 and i0 + 7 >= HALO:
                            t = jnp.where(sub + i0 < self.lim[0], t, 0.0)
                        if n == 1 and i0 < HALO:
                            t = jnp.where(sub + i0 >= self.lim[1], t, 0.0)
                        t = t * self.w[k]
                        if acc is None:
                            acc = tie(self.prev[n % self.nch], t) if self.nch else t
                        else:
                            acc = acc + t
                    dc[cb, pl.ds(pl.multiple_of(j * TM + 8 * n, 8), 8), :] = acc
                    if self.nch:
                        self.prev[n % self.nch] = acc
                    return acc

                def run(self):
                    j, cb = self.j, self.cb
                    ns = TM // 8
                    shift = self.step(1)
                    s1 = s2 = None
                    for n in [0] + list(range(2, ns)):
                        d = self.step(n) - shift
                        if n == 0:
                            d = jnp.where(j > 0, d, 0.0)
                        s1 = d if s1 is None else s1 + d
                        s2 = d * d if s2 is None else s2 + d * d
                    inv = jnp.where(j > 0, 1.0 / ns, 1.0 / (ns - 1))
                    js = pl.ds(pl.multiple_of(j * 8, 8), 8)
                    stats[0, cb, js, :] = shift + s1 * inv
                    stats[1, cb, js, :] = s2 - s1 * s1 * inv
                    return self.prev[-1]

            for cb in range(4):
                gbuf[0, cb, 0:HALO, :] = jnp.zeros((HALO, 128), f32)
                gbuf[1, cb, HALO:2 * HALO, :] = jnp.zeros((HALO, 128), f32)

            def p2(i, carry):
                a = stage_D1(i - 1)
                att_qk(i)
                stage_D2(i - 1, a)
                att_stats()
                att_pv(i, lambda c, prev: Conv(i - 1, c, ECH, prev).run(), PVU)
                return carry

            if ONLY in ('p1', 'p4', 'f0', 't0'):
                return
            if ONLY != 'e0':
                with jax.named_scope("p2loop"):
                    lax.fori_loop(1, P2END, p2, 0)
            if ONLY not in (None, 'e0'):
                return

            stage_D2(NT - 1, stage_D1(NT - 1, chained=False))
            for cb in range(4):
                Conv(NT - 1, cb, EPI_LAST).run()
                acc = Conv(NT, cb, 0).step(0)
                stats[0, cb, 8 * NT:8 * NT + 8, :] = acc
                stats[1, cb, 8 * NT:8 * NT + 8, :] = jnp.zeros((8, 128), f32)

        pl.run_scoped(attention, V((2, 4, TM + HALO, 128), f32))

        st0 = jnp.concatenate([stats[0, cb] for cb in range(4)], axis=1)
        st1 = jnp.concatenate([stats[1, cb] for cb in range(4)], axis=1)
        grow = lax.broadcasted_iota(jnp.int32, st0.shape, 0)
        cnt = jnp.where(grow < 8, TM // 8 - 1, jnp.where(grow < 8 * NT, TM // 8, 1)).astype(f32)
        mu = jnp.sum(cnt * st0, axis=0, keepdims=True) * (1.0 / N)
        dm = st0 - mu
        var = jnp.sum(st1 + cnt * dm * dm, axis=0, keepdims=True) * (1.0 / N)
        rsd = 0.5 * lax.rsqrt(var + EPS)

        def final(hnops, zops, obuf, osem):
            def ocopy(t, slot):
                return pltpu.make_async_copy(obuf.at[slot], out_hbm.at[pl.ds(pl.multiple_of(t * TM, 16), TM), :], osem.at[slot])

            def stage_F1(j, prev=None, chained=True, nch=1):
                def zq(r0, n, hi):
                    rr = pl.ds(pl.multiple_of(j * TM + 8 + r0, 8), n)
                    d = jnp.concatenate([dc[2 * hi + t, rr, :] for t in range(2)], axis=1)
                    return (d - mu[:, hi * Dh:(hi + 1) * Dh]) * rsd[:, hi * Dh:(hi + 1) * Dh]
                if not chained:
                    return _a_ops(*[_hsilu(zq(r0, H, hi)) for r0 in (0, H) for hi in (0, 1)])
                heads = [prev] * nch
                for r in range(0, H, 16):
                    z = []
                    for r0 in (0, H):
                        for hi in (0, 1):
                            ch = (2 * (r0 // H) + hi) % nch
                            t = _hsilu(tie0(heads[ch], zq(r0 + r, 16, hi)))
                            heads[ch] = t[:, :128] + t[:, 128:]
                            z.append(t)
                    for k, o in enumerate(_a_ops(*z)):
                        zops[k, _hrf(r, 16), :] = _pkf(o)
                return functools.reduce(jnp.add, heads)

            def stage_F2(j, a=None):
                E = _smm((lambda k: _unf(zops[k])) if a is None else (lambda k: a[k]), lambda k: _unf(wp2[k]))
                for q in QORD:
                    xr[qidx(j, q)] = xr[qidx(j, q)] + E[q]

            def stage_F3(j, slot, prev=None, nch=None):
                def st(k, r, n, v):
                    hnops[slot, k, _hrf(r, n), :] = _pkf(v)
                return ln_chain(lambda r, n: xr[rows(j, r, n), :], st, prev, nch=nch or LCH4)[1]

            def stage_G2(i, U):
                d = ff_down(U)
                for q in DQORD:
                    xr[qidx(i, q)] = xr[qidx(i, q)] + d[q]

            def stage_Hh(j, chained=True):
                slot = j % 2
                if not chained:
                    obuf[slot, 0:H, :] = _ln(xr[rows(j), :]).astype(bf16)
                    obuf[slot, H:TM, :] = _ln(xr[rows(j, H), :]).astype(bf16)
                    return None
                heads = [None] * HCH
                for n, r in enumerate(range(0, TM, HG)):
                    y = _ln(tie0(heads[n % HCH], xr[rows(j, r, HG), :]))
                    prev = heads[n % HCH] = y[:, :128]
                    obuf[slot, r:r + HG, :] = y.astype(bf16)
                return prev

            if ONLY in ('p1', 'p2', 'f0'):
                return
            if ONLY in (None, 'e0'):
                stage_F2(0, stage_F1(0, chained=False))
                stage_F3(0, 0, stage_F1(1, nch=EPI_F1), nch=EPI_LN)

            def p4(i, carry):
                if ONLY is None:
                    @pl.when(i >= 3)
                    def _():
                        ocopy(i - 3, (i - 3) % 2).wait()
                stage_F2(i + 1)
                U = ff_up(hnops, i % 2)
                prev = stage_Hh(jnp.maximum(i - 1, 0))
                prev = stage_F3(i + 1, (i + 1) % 2, prev[0:16] if LINK & 1 else None)
                stage_F1(jnp.minimum(i + 2, NT - 1), prev if LINK & 2 else None)
                stage_G2(i, U)

                if ONLY is None:
                    @pl.when(i >= 1)
                    def _():
                        ocopy(i - 1, (i - 1) % 2).start()
                return carry

            if ONLY == 'e0':
                for src in (hnops.at[0], zops):
                    c_ = pltpu.make_async_copy(src, hnops.at[1], osem.at[0])
                    c_.start()
                    c_.wait()
                ocopy(0, 0).start()
                ocopy(0, 0).wait()
                return
            if ONLY != 't0':
                with jax.named_scope("p4loop"):
                    lax.fori_loop(0, P4END, p4, 0)
            if ONLY not in (None, 't0'):
                return

            ocopy(NT - 4, (NT - 4) % 2).wait()
            ocopy(NT - 3, (NT - 3) % 2).wait()
            U = ff_up(hnops, (NT - 1) % 2)
            stage_Hh(NT - 2)
            d = ff_down(U)
            slot = (NT - 1) % 2
            last = [ocopy(NT - 2, (NT - 2) % 2)]
            for half in range(2):
                x4 = cat(*[xr[qidx(NT - 1, 2 * half + t)] + d[2 * half + t] for t in range(2)])
                obuf[slot, half * H:(half + 1) * H, :] = _ln(x4).astype(bf16)
                last.append(pltpu.make_async_copy(obuf.at[slot, half * H:(half + 1) * H, :],
                                                  out_hbm.at[pl.ds((NT - 1) * TM + half * H, H), :], osem.at[1 + half]))
                if half == 0:
                    last[0].start()
                last[-1].start()
            for c_ in last:
                c_.wait()

        pl.run_scoped(final, VF((2, 7, H, Dh)), VF((7, H, Dh)), V((2, TM, D), bf16),
                      pltpu.SemaphoreType.DMA((3,)))

    with jax.named_scope("back"):
        pl.run_scoped(back, V((4, N + 8, 128), f32), V((2, 4, 8 * NT + 8, 128), f32))


@jax.jit
def pallas_standalone__conformer_family_conformer__speech_kernel(
    x, w_ff1_a, w_ff1_b, w_q, w_k, w_v, w_o, w_pw1, dw, w_pw2, w_ff2_a, w_ff2_b):
    B, T, D = x.shape
    K = dw.shape[0]
    F = w_ff1_a.shape[1]
    N = B * T
    TM = 2 * H
    NT = N // TM
    TP = (T // 2 + 127) // 128 * 128
    Dh = D // 2
    kern = functools.partial(_kernel, B=B, T=T, D=D, K=K, F=F)
    hbm = pl.BlockSpec(memory_space=pl.ANY)
    V = pltpu.VMEM
    out = pl.pallas_call(
        kern,
        out_shape=jax.ShapeDtypeStruct((N, D), x.dtype),
        in_specs=[hbm] * 12,
        out_specs=hbm,
        scratch_shapes=[
            V((N, D), f32),
            V((NT, 7, H // 2, Dh), u32),
            V((B, 7, TP // 2, Dh), u32),
            V((B, 7, TP // 2, Dh), u32),
            VF((7, Dh, F // 2)),
            VF((7, F // 2, Dh)),
            V((2, 7, Dh // 2, Dh), u32),
            VF((7, Dh, Dh)),
            V((K, 4, 8, 128), f32),
            V((TP // W, 4, H, W), f32),
            V((2, H, 128), f32),
            V((2, TP // W - 1, 2, H, 128), f32),
            V((8, 128), jnp.int32),
            V((8, 128), jnp.int32),
            pltpu.SemaphoreType.DMA(()),
        ],
        compiler_params=pltpu.CompilerParams(vmem_limit_bytes=VMEM_LIMIT),
    )(x.reshape(N, D), w_ff1_a, w_ff1_b, w_q, w_k, w_v, w_o, w_pw1, dw, w_pw2, w_ff2_a, w_ff2_b)
    return out.reshape(B, T, D)
```

```python
import functools
import jax
import jax.numpy as jnp
from jax import lax
import jax.experimental.pallas as pl
import jax.experimental.pallas.tpu as pltpu

H = 400
W = 512
HALO = 16
EPS = 1e-5
LOG2E = 1.4426950408889634
NEG = -1e30
UPO = (1, 2, 0, 5, 3, 4, 6)
DNO = (1, 3, 6, 0, 2, 4, 5)
QORD = (3, 2, 1, 0)
DQORD = (2, 0, 1, 3)
PR = 40
PCH, PCHF = 3, 8
PVU = 2
HG = 32
VMEM_LIMIT = 127 * 1024 * 1024

bf16 = jnp.bfloat16
f32 = jnp.float32
u32 = jnp.uint32


def _ln(x):
    m = jnp.mean(x, axis=-1, keepdims=True)
    c = x - m
    v = jnp.mean(c * c, axis=-1, keepdims=True)
    return c * lax.rsqrt(v + EPS)


def _hsilu(h):
    return h * jnp.tanh(h) + h


def _hglu(a, b):
    return a * jnp.tanh(b) + a


def _dot(a, b):
    return jnp.dot(a, b, preferred_element_type=f32)


def _dot_nt(a, b):
    return lax.dot_general(a, b, (((1,), (1,)), ((), ())), preferred_element_type=f32)


def _a_sums(A11, A12, A21, A22):
    return [A11 + A22, A21 + A22, A11, A22, A11 + A12, A21 - A11, A12 - A22]


def _a_ops(*q):
    return [t.astype(bf16) for t in _a_sums(*q)]


def _b_ops(B11, B12, B21, B22):
    return [t.astype(bf16) for t in
            (B11 + B22, B11, B12 - B22, B21 - B11, B22, B11 + B12, B21 + B22)]


def _smm(a, w, order=UPO, dot=_dot, mid=None):
    M = [None] * 7
    for n, k in enumerate(order):
        if mid is not None and n == mid[0]:
            mid[1]()
        M[k] = dot(a(k), w(k))
    return _comb(M)


def _comb(M):
    return (M[0] + M[3] - M[4] + M[6], M[2] + M[4], M[1] + M[3], M[0] - M[1] + M[2] + M[5])


def _pk(v):
    return pltpu.bitcast(v, jnp.uint32)


def _un(v):
    return pltpu.bitcast(v, bf16)


def _hr(r0, n):
    h = r0 // 2
    return pl.ds(h if isinstance(h, int) else pl.multiple_of(h, 8), n // 2)


def _cat(a, b):
    return jnp.concatenate([a, b], axis=1)


def _kernel(x_hbm, w1a_h, w1b_h, wq_h, wk_h, wv_h, wo_h, wp1_h, dw_h, wp2_h, w2a_h, w2b_h, out_hbm,
            xr, hops, kops, vops, wa, wb, wp1, wp2, dwb, sbuf, mbuf, cstat, zsrc, zref, zsem, *, B, T, D, K, F):
    N = B * T
    TM = 2 * H
    NTB = T // TM
    NT = B * NTB
    TH = T // 2
    TP = 2 * kops.shape[2]
    NC = TP // W
    Dh = D // 2
    cat = _cat
    ident = tuple(range(7))

    zsrc[...] = jnp.zeros_like(zsrc)
    zcopy = pltpu.make_async_copy(zsrc, zref, zsem)
    zcopy.start()
    zcopy.wait()

    def tie(prev, v):
        if prev is None:
            return v
        never = jnp.tile(zref[0:8, :], (v.shape[0] // 8, 1)) != 0
        return jnp.where(never, prev, v)

    def tie0(prev, v):
        return v if prev is None else cat(tie(prev, v[:, :128]), v[:, 128:])

    def al16(v):
        return v if isinstance(v, int) else pl.multiple_of(v, 16)

    def rows(i, off=0, n=H):
        return pl.ds(al16(i * TM + off), n)

    def ln_chain(load, store=None, prev=None, chained=True, nch=1):
        if not chained:
            ht, hb = _ln(load(0, H)), _ln(load(H, H))
            ops = _a_ops(ht[:, :Dh], ht[:, Dh:], hb[:, :Dh], hb[:, Dh:])
            if store is not None:
                for k in range(7):
                    store(k, 0, H, ops[k])
            return ops, None
        outs = [[] for _ in range(7)]
        heads = [prev] * nch
        for n, r in enumerate(range(0, H, 16)):
            ht, hb = _ln(tie0(heads[n % nch], load(r, 16))), _ln(load(H + r, 16))
            s = _a_sums(ht[:, :Dh], ht[:, Dh:], hb[:, :Dh], hb[:, Dh:])
            prev = heads[n % nch] = s[0][:, :128]
            for k in range(7):
                o = s[k].astype(bf16)
                outs[k].append(o)
                if store is not None:
                    store(k, r, 16, o)
        return [jnp.concatenate(o, axis=0) for o in outs], prev

    def chained(fn, x, pr):
        prev = None
        cols = []
        for t in range(x.shape[1] // 128):
            parts = []
            for r in range(0, x.shape[0], pr):
                prev = fn(tie(prev, x[r:r + pr, t * 128:(t + 1) * 128]))
                parts.append(prev)
            cols.append(jnp.concatenate(parts, axis=0))
        return jnp.concatenate(cols, axis=1)

    def build_b_ops(raw, dst, r0, nr, c0, n, scale, chained=True, prev=None):
        k = raw.shape[0] // 2
        nh = n // 2
        n_ = 0
        for r in range(0, nr, 16):
            for c in range(0, nh, 128):
                def blk(ro, co):
                    return raw[pl.ds(al16(ro + r0 + r), 16), c0 + co + c:c0 + co + c + 128].astype(f32) * scale
                B11, B12, B21, B22 = tie(prev if chained else None, blk(0, 0)), blk(0, nh), blk(k, 0), blk(k, nh)
                n_ += 1
                if n_ % 2 == 0:
                    prev = jnp.broadcast_to(jnp.max((B11 + B12) + (B21 + B22), axis=-1, keepdims=True), (16, 128))
                ops = _b_ops(B11, B12, B21, B22)
                for i in range(7):
                    if dst.dtype == u32:
                        dst[i, _hr(r0 + r, 16), c:c + 128] = _pk(ops[i])
                    else:
                        dst[i, pl.ds(al16(r0 + r), 16), c:c + 128] = ops[i]
        return prev

    def qidx(i, q):
        return rows(i, (q // 2) * H), slice((q % 2) * Dh, (q % 2 + 1) * Dh)

    def ff_up(hnops, slot, mid=None):
        C = _smm(lambda k: hnops[slot, k], lambda k: wa[k], UPO, mid=mid)
        return [chained(_hsilu, C[q], PR) for q in range(4)]

    def ff_down(U):
        a = _a_ops(*U)
        return _smm(lambda k: a[k], lambda k: wb[k], DNO)

    def stage_C1(i, prev=None, chained=True):
        def st(k, r, n, v):
            hops[i, k, _hr(r, n), :] = _pk(v)
        return ln_chain(lambda r, n: xr[rows(i, r, n), :], st, prev, chained=chained, nch=2)

    def stage_C2(wkv, i, a):
        b = i // NTB
        r = _hr((i % NTB) * H, H)
        c = D ** -0.5 * LOG2E
        ktl, kth, kbl, kbh = [t * c for t in _smm(lambda k: a[k], lambda k: wkv[0, k])]
        ops = _b_ops(ktl, kbl, kth, kbh)
        for k in range(7):
            kops[b, k, r, :] = _pk(ops[k])
        vtl, vth, vbl, vbh = _smm(lambda k: a[k], lambda k: wkv[1, k])
        ops = _b_ops(vtl, vth, vbl, vbh)
        for k in range(7):
            vops[b, k, r, :] = _pk(ops[k])

    def att_qk(i):
        b = i // NTB

        def chunk(c):
            kr = _hr(c * W, W)
            s = list(_smm(lambda k: _un(hops[i, k]), lambda k: _un(kops[b, k, kr, :]), ident, _dot_nt))
            nv = TH - c * W
            for j in range(4):
                t = s[j]
                if nv < W:
                    lo = nv // 128 * 128
                    col = lax.broadcasted_iota(jnp.int32, (H, W - lo), 1)
                    t = cat(t[:, :lo], jnp.where(col < nv - lo, t[:, lo:], NEG))
                sbuf[c, j] = t

        for c in range(NC):
            chunk(c)

    def att_stats():
        prev = [None] * PCH
        n = 0
        for c in range(NC):
            if c == NC - 1:
                prev = [prev[t % PCH] for t in range(PCHF)]
            nch = len(prev)
            for r in range(0, H, 8):
                for half in range(2):
                    rs = slice(r, r + 8)
                    blocks = [sbuf[c, 2 * half + j, rs, t * 128:(t + 1) * 128]
                              for j in (0, 1) for t in range(W // 128)]
                    blocks[0] = tie(prev[n % nch], blocks[0])
                    m = jnp.broadcast_to(
                        jnp.max(functools.reduce(jnp.maximum, blocks), axis=-1, keepdims=True), (8, 128))
                    if c < NC - 1:
                        l = functools.reduce(jnp.add, [jnp.exp2(t - m) for t in blocks])
                        cstat[0, c, half, rs, :] = m
                        cstat[1, c, half, rs, :] = l
                        prev[n % nch] = l
                    else:
                        ms = [cstat[0, cc, half, rs, :] for cc in range(NC - 1)]
                        m = functools.reduce(jnp.maximum, ms + [m])
                        l = functools.reduce(jnp.add, [jnp.exp2(t - m) for t in blocks]
                                             + [cstat[1, cc, half, rs, :] * jnp.exp2(ms[cc] - m) for cc in range(NC - 1)])
                        mp = m + jnp.log2(jnp.sum(l, axis=-1, keepdims=True))
                        mbuf[half, rs, :] = mp
                        prev[n % nch] = mp
                    n += 1

    def att_pv(i, side, unroll=1):
        b = i // NTB

        def operands(c):
            mt = jnp.concatenate([mbuf[0]] * (W // 128), axis=1)
            mb = jnp.concatenate([mbuf[1]] * (W // 128), axis=1)
            ms = (mt, mt, mb, mb)
            a = _a_ops(*[jnp.exp2(sbuf[c, j] - ms[j]) for j in range(4)])
            return a, _hr(c * W, W)

        def rolled(t, carry):
            prev = None
            acc = [None] * 7
            for u in range(unroll):
                c = t * unroll + u
                a, kr = operands(c)
                for k in DNO:
                    m = _dot(a[k], _un(vops[b, k, kr, :]))
                    acc[k] = m if acc[k] is None else acc[k] + m
                prev = side(c, prev)
            O = _comb(acc)
            for q in DQORD:
                xr[qidx(i, q)] = xr[qidx(i, q)] + O[q]
            return carry

        if unroll >= NC:
            rolled(0, 0)
        else:
            lax.fori_loop(0, NC // unroll, rolled, 0)

    def front(hnops, wkv, xbuf, rawa, rawb, rawq, rawp1, rawp2, rawdw, xsem, wsem):
        def xcopy(t, slot):
            return pltpu.make_async_copy(x_hbm.at[pl.ds(pl.multiple_of(t * TM, 16), TM), :], xbuf.at[slot], xsem.at[slot])

        cp = [
            pltpu.make_async_copy(wq_h, rawq.at[0], wsem.at[0]),
            pltpu.make_async_copy(wk_h, rawq.at[1], wsem.at[1]),
            pltpu.make_async_copy(wv_h, rawq.at[2], wsem.at[2]),
            pltpu.make_async_copy(wo_h, rawq.at[3], wsem.at[3]),
            pltpu.make_async_copy(w1a_h, rawa, wsem.at[4]),
            pltpu.make_async_copy(w1b_h, rawb, wsem.at[5]),
            pltpu.make_async_copy(dw_h, rawdw, wsem.at[6]),
            pltpu.make_async_copy(wp1_h, rawp1, wsem.at[7]),
            pltpu.make_async_copy(wp2_h, rawp2, wsem.at[8]),
            pltpu.make_async_copy(w2a_h, rawa, wsem.at[9]),
            pltpu.make_async_copy(w2b_h, rawb, wsem.at[10]),
        ]
        CQ, CK, CV, CO, C1A, C1B, CDW, CP1, CP2, C2A, C2B = range(11)

        def stage_A(t, slot, chained=True):
            xs = t % 3

            def st(k, r, n, v):
                hnops[slot, k, r:r + n, :] = v
            return ln_chain(lambda r, n: xbuf[xs, r:r + n, :].astype(f32), st, chained=chained, nch=2)[1]

        def stage_B2(i, U):
            d = ff_down(U)
            xs = i % 3
            for q in DQORD:
                r0, c0 = (q // 2) * H, (q % 2) * Dh
                xr[qidx(i, q)] = xbuf[xs, r0:r0 + H, c0:c0 + Dh].astype(f32) + d[q]

        def p1(i, carry):
            @pl.when(i + 1 < NT)
            def _():
                xcopy(i + 1, (i + 1) % 3).wait()

                @pl.when(i + 2 < NT)
                def _():
                    xcopy(i + 2, (i + 2) % 3).start()
            U = ff_up(hnops, i % 2)
            prev = stage_A(jnp.minimum(i + 1, NT - 1), (i + 1) % 2)
            hq, _ = stage_C1(i - 1, prev)
            stage_B2(i, U)
            stage_C2(wkv, i - 1, hq)
            return carry


        cp[C1A].start()
        xcopy(0, 0).start()
        for b in range(B):
            for k in range(7):
                kops[b, k, TH // 2:, :] = jnp.zeros(((TP - TH) // 2, Dh), jnp.uint32)
                vops[b, k, TH // 2:, :] = jnp.zeros(((TP - TH) // 2, Dh), jnp.uint32)
        xcopy(0, 0).wait()
        cp[C1B].start()
        stage_A(0, 0, chained=False)
        cp[C1A].wait()
        build_b_ops(rawa, wa, 0, Dh, 0, F, 0.5, chained=False)
        early = (cp[CQ], cp[CK], cp[CV], cp[CO], xcopy(1, 1), cp[CDW])

        def mid_up():
            cp[C1B].wait()
            for c_ in early:
                c_.start()
            build_b_ops(rawb, wb, 0, F // 2, 0, D, 0.5)

        U = ff_up(hnops, 0, mid=(2, mid_up))
        for c_ in early:
            c_.wait()
        for c_ in (xcopy(2, 2), cp[CP1], cp[CP2]):
            c_.start()
        wf = _dot_nt(rawq[1], rawq[0])
        ops = _b_ops(wf[:Dh, :Dh], wf[:Dh, Dh:], wf[Dh:, :Dh], wf[Dh:, Dh:])
        for k in range(7):
            wkv[0, k] = ops[k]
        wf = _dot(rawq[2], rawq[3])
        ops = _b_ops(wf[:Dh, :Dh], wf[:Dh, Dh:], wf[Dh:, :Dh], wf[Dh:, Dh:])
        for k in range(7):
            wkv[1, k] = ops[k]
        stage_A(1, 1)
        stage_B2(0, U)
        dwv = rawdw[...].astype(f32)
        for k in range(K):
            for cb in range(4):
                dwb[k, cb] = jnp.broadcast_to(dwv[k:k + 1, cb * 128:(cb + 1) * 128], (8, 128))
        cp[C2A].start()
        cp[C2B].start()

        with jax.named_scope("p1loop"):
            lax.fori_loop(1, NT, p1, 0)

        cp[CP1].wait()
        cp[CP2].wait()
        cp[C2A].wait()
        cp[C2B].wait()

        def wops(c, prev):
            q = Dh // NC
            r0 = c * q if isinstance(c, int) else pl.multiple_of(c * q, 16)
            r1 = c * (F // 2 // NC) if isinstance(c, int) else pl.multiple_of(c * (F // 2 // NC), 16)
            prev = build_b_ops(rawp1, wp1.at[0], r0, q, 0, D, 0.5, prev=prev)
            prev = build_b_ops(rawp1, wp1.at[1], r0, q, D, D, 0.5, prev=prev)
            prev = build_b_ops(rawp2, wp2, r0, q, 0, D, 1.0, prev=prev)
            prev = build_b_ops(rawa, wa, r0, q, 0, F, 0.5, prev=prev)
            return build_b_ops(rawb, wb, r1, F // 2 // NC, 0, D, 0.5, prev=prev)

        with jax.named_scope("p2peel"):
            hq, _ = stage_C1(NT - 1)
            att_qk(0)
            stage_C2(wkv, NT - 1, hq)
            att_stats()
            att_pv(0, wops, unroll=PVU)

    V = pltpu.VMEM
    with jax.named_scope("front"):
        pl.run_scoped(front, V((2, 7, H, Dh), bf16), V((2, 7, Dh, Dh), bf16), V((3, TM, D), bf16), V((D, F), bf16), V((F, D), bf16), V((4, D, D), bf16),
                      V((D, 2 * D), bf16), V((D, D), bf16), V((K, D), bf16),
                      pltpu.SemaphoreType.DMA((3,)), pltpu.SemaphoreType.DMA((11,)))

    def back(dc, stats):
        def attention(gbuf):
            def stage_D1(j, chained=True):
                return ln_chain(lambda r, n: xr[rows(j, r, n), :], chained=chained)[0]

            def stage_D2(j, a):
                ga = _smm(lambda k: a[k], lambda k: _un(wp1[0, k]))
                gb_ = _smm(lambda k: a[k], lambda k: _un(wp1[1, k]))
                g = [_hglu(u, v) for u, v in zip(ga, gb_)]
                for q in QORD:
                    for t in range(2):
                        cb = 2 * (q % 2) + t
                        v = g[q][:, t * 128:(t + 1) * 128]
                        r0 = HALO + (q // 2) * H
                        gbuf[j % 2, cb, r0:r0 + H, :] = v
                        if q // 2 == 1:
                            gbuf[(j + 1) % 2, cb, 0:HALO, :] = v[H - HALO:H]

            class Conv:
                def __init__(self, j, cb, nch, head=None):
                    self.j, self.cb, self.nch = j, cb, nch
                    self.w = [dwb[k, cb] for k in range(K)]
                    self.prev = [head] * max(nch, 1)
                    self.shift = self.s1 = self.s2 = None
                    first = j % NTB == 0
                    self.lim = (jnp.where(first, HALO, 2 * HALO), jnp.where(first, HALO, 0))

                def step(self, n):
                    j, cb = self.j, self.cb
                    sub = lax.broadcasted_iota(jnp.int32, (8, 128), 0)
                    acc = None
                    for k in range(K):
                        i0 = 8 * n + k + 1
                        t = gbuf[j % 2, cb, pl.ds(i0, 8), :]
                        if n == 0 and i0 + 7 >= HALO:
                            t = jnp.where(sub + i0 < self.lim[0], t, 0.0)
                        if n == 1 and i0 < HALO:
                            t = jnp.where(sub + i0 >= self.lim[1], t, 0.0)
                        t = t * self.w[k]
                        if acc is None:
                            acc = tie(self.prev[n % self.nch], t) if self.nch else t
                        else:
                            acc = acc + t
                    dc[cb, pl.ds(pl.multiple_of(j * TM + 8 * n, 8), 8), :] = acc
                    if self.nch:
                        self.prev[n % self.nch] = acc
                    return acc

                def run(self):
                    j, cb = self.j, self.cb
                    ns = TM // 8
                    shift = self.step(1)
                    s1 = s2 = None
                    for n in [0] + list(range(2, ns)):
                        d = self.step(n) - shift
                        if n == 0:
                            d = jnp.where(j > 0, d, 0.0)
                        s1 = d if s1 is None else s1 + d
                        s2 = d * d if s2 is None else s2 + d * d
                    inv = jnp.where(j > 0, 1.0 / ns, 1.0 / (ns - 1))
                    js = pl.ds(pl.multiple_of(j * 8, 8), 8)
                    stats[0, cb, js, :] = shift + s1 * inv
                    stats[1, cb, js, :] = s2 - s1 * s1 * inv
                    return self.prev[-1]

            for cb in range(4):
                gbuf[0, cb, 0:HALO, :] = jnp.zeros((HALO, 128), f32)
                gbuf[1, cb, HALO:2 * HALO, :] = jnp.zeros((HALO, 128), f32)

            def p2(i, carry):
                a = stage_D1(i - 1)
                att_qk(i)
                stage_D2(i - 1, a)
                att_stats()
                att_pv(i, lambda c, prev: Conv(i - 1, c, 1, prev).run(), PVU)
                return carry

            with jax.named_scope("p2loop"):
                lax.fori_loop(1, NT, p2, 0)

            stage_D2(NT - 1, stage_D1(NT - 1, chained=False))
            for cb in range(4):
                Conv(NT - 1, cb, 0).run()
                acc = Conv(NT, cb, 0).step(0)
                stats[0, cb, 8 * NT:8 * NT + 8, :] = acc
                stats[1, cb, 8 * NT:8 * NT + 8, :] = jnp.zeros((8, 128), f32)

        pl.run_scoped(attention, V((2, 4, TM + HALO, 128), f32))

        st0 = jnp.concatenate([stats[0, cb] for cb in range(4)], axis=1)
        st1 = jnp.concatenate([stats[1, cb] for cb in range(4)], axis=1)
        grow = lax.broadcasted_iota(jnp.int32, st0.shape, 0)
        cnt = jnp.where(grow < 8, TM // 8 - 1, jnp.where(grow < 8 * NT, TM // 8, 1)).astype(f32)
        mu = jnp.sum(cnt * st0, axis=0, keepdims=True) * (1.0 / N)
        dm = st0 - mu
        var = jnp.sum(st1 + cnt * dm * dm, axis=0, keepdims=True) * (1.0 / N)
        rsd = 0.5 * lax.rsqrt(var + EPS)

        def final(hnops, zops, obuf, osem):
            def ocopy(t, slot):
                return pltpu.make_async_copy(obuf.at[slot], out_hbm.at[pl.ds(pl.multiple_of(t * TM, 16), TM), :], osem.at[slot])

            def stage_F1(j, prev=None, chained=True, nch=1):
                def zq(r0, n, hi):
                    rr = pl.ds(pl.multiple_of(j * TM + 8 + r0, 8), n)
                    d = jnp.concatenate([dc[2 * hi + t, rr, :] for t in range(2)], axis=1)
                    return (d - mu[:, hi * Dh:(hi + 1) * Dh]) * rsd[:, hi * Dh:(hi + 1) * Dh]
                if not chained:
                    return _a_ops(*[_hsilu(zq(r0, H, hi)) for r0 in (0, H) for hi in (0, 1)])
                heads = [prev] * nch
                for r in range(0, H, 16):
                    z = []
                    for r0 in (0, H):
                        for hi in (0, 1):
                            ch = (2 * (r0 // H) + hi) % nch
                            t = _hsilu(tie0(heads[ch], zq(r0 + r, 16, hi)))
                            heads[ch] = t[:, :128] + t[:, 128:]
                            z.append(t)
                    for k, o in enumerate(_a_ops(*z)):
                        zops[k, r:r + 16, :] = o
                return functools.reduce(jnp.add, heads)

            def stage_F2(j, a=None):
                E = _smm((lambda k: zops[k]) if a is None else (lambda k: a[k]), lambda k: wp2[k])
                for q in QORD:
                    xr[qidx(j, q)] = xr[qidx(j, q)] + E[q]

            def stage_F3(j, slot, prev=None, nch=2):
                def st(k, r, n, v):
                    hnops[slot, k, r:r + n, :] = v
                return ln_chain(lambda r, n: xr[rows(j, r, n), :], st, prev, nch=nch)[1]

            def stage_G2(i, U):
                d = ff_down(U)
                for q in DQORD:
                    xr[qidx(i, q)] = xr[qidx(i, q)] + d[q]

            def stage_Hh(j, chained=True):
                slot = j % 2
                if not chained:
                    obuf[slot, 0:H, :] = _ln(xr[rows(j), :]).astype(bf16)
                    obuf[slot, H:TM, :] = _ln(xr[rows(j, H), :]).astype(bf16)
                    return None
                prev = None
                for r in range(0, TM, HG):
                    y = _ln(tie0(prev, xr[rows(j, r, HG), :]))
                    prev = y[:, :128]
                    obuf[slot, r:r + HG, :] = y.astype(bf16)
                return prev

            stage_F2(0, stage_F1(0, chained=False))
            stage_F3(0, 0, stage_F1(1, nch=4), nch=25)

            def p4(i, carry):
                @pl.when(i >= 3)
                def _():
                    ocopy(i - 3, (i - 3) % 2).wait()
                stage_F2(i + 1)
                U = ff_up(hnops, i % 2)
                prev = stage_Hh(jnp.maximum(i - 1, 0))
                stage_F3(i + 1, (i + 1) % 2, prev[0:16])
                stage_F1(jnp.minimum(i + 2, NT - 1))
                stage_G2(i, U)

                @pl.when(i >= 1)
                def _():
                    ocopy(i - 1, (i - 1) % 2).start()
                return carry

            with jax.named_scope("p4loop"):
                lax.fori_loop(0, NT - 1, p4, 0)

            ocopy(NT - 4, (NT - 4) % 2).wait()
            ocopy(NT - 3, (NT - 3) % 2).wait()
            U = ff_up(hnops, (NT - 1) % 2)
            stage_Hh(NT - 2)
            d = ff_down(U)
            slot = (NT - 1) % 2
            last = [ocopy(NT - 2, (NT - 2) % 2)]
            for half in range(2):
                x4 = cat(*[xr[qidx(NT - 1, 2 * half + t)] + d[2 * half + t] for t in range(2)])
                obuf[slot, half * H:(half + 1) * H, :] = _ln(x4).astype(bf16)
                last.append(pltpu.make_async_copy(obuf.at[slot, half * H:(half + 1) * H, :],
                                                  out_hbm.at[pl.ds((NT - 1) * TM + half * H, H), :], osem.at[1 + half]))
                if half == 0:
                    last[0].start()
                last[-1].start()
            for c_ in last:
                c_.wait()

        pl.run_scoped(final, V((2, 7, H, Dh), bf16), V((7, H, Dh), bf16), V((2, TM, D), bf16),
                      pltpu.SemaphoreType.DMA((3,)))

    with jax.named_scope("back"):
        pl.run_scoped(back, V((4, N + 8, 128), f32), V((2, 4, 8 * NT + 8, 128), f32))


@jax.jit
def pallas_standalone__conformer_family_conformer__speech_kernel(
    x, w_ff1_a, w_ff1_b, w_q, w_k, w_v, w_o, w_pw1, dw, w_pw2, w_ff2_a, w_ff2_b):
    B, T, D = x.shape
    K = dw.shape[0]
    F = w_ff1_a.shape[1]
    N = B * T
    TM = 2 * H
    NT = N // TM
    TP = (T // 2 + 127) // 128 * 128
    Dh = D // 2
    kern = functools.partial(_kernel, B=B, T=T, D=D, K=K, F=F)
    hbm = pl.BlockSpec(memory_space=pl.ANY)
    V = pltpu.VMEM
    out = pl.pallas_call(
        kern,
        out_shape=jax.ShapeDtypeStruct((N, D), x.dtype),
        in_specs=[hbm] * 12,
        out_specs=hbm,
        scratch_shapes=[
            V((N, D), f32),
            V((NT, 7, H // 2, Dh), u32),
            V((B, 7, TP // 2, Dh), u32),
            V((B, 7, TP // 2, Dh), u32),
            V((7, Dh, F // 2), bf16),
            V((7, F // 2, Dh), bf16),
            V((2, 7, Dh // 2, Dh), u32),
            V((7, Dh, Dh), bf16),
            V((K, 4, 8, 128), f32),
            V((TP // W, 4, H, W), f32),
            V((2, H, 128), f32),
            V((2, TP // W - 1, 2, H, 128), f32),
            V((8, 128), jnp.int32),
            V((8, 128), jnp.int32),
            pltpu.SemaphoreType.DMA(()),
        ],
        compiler_params=pltpu.CompilerParams(vmem_limit_bytes=VMEM_LIMIT),
    )(x.reshape(N, D), w_ff1_a, w_ff1_b, w_q, w_k, w_v, w_o, w_pw1, dw, w_pw2, w_ff2_a, w_ff2_b)
    return out.reshape(B, T, D)
```
